```python
import jax
import jax.numpy as jnp

def _softmax(x, axis=-1):
    return jax.nn.softmax(x, axis=axis)
def _gelu(x):
    return jax.nn.gelu(x, approximate=True)
def _silu(x):
    return jax.nn.silu(x)
def _sigmoid(x):
    return jax.nn.sigmoid(x)
def _layernorm(x, axis=-1, eps=1e-5):
    m = jnp.mean(x, axis=axis, keepdims=True)
    v = jnp.var(x, axis=axis, keepdims=True)
    return (x - m) / jnp.sqrt(v + eps)
def _scatter_add(tgt, idx, src, axis=0):
    return tgt.at[idx].add(src)
def _segment_sum(src, seg, n):
    return jax.ops.segment_sum(src, seg, n)
class _Rng:
    def __init__(self, key):
        self._k = key
    def _next(self):
        self._k, sub = jax.random.split(self._k)
        return sub
    def normal(self, shape):
        return jax.random.normal(self._next(), shape, dtype=jnp.bfloat16)
    def randint(self, lo, hi, shape):
        return jax.random.randint(self._next(), shape, lo, hi, dtype=jnp.int32)
    def uniform(self, shape, lo=0.0, hi=1.0):
        return jax.random.uniform(self._next(), shape, jnp.bfloat16, lo, hi)
    def permutation(self, n):
        return jax.random.permutation(self._next(), n)


kernel_name = 'gated_mix__linear_attn_block__moe_arch_mod__prompt'

def setup_inputs():
    _rng = _Rng(jax.random.key(int.from_bytes(__import__("os").urandom(4), "little")))
    _w = (lambda a: (lambda t: t.astype(jnp.bfloat16) if jnp.issubdtype(t.dtype, jnp.floating) else t)(jnp.asarray(a)))
    def _A_setup():
        B, S, D = 1, 2048, 1024
        return {
            "x": _w((lambda *s: _rng.normal(s) * 0.05)(B, S, D)),
            "wqkv": _w((lambda *s: _rng.normal(s) * 0.05)(D, 3 * D)),
            "wo": _w((lambda *s: _rng.normal(s) * 0.05)(D, D)),
        }
    _A_in = _A_setup()

    def _B_setup():
        B, S, D, F, C = 1, 2048, 1024, 3584, 1
        return {
            "x": _w((lambda *s: _rng.normal(s) * 0.05)(B, S, D)),
            "w_r": _w((lambda *s: _rng.normal(s) * 0.05)(D)),
            "w_gate": _w((lambda *s: _rng.normal(s) * 0.05)(D, F)),
            "w_up": _w((lambda *s: _rng.normal(s) * 0.05)(D, F)),
            "w_down": _w((lambda *s: _rng.normal(s) * 0.05)(F, D)),
        }
    _B_in = _B_setup()

    return {
        "A_x": _A_in["x"],
        "A_wqkv": _A_in["wqkv"],
        "A_wo": _A_in["wo"],
        "B_x": _B_in["x"],
        "B_w_r": _B_in["w_r"],
        "B_w_gate": _B_in["w_gate"],
        "B_w_up": _B_in["w_up"],
        "B_w_down": _B_in["w_down"],
        "gate_w": _w((lambda *s: _rng.normal(s) * 0.05)(1024)),
    }

def reference(A_x, A_wqkv, A_wo, B_x, B_w_r, B_w_gate, B_w_up, B_w_down, gate_w):
    def _A_ref(x, wqkv, wo):
        B, S, D = x.shape
        H = 32; Dh = D // H
        qkv = (lambda x, *d: x.transpose(*d))((x @ wqkv).reshape(B, S, 3, H, Dh), 2, 0, 3, 1, 4)
        q, k, v = qkv[0], qkv[1], qkv[2]
        phi = lambda t: jnp.where(t > 0, t + 1, jnp.exp(t)) + 1e-6
        pq, pk = phi(q), phi(k)
        kv = jnp.einsum("bhsd,bhse->bhde", pk, v)
        z = jnp.einsum("bhsd->bhd", pk)
        num = jnp.einsum("bhqd,bhde->bhqe", pq, kv)
        den = jnp.einsum("bhqd,bhd->bhq", pq, z)[..., None] + 1e-6
        o = num / den
        return (lambda x, *d: x.transpose(*d))(o, 0, 2, 1, 3).reshape(B, S, D) @ wo

    def _B_ref(x, w_r, w_gate, w_up, w_down):
        B, S, D = x.shape
        C = 1
        r = x @ w_r
        idx = jnp.argsort(-r, axis=-1)[:, :C]
        idx_e = jnp.repeat(idx.reshape(B, C, 1), D, axis=2)
        x_sel = jnp.take_along_axis(x, idx_e, axis=1)
        g = _silu(x_sel @ w_gate)
        u = x_sel @ w_up
        y = (g * u) @ w_down
        r_sel = _sigmoid(jnp.take_along_axis(r, idx, axis=1))
        y = y * r_sel.reshape(B, C, 1)
        b_off = (jnp.arange(B) * S).reshape(B, 1)
        flat_idx = (idx + b_off).reshape(B * C)
        zero = (x * 0.0).reshape(B * S, D)
        upd = _scatter_add(zero, flat_idx, y.reshape(B * C, D), axis=0)
        return x + upd.reshape(B, S, D)

    x = A_x
    g = _sigmoid((x * gate_w).sum(-1, keepdims=True))
    a = _A_ref(x, A_wqkv, A_wo)
    b = _B_ref(x, B_w_r, B_w_gate, B_w_up, B_w_down)
    return g * a + (1 - g) * b
```

```python
import functools

import jax
import jax.numpy as jnp
from jax import lax
import jax.experimental.pallas as pl
import jax.experimental.pallas.tpu as pltpu

F32 = jnp.float32
BF16 = jnp.bfloat16
HEADS = 32
BIG = 1 << 30
NT = (((1,), (1,)), ((), ()))
TN = (((0,), (0,)), ((), ()))


def _phi(t):
    return jnp.where(t > 0, t + 1.0, jnp.exp(t)) + 1e-6


def _sigmoid(t):
    return 1.0 / (1.0 + jnp.exp(-t))


def _kernel(x_hbm, wqkv_hbm, wo_hbm, wr_ref, wg_hbm, wu_hbm, wd_hbm, gw_ref,
            out_hbm,
            x_v, wq_v, wk_v, wv_v, wo_v, wg_v, wu_v, wd_v,
            wqt_v, wkt_v, g_v, m_v, z_v, xb_v, y_v, o_v,
            sem_x, sem_w, sem_f, sem_o, *, ts, rc1, rc2):
    S, D = x_v.shape
    F = wg_v.shape[1]
    nt = S // ts
    fc = F // nt
    dh = D // HEADS

    def rows(i):
        return pl.ds(pl.multiple_of(i * ts, ts), ts)

    def fcols(i):
        return pl.ds(pl.multiple_of(i * fc, 128), fc)

    def cp_x(i):
        return pltpu.make_async_copy(x_hbm.at[rows(i), :], x_v.at[rows(i), :], sem_x.at[i])

    def cp_w(j, dst):
        return pltpu.make_async_copy(wqkv_hbm.at[:, pl.ds(j * D, D)], dst, sem_w.at[j])

    cp_wo = pltpu.make_async_copy(wo_hbm, wo_v, sem_w.at[3])

    def cp_f(i):
        return (pltpu.make_async_copy(wg_hbm.at[:, fcols(i)], wg_v.at[:, fcols(i)], sem_f.at[3 * i]),
                pltpu.make_async_copy(wu_hbm.at[:, fcols(i)], wu_v.at[:, fcols(i)], sem_f.at[3 * i + 1]),
                pltpu.make_async_copy(wd_hbm.at[fcols(i), :], wd_v.at[fcols(i), :], sem_f.at[3 * i + 2]))

    def cp_o(slot, t):
        return pltpu.make_async_copy(o_v.at[slot], out_hbm.at[rows(t), :], sem_o.at[slot])

    cp_w(1, wk_v).start()
    cp_x(0).start()
    for i in range(1, nt):
        cp_x(i).start()
    cp_w(0, wq_v).start()
    cp_w(2, wv_v).start()
    cp_wo.start()
    for i in range(nt):
        for c in cp_f(i):
            c.start()

    cp_w(1, wk_v).wait()
    for c in range(D // 256):
        wkt_v[c * 256:(c + 1) * 256, :] = wk_v[:, c * 256:(c + 1) * 256].T
    g_v[...] = jnp.zeros_like(g_v)
    z_v[...] = jnp.zeros_like(z_v)

    def phase1(i, carry):
        best, besti = carry
        cp_x(i).wait()
        xt = x_v[rows(i), :]
        for c in range(D // rc1):
            r = slice(c * rc1, (c + 1) * rc1)
            pk = _phi(lax.dot_general(wkt_v[r, :], xt, NT, preferred_element_type=F32))
            zs = pk[:, 0:128]
            for j in range(1, ts // 128):
                zs = zs + pk[:, j * 128:(j + 1) * 128]
            z_v[r, :] += zs
            g_v[r, :] += jnp.dot(pk.astype(BF16), xt, preferred_element_type=F32)
        sc = jnp.sum(xt.astype(F32) * wr_ref[...].astype(F32), axis=-1, keepdims=True)
        sc = sc.astype(BF16).astype(F32)
        m = jnp.max(jnp.where(sc != sc, -jnp.inf, sc), axis=0, keepdims=True)
        tok = lax.broadcasted_iota(jnp.int32, (ts, 1), 0) + i * ts
        mi = jnp.min(jnp.where(sc == m, tok, BIG), axis=0, keepdims=True)
        take = (m > best) | (besti == BIG)
        return jnp.where(take, m, best), jnp.where(take, mi, besti)

    best, besti = lax.fori_loop(
        0, nt, phase1, (jnp.full((1, 1), -jnp.inf, F32), jnp.full((1, 1), BIG, jnp.int32)))
    none = besti == BIG
    r_sel = _sigmoid(jnp.where(none, jnp.nan, best))
    idx = jnp.where(none, 0, besti)[0, 0]

    cp_w(0, wq_v).wait()
    for c in range(D // 256):
        wqt_v[c * 256:(c + 1) * 256, :] = wq_v[:, c * 256:(c + 1) * 256].T
    cp_w(2, wv_v).wait()
    cp_wo.wait()
    same_head = (lax.broadcasted_iota(jnp.int32, (128, 128), 0) // dh
                 == lax.broadcasted_iota(jnp.int32, (128, 128), 1) // dh)
    for g in range(D // 128):
        r = slice(g * 128, (g + 1) * 128)
        kv = jnp.dot(g_v[r, :].astype(BF16), wv_v[:, r], preferred_element_type=F32)
        kv = jnp.where(same_head, kv, 0.0).astype(BF16)
        m_v[r, :] = jnp.dot(kv, wo_v[r, :], preferred_element_type=F32).astype(BF16)
    z_v[...] = jnp.broadcast_to(jnp.sum(z_v[...], axis=-1, keepdims=True), z_v.shape)

    base = pl.multiple_of((idx // 16) * 16, 16)
    slab = x_v[pl.ds(base, 16), :].astype(F32)
    pick = lax.broadcasted_iota(jnp.int32, (16, 1), 0) == idx - base
    xs = jnp.sum(jnp.where(pick, slab, 0.0), axis=0, keepdims=True)
    xb_v[...] = jnp.broadcast_to(xs, (128, D)).T
    y_v[...] = jnp.zeros_like(y_v)
    t_sel = idx // ts

    def phase2(i, _):
        t = lax.rem(t_sel + 1 + i, nt)
        slot = lax.rem(i, 2)
        for c in cp_f(i):
            c.wait()
        xb = jnp.tile(xb_v[...], (1, fc // 128))
        hg = jnp.sum((wg_v[:, fcols(i)].astype(F32) * xb).reshape(D // 8, 8, fc), axis=0)
        hu = jnp.sum((wu_v[:, fcols(i)].astype(F32) * xb).reshape(D // 8, 8, fc), axis=0)
        hg = jnp.sum(hg, axis=0, keepdims=True)
        hu = jnp.sum(hu, axis=0, keepdims=True)
        h = hg * _sigmoid(hg) * hu
        hb = jnp.tile(jnp.broadcast_to(h, (128, fc)).T, (1, D // 128))
        y8 = y_v[...] + jnp.sum((wd_v[fcols(i), :].astype(F32) * hb).reshape(fc // 8, 8, D), axis=0)
        y_v[...] = y8
        y = jnp.sum(y8, axis=0, keepdims=True) * r_sel

        xt = x_v[rows(t), :]
        parts = []
        for c in range(D // rc2):
            r = slice(c * rc2, (c + 1) * rc2)
            pq = _phi(lax.dot_general(wqt_v[r, :], xt, NT, preferred_element_type=F32))
            zb = jnp.tile(z_v[r, :], (1, ts // 128))
            den = jnp.sum((pq * zb).reshape(rc2 // dh, dh, ts), axis=1, keepdims=True) + 1e-6
            o = pq.reshape(rc2 // dh, dh, ts) * (1.0 / den)
            parts.append(o.reshape(rc2, ts).astype(BF16))
        ot = jnp.concatenate(parts, axis=0)
        a = lax.dot_general(ot, m_v[...], TN, preferred_element_type=F32)
        bx = xt.astype(F32)
        gate = _sigmoid(jnp.sum(bx * gw_ref[...].astype(F32), axis=-1, keepdims=True))
        tok = lax.broadcasted_iota(jnp.int32, (ts, 1), 0) + t * ts
        b = bx + (bx * 0.0 + jnp.where(tok == idx, y, 0.0))
        res = (gate * a + (1.0 - gate) * b).astype(BF16)

        @pl.when(i >= 2)
        def _():
            cp_o(slot, t).wait()

        o_v[slot] = res
        cp_o(slot, t).start()
        return 0

    lax.fori_loop(0, nt, phase2, 0)
    for slot in range(2):
        cp_o(slot, 0).wait()


def _build(ts=512, rc1=256, rc2=256, flags=None):
    def run(A_x, A_wqkv, A_wo, B_x, B_w_r, B_w_gate, B_w_up, B_w_down, gate_w):
        B, S, D = A_x.shape
        F = B_w_gate.shape[1]
        nt = S // ts
        hbm = pl.BlockSpec(memory_space=pl.ANY)
        vec = pl.BlockSpec(memory_space=pltpu.VMEM)
        out = pl.pallas_call(
            functools.partial(_kernel, ts=ts, rc1=rc1, rc2=rc2),
            out_shape=jax.ShapeDtypeStruct((S, D), BF16),
            in_specs=[hbm, hbm, hbm, vec, hbm, hbm, hbm, vec],
            out_specs=hbm,
            scratch_shapes=[
                pltpu.VMEM((S, D), BF16),
                pltpu.VMEM((D, D), BF16), pltpu.VMEM((D, D), BF16),
                pltpu.VMEM((D, D), BF16), pltpu.VMEM((D, D), BF16),
                pltpu.VMEM((D, F), BF16), pltpu.VMEM((D, F), BF16), pltpu.VMEM((F, D), BF16),
                pltpu.VMEM((D, D), BF16), pltpu.VMEM((D, D), BF16),
                pltpu.VMEM((D, D), F32), pltpu.VMEM((D, D), BF16),
                pltpu.VMEM((D, 128), F32), pltpu.VMEM((D, 128), F32), pltpu.VMEM((8, D), F32),
                pltpu.VMEM((2, ts, D), BF16),
                pltpu.SemaphoreType.DMA((nt,)),
                pltpu.SemaphoreType.DMA((4,)), pltpu.SemaphoreType.DMA((3 * nt,)),
                pltpu.SemaphoreType.DMA((2,)),
            ],
            compiler_params=pltpu.CompilerParams(
                vmem_limit_bytes=110 * 1024 * 1024, flags=flags),
        )(A_x.reshape(S, D), A_wqkv, A_wo, B_w_r.reshape(1, D),
          B_w_gate, B_w_up, B_w_down, gate_w.reshape(1, D))
        return out.reshape(B, S, D)
    return run


@jax.jit
def pallas_gated_mix__linear_attn_block__moe_arch_mod__prompt_kernel(
    A_x: jax.Array,
    A_wqkv: jax.Array,
    A_wo: jax.Array,
    B_x: jax.Array,
    B_w_r: jax.Array,
    B_w_gate: jax.Array,
    B_w_up: jax.Array,
    B_w_down: jax.Array,
    gate_w: jax.Array,
):
    return _build()(A_x, A_wqkv, A_wo, B_x, B_w_r, B_w_gate, B_w_up, B_w_down, gate_w)
```

```python
import functools

import jax
import jax.numpy as jnp
from jax import lax
import jax.experimental.pallas as pl
import jax.experimental.pallas.tpu as pltpu

F32 = jnp.float32
BF16 = jnp.bfloat16
U32 = jnp.uint32
HEADS = 32
BIG = 1 << 30
NT = (((1,), (1,)), ((), ()))
TN = (((0,), (0,)), ((), ()))


def _phi(t):
    return jnp.where(t > 0, t + 1.0, jnp.exp(t)) + 1e-6


def _sigmoid(t):
    return 1.0 / (1.0 + jnp.exp(-t))


def _pack(v):
    return pltpu.bitcast(v, jnp.uint32)


def _unpack(v):
    return pltpu.bitcast(v, BF16)


def _kernel(x_hbm, wqkv_hbm, wo_hbm, wr_ref, wg_hbm, wu_hbm, wd_hbm, gw_ref,
            out_hbm,
            x_v, wq_v, wk_v, wv_v, wo_v, wg_v, wu_v, wd_v,
            xp_v, wqt_v, wkt_v, pk_v, g_v, m_v, on_v, z_v, gate_v, best_v, besti_v,
            xb_v, hg_v, hu_v, hb_v, y_v, o_v,
            sem_x, sem_w, sem_k, sem_f, sem_o, *, pin, rc, tw, tb, xc, skew, t_sel, t_mid, t_down):
    S, D = x_v.shape
    F = wg_v.shape[1]
    L = 128
    nc = D // rc
    nl = S // tw
    nb = S // tb
    dh = D // HEADS
    fh = F // 2
    gw = tw

    def cp_x(i):
        r = pl.ds(i * xc, xc)
        return pltpu.make_async_copy(x_hbm.at[r, :], x_v.at[r, :], sem_x.at[i])

    def cp_k(c):
        return pltpu.make_async_copy(wqkv_hbm.at[:, pl.ds(D + c * rc, rc)],
                                     wk_v.at[:, pl.ds(c * rc, rc)], sem_k.at[c])

    cp_q = pltpu.make_async_copy(wqkv_hbm.at[:, pl.ds(0, D)], wq_v, sem_w.at[0])
    cp_v = pltpu.make_async_copy(wqkv_hbm.at[:, pl.ds(2 * D, D)], wv_v, sem_w.at[1])
    cp_wo = pltpu.make_async_copy(wo_hbm, wo_v, sem_w.at[2])
    cp_d = pltpu.make_async_copy(wd_hbm, wd_v, sem_f.at[4])

    def cp_up(j):
        f = pl.ds(j * fh, fh)
        return (pltpu.make_async_copy(wg_hbm.at[:, f], wg_v.at[:, f], sem_f.at[2 * j]),
                pltpu.make_async_copy(wu_hbm.at[:, f], wu_v.at[:, f], sem_f.at[2 * j + 1]))

    def cp_o(i, t):
        return pltpu.make_async_copy(o_v.at[pl.ds(i * tb, tb), :],
                                     out_hbm.at[pl.ds(pl.multiple_of(t * tb, tb), tb), :], sem_o.at[i])

    def start(*cps):
        return lambda: [cp.start() for cp in cps] and None

    def wait(*cps):
        return lambda: [cp.wait() for cp in cps] and None

    def packed(ref, lo, n, cols=slice(None)):
        if isinstance(lo, int):
            return _unpack(ref[lo // 2:(lo + n) // 2, cols])
        return _unpack(ref[pl.ds(pl.multiple_of(lo // 2, n // 2), n // 2), cols])

    tokens = []
    never = (pltpu.bitcast(jnp.broadcast_to(gw_ref[:, 0:L], (8, L)).astype(F32), jnp.int32) & 0xFFFF) != 0

    def digest(*vals):
        acc = None
        for v in vals:
            v = v if v.dtype == jnp.int32 else pltpu.bitcast(v, jnp.int32)
            for i in range(v.shape[0] // 8):
                for j in range(v.shape[1] // L):
                    e = v[i * 8:(i + 1) * 8, j * L:(j + 1) * L]
                    acc = e if acc is None else acc ^ e
        return acc

    def tie(v):
        if not tokens:
            return v
        token = pltpu.bitcast(digest(*tokens), F32)
        tokens.clear()
        head = jnp.where(never, token, v[0:8, 0:L])
        if v.shape[1] > L:
            head = jnp.concatenate([head, v[0:8, L:]], axis=1)
        return jnp.concatenate([head, v[8:]], axis=0)

    def k_unit(c, t):
        r = slice(c * rc, (c + 1) * rc)
        kt = lax.dot_general(packed(wkt_v, c * rc, rc), packed(xp_v, t * tw, tw), NT,
                             preferred_element_type=F32)

        def post():
            pk = _phi(tie(kt))
            zs = pk[:, 0:L]
            for j in range(1, tw // L):
                zs = zs + pk[:, j * L:(j + 1) * L]
            if t > 0:
                zs = zs + z_v[r, :]
            if t == nl - 1:
                zs = jnp.broadcast_to(jnp.sum(zs, axis=-1, keepdims=True), zs.shape)
            z_v[r, :] = zs
            pk_v[c % 2, :, t * tw:(t + 1) * tw] = _pack(pk.astype(BF16))
        return post

    def g_unit(c, n):
        cols = slice(n * gw, (n + 1) * gw)
        g = jnp.dot(_unpack(pk_v[c % 2]), packed(xp_v, 0, S, cols), preferred_element_type=F32)

        def post():
            g_v[c * rc // 2:(c + 1) * rc // 2, cols] = _pack(tie(g).astype(BF16))
        return post

    def kv_unit(j):
        q = slice(j * L, (j + 1) * L)
        kv = jnp.dot(packed(g_v, j * L, L), wv_v[:, q], preferred_element_type=F32)

        def post():
            same_head = (lax.broadcasted_iota(jnp.int32, (L, L), 0) // dh
                         == lax.broadcasted_iota(jnp.int32, (L, L), 1) // dh)
            kvm = jnp.where(same_head, kv, 0.0).astype(BF16)
            m = jnp.dot(kvm, wo_v[q, :], preferred_element_type=F32)
            m_v[j * L // 2:(j + 1) * L // 2, :] = _pack(m.astype(BF16))
        return post

    sel = {}

    def block_of(i):
        return lax.rem(sel["blk"] + 1 + i, nb)

    def q_unit(i, c, t):
        r = slice(c * rc, (c + 1) * rc)
        q = lax.dot_general(packed(wqt_v, c * rc, rc), packed(xp_v, block_of(i) * tb + t * tw, tw), NT,
                            preferred_element_type=F32)

        def post():
            pq = _phi(tie(q))
            z = jnp.tile(z_v[r, :], (1, tw // L))
            den = jnp.sum((pq * z).reshape(rc // dh, dh, tw), axis=1, keepdims=True) + 1e-6
            o = (pq.reshape(rc // dh, dh, tw) * (1.0 / den)).reshape(rc, tw)
            lo = (i % 2) * tb + t * tw
            on_v[lo // 2:(lo + tw) // 2, r] = _pack(o.T.astype(BF16))
        return post

    def out_unit(i, n):
        cols = slice(n * L, (n + 1) * L)
        a = jnp.dot(packed(on_v, (i % 2) * tb, tb), _unpack(m_v[:, cols]), preferred_element_type=F32)

        def post():
            lo = block_of(i) * tb
            gate = gate_v[pl.ds(pl.multiple_of(lo, tb), tb), :]
            bx = packed(xp_v, lo, tb, cols).astype(F32)
            upd = bx * 0.0
            if i == nb - 1:
                y = jnp.sum(y_v[:, cols], axis=0, keepdims=True) * sel["w"]
                is_sel = lax.broadcasted_iota(jnp.int32, (tb, L), 0) + lo == sel["idx"]
                upd = upd + jnp.where(is_sel, y, 0.0)
            o_v[i * tb:(i + 1) * tb, cols] = (gate * tie(a) + (1.0 - gate) * (bx + upd)).astype(BF16)
            if n == D // L - 1:
                cp_o(i, block_of(i)).start()
        return post

    def repack(i):
        xp_v[i * xc // 2:(i + 1) * xc // 2, :] = _pack(x_v[i * xc:(i + 1) * xc, :])

    def transpose_w(src, dst, j):
        wt = _pack(src[:, j * L:(j + 1) * L].T)
        dst[j * L // 2:(j + 1) * L // 2, :] = wt
        return digest(wt)

    def route(lo, n):
        xf = packed(xp_v, lo, n).astype(F32)
        gl = jnp.sum(xf * gw_ref[...].astype(F32), axis=-1, keepdims=True)
        gate = jnp.broadcast_to(_sigmoid(gl), (n, L))
        gate_v[lo:lo + n, :] = gate
        sc = jnp.sum(xf * wr_ref[...].astype(F32), axis=-1, keepdims=True)
        sc = jnp.broadcast_to(sc.astype(BF16).astype(F32), (n, L))
        best, besti = best_v[...], besti_v[...]
        for k in range(n // 8):
            s8 = sc[k * 8:(k + 1) * 8, :]
            take = (s8 > best) | ((s8 == best) & (besti == BIG))
            best = jnp.where(take, s8, best)
            besti = jnp.where(take, lax.broadcasted_iota(jnp.int32, (8, L), 0) + (lo + k * 8), besti)
        best_v[...] = best
        besti_v[...] = besti
        return digest(gate, besti)

    def select():
        best, besti = best_v[...], besti_v[...]
        m = jnp.max(best, axis=0, keepdims=True)
        mi = jnp.min(jnp.where(best == m, besti, BIG), axis=0, keepdims=True)
        none = mi == BIG
        sel["w"] = _sigmoid(jnp.where(none, jnp.nan, m))
        sel["idx"] = jnp.where(none, 0, mi)[0, 0]
        sel["blk"] = sel["idx"] // tb

    def gather():
        base = pl.multiple_of((sel["idx"] // 16) * 16, 16)
        slab = x_v[pl.ds(base, 16), :].astype(F32)
        pick = lax.broadcasted_iota(jnp.int32, (16, 1), 0) == sel["idx"] - base
        xs = jnp.sum(jnp.where(pick, slab, 0.0), axis=0, keepdims=True)
        xb_v[...] = jnp.broadcast_to(xs, (L, D)).T

    def ffn_up(j, k, kr=256):
        f, r = slice(j * L, (j + 1) * L), slice(k * kr, (k + 1) * kr)
        xb = xb_v[r, :]
        parts = []
        for w_v, h_v in ((wg_v, hg_v), (wu_v, hu_v)):
            part = jnp.sum((w_v[r, f].astype(F32) * xb).reshape(kr // 8, 8, L), axis=0)
            parts.append(part if k == 0 else h_v[:, f] + part)
            h_v[:, f] = parts[-1]
        return digest(*parts)

    def ffn_act(j):
        f = slice(j * L, (j + 1) * L)
        hg = jnp.sum(hg_v[:, f], axis=0, keepdims=True)
        hu = jnp.sum(hu_v[:, f], axis=0, keepdims=True)
        hb = jnp.broadcast_to(hg * _sigmoid(hg) * hu, (L, L)).T
        hb_v[f, :] = hb
        return digest(hb)

    def ffn_down(j, n, nw=512):
        f, cols = slice(j * L, (j + 1) * L), slice(n * nw, (n + 1) * nw)
        hb = jnp.tile(hb_v[f, :], (1, nw // L))
        part = jnp.sum((wd_v[f, cols].astype(F32) * hb).reshape(L // 8, 8, nw), axis=0)
        part = part if j == 0 else y_v[:, cols] + part
        y_v[:, cols] = part
        return digest(part)

    P = functools.partial
    units, before, after = [], {}, {}
    for c in range(nc):
        units += [P(k_unit, c, t) for t in range(nl)]
        if c > 0:
            units += [P(g_unit, c - 1, n) for n in range(D // gw)]
    units += [P(g_unit, nc - 1, n) for n in range(D // gw)]
    q_units = lambda i: [P(q_unit, i, c, t) for t in range(tb // tw) for c in range(nc)]
    first_q = q_units(0)
    for j in range(D // L):
        units += [P(kv_unit, j)] + first_q[j * len(first_q) // (D // L):(j + 1) * len(first_q) // (D // L)]
    for i in range(nb):
        if i + 1 < nb:
            units += q_units(i + 1)
        units += [P(out_unit, i, n) for n in range(D // L)]
    cost = {k_unit: rc * tw * D, g_unit: rc * gw * S, kv_unit: 2 * L * L * D,
            q_unit: rc * tw * D, out_unit: tb * L * D}
    clock = [0]
    for unit in units:
        clock.append(clock[-1] + cost[unit.func] / (S * D * D))

    def at(time):
        return max(u for u in range(len(units)) if clock[u] <= time)

    def spread(jobs, t0, t1):
        for n, job in enumerate(jobs):
            after.setdefault(at(t0 + (t1 - t0) * n / len(jobs)), []).append(job)

    nx = S // xc
    cp_k(0).start()
    cp_x(0).start()
    cp_x(1).start()
    best_v[...] = jnp.full(best_v.shape, -jnp.inf, F32)
    besti_v[...] = jnp.full(besti_v.shape, BIG, jnp.int32)
    before[0] = [wait(cp_k(0))] + [P(transpose_w, wk_v, wkt_v, j) for j in range(rc // L)]
    for i in range(nx):
        jobs = [wait(cp_x(i)), P(repack, i)]
        if i + 2 < nx:
            jobs.append(start(cp_x(i + 2)))
        if i + 2 == nx:
            jobs.append(start(*[cp_k(c) for c in range(1, nc)]))
        if i + 1 == nx:
            jobs.append(start(*cp_up(0)))
        before.setdefault(i * xc // tw, []).extend(jobs)
    before.setdefault(nl - 1, []).append(wait(*[cp_k(c) for c in range(1, nc)]))
    after.setdefault(nl - 1, []).extend(P(transpose_w, wk_v, wkt_v, j) for j in range(rc // L, 2 * rc // L))
    spread([P(transpose_w, wk_v, wkt_v, j) for j in range(2 * rc // L, D // L)], clock[nl], clock[2 * nl])
    spread([P(route, lo, 32) for lo in range(0, S, 32)], clock[nl], t_sel)
    before.setdefault(at(0.5), []).append(start(cp_q, cp_v, cp_wo))
    before.setdefault(at(0.9), []).append(start(*cp_up(1)))
    before.setdefault(at(1.3), []).append(start(cp_d))
    u_sel = at(t_sel)
    after.setdefault(u_sel, []).append(select)
    after.setdefault(u_sel + 1, []).append(gather)
    before.setdefault(u_sel + 2, []).append(wait(*cp_up(0)))
    ups = lambda j0, j1: [job for j in range(j0, j1)
                          for job in [P(ffn_up, j, k) for k in range(D // 256)] + [P(ffn_act, j)]]
    spread(ups(0, fh // L), clock[u_sel + 2], t_mid)
    before.setdefault(at(t_mid), []).append(wait(*cp_up(1)))
    spread(ups(fh // L, F // L), t_mid, t_down)
    before.setdefault(at(1.5), []).append(wait(cp_q, cp_v, cp_wo))
    spread([P(transpose_w, wq_v, wqt_v, j) for j in range(D // L)], 1.5, 1.95)
    before.setdefault(at(t_down), []).append(wait(cp_d))
    spread([P(ffn_down, j, n) for j in range(F // L) for n in range(D // 512)],
           t_down, clock[len(units) - D // L - 2])

    posts = []
    for u, unit in enumerate(units):
        for job in before.get(u, []):
            job()
        posts.append(unit())
        if len(posts) > skew:
            posts.pop(0)()
        for job in after.get(u, []):
            token = job()
            if token is not None and pin:
                tokens.append(token)
    for post in posts:
        post()
    for i in range(nb):
        cp_o(i, 0).wait()


def _build(rc=256, tw=256, tb=256, xc=256, skew=1, t_sel=1.1, t_mid=2.1, t_down=3.1, pin=1, flags=None):
    def run(A_x, A_wqkv, A_wo, B_x, B_w_r, B_w_gate, B_w_up, B_w_down, gate_w):
        B, S, D = A_x.shape
        F = B_w_gate.shape[1]
        hbm = pl.BlockSpec(memory_space=pl.ANY)
        vec = pl.BlockSpec(memory_space=pltpu.VMEM)
        vmem, dma = pltpu.VMEM, pltpu.SemaphoreType.DMA
        out = pl.pallas_call(
            functools.partial(_kernel, rc=rc, tw=tw, tb=tb, xc=xc, skew=skew,
                              t_sel=t_sel, t_mid=t_mid, t_down=t_down, pin=pin),
            out_shape=jax.ShapeDtypeStruct((S, D), BF16),
            in_specs=[hbm, hbm, hbm, vec, hbm, hbm, hbm, vec],
            out_specs=hbm,
            scratch_shapes=[
                vmem((S, D), BF16),
                vmem((D, D), BF16), vmem((D, D), BF16),
                vmem((D, D), BF16), vmem((D, D), BF16),
                vmem((D, F), BF16), vmem((D, F), BF16), vmem((F, D), BF16),
                vmem((S // 2, D), U32),
                vmem((D // 2, D), U32), vmem((D // 2, D), U32),
                vmem((2, rc // 2, S), U32),
                vmem((D // 2, D), U32), vmem((D // 2, D), U32),
                vmem((tb, D), U32),
                vmem((D, 128), F32), vmem((S, 128), F32),
                vmem((8, 128), F32), vmem((8, 128), jnp.int32),
                vmem((D, 128), F32),
                vmem((8, F), F32), vmem((8, F), F32), vmem((F, 128), F32),
                vmem((8, D), F32),
                vmem((S, D), BF16),
                dma((S // xc,)), dma((3,)), dma((D // rc,)), dma((5,)), dma((S // tb,)),
            ],
            compiler_params=pltpu.CompilerParams(
                vmem_limit_bytes=110 * 1024 * 1024, flags=flags),
        )(A_x.reshape(S, D), A_wqkv, A_wo, B_w_r.reshape(1, D),
          B_w_gate, B_w_up, B_w_down, gate_w.reshape(1, D))
        return out.reshape(B, S, D)
    return run


@jax.jit
def pallas_gated_mix__linear_attn_block__moe_arch_mod__prompt_kernel(
    A_x: jax.Array,
    A_wqkv: jax.Array,
    A_wo: jax.Array,
    B_x: jax.Array,
    B_w_r: jax.Array,
    B_w_gate: jax.Array,
    B_w_up: jax.Array,
    B_w_down: jax.Array,
    gate_w: jax.Array,
):
    return _build()(A_x, A_wqkv, A_wo, B_x, B_w_r, B_w_gate, B_w_up, B_w_down, gate_w)
```

```python
import functools

import jax
import jax.numpy as jnp
from jax import lax
import jax.experimental.pallas as pl
import jax.experimental.pallas.tpu as pltpu

F32 = jnp.float32
BF16 = jnp.bfloat16
U32 = jnp.uint32
HEADS = 32
BIG = 1 << 30
NT = (((1,), (1,)), ((), ()))
TN = (((0,), (0,)), ((), ()))


def _phi(t):
    return jnp.where(t > 0, t + 1.0, jnp.exp(t)) + 1e-6


def _sigmoid(t):
    return 1.0 / (1.0 + jnp.exp(-t))


def _pack(v):
    return pltpu.bitcast(v, jnp.uint32)


def _unpack(v):
    return pltpu.bitcast(v, BF16)


def _kernel(x_hbm, wqkv_hbm, wo_hbm, wr_ref, wg_hbm, wu_hbm, wd_hbm, gw_ref,
            out_hbm,
            x_v, wq_v, wk_v, wv_v, wo_v, wg_v, wu_v, wd_v,
            xp_v, wqt_v, wkt_v, pk_v, g_v, m_v, on_v, z_v, gate_v, best_v, besti_v,
            xb_v, hg_v, hu_v, hb_v, y_v, o_v,
            sem_x, sem_w, sem_k, sem_o, *, pin, t_up, boot, ns, gw, t_route, t_dma, rc, tw, tb, xc, skew, t_sel, t_mid, t_down):
    S, D = x_v.shape
    F = wg_v.shape[1]
    L = 128
    nc = D // rc
    nl = S // tw
    nb = S // tb
    dh = D // HEADS
    fh = F // 2

    def copies(src, dst, sem, rows, cols, shift, n):
        (r0, nr), (c0, ncol) = rows, cols
        return [pltpu.make_async_copy(src.at[pl.ds(r0 + k * nr // n, nr // n), pl.ds(c0 + shift, ncol)],
                                      dst.at[pl.ds(r0 + k * nr // n, nr // n), pl.ds(c0, ncol)], sem)
                for k in range(n)]

    cp_x = lambda i: copies(x_hbm, x_v, sem_x.at[i], (i * xc, xc), (0, D), 0, ns)
    cp_k = lambda c: copies(wqkv_hbm, wk_v, sem_k.at[c], (0, D), (c * rc, rc), D, ns)
    cp_qvo = lambda: (copies(wqkv_hbm, wq_v, sem_w.at[0], (0, D), (0, D), 0, 2)
                      + copies(wqkv_hbm, wv_v, sem_w.at[0], (0, D), (0, D), 2 * D, 2)
                      + copies(wo_hbm, wo_v, sem_w.at[0], (0, D), (0, D), 0, 2))
    cp_up = lambda j: (copies(wg_hbm, wg_v, sem_w.at[1 + j], (0, D), (j * fh, fh), 0, 2)
                       + copies(wu_hbm, wu_v, sem_w.at[1 + j], (0, D), (j * fh, fh), 0, 2))
    cp_d = lambda: copies(wd_hbm, wd_v, sem_w.at[3], (0, F), (0, D), 0, 4)

    def cp_o(i, t, n=None):
        cols = pl.ds(0, D) if n is None else pl.ds(n * L, L)
        return pltpu.make_async_copy(o_v.at[pl.ds(i * tb, tb), cols],
                                     out_hbm.at[pl.ds(pl.multiple_of(t * tb, tb), tb), cols],
                                     sem_o.at[i + (n or 0)])

    def start(*cps):
        return lambda: [cp.start() for cp in cps] and None

    def wait(*cps):
        return lambda: [cp.wait() for cp in cps] and None

    def packed(ref, lo, n, cols=slice(None)):
        if isinstance(lo, int):
            return _unpack(ref[lo // 2:(lo + n) // 2, cols])
        return _unpack(ref[pl.ds(pl.multiple_of(lo // 2, n // 2), n // 2), cols])

    tokens = []
    w_g, w_r = gw_ref[...].astype(F32), wr_ref[...].astype(F32)
    never = (pltpu.bitcast(w_g, jnp.int32) & 0xFFFF) != 0
    w_g, w_r = (jnp.concatenate([w[j:j + 1, :] for j in range(D // L)], axis=1) for w in (w_g, w_r))

    def digest(*vals):
        acc = None
        for v in vals:
            v = v if v.dtype == jnp.int32 else pltpu.bitcast(v, jnp.int32)
            for i in range(v.shape[0] // 8):
                for j in range(v.shape[1] // L):
                    e = v[i * 8:(i + 1) * 8, j * L:(j + 1) * L]
                    acc = e if acc is None else acc ^ e
        return acc

    def tie(v):
        if not tokens:
            return v
        token = pltpu.bitcast(digest(*tokens), F32)
        tokens.clear()
        head = jnp.where(never, token, v[0:8, 0:L])
        if v.shape[1] > L:
            head = jnp.concatenate([head, v[0:8, L:]], axis=1)
        return jnp.concatenate([head, v[8:]], axis=0)

    def k_unit(c, t):
        r = slice(c * rc, (c + 1) * rc)
        xt = x_v[t * tw:(t + 1) * tw, :] if t < 2 else packed(xp_v, t * tw, tw)
        kt = lax.dot_general(packed(wkt_v, c * rc, rc), xt, NT, preferred_element_type=F32)

        def post():
            pk = _phi(tie(kt))
            zs = pk[:, 0:L]
            for j in range(1, tw // L):
                zs = zs + pk[:, j * L:(j + 1) * L]
            if t > 0:
                zs = zs + z_v[r, :]
            if t == nl - 1:
                zs = jnp.broadcast_to(jnp.sum(zs, axis=-1, keepdims=True), zs.shape)
            z_v[r, :] = zs
            pk_v[c * rc // 2:(c + 1) * rc // 2, t * tw:(t + 1) * tw] = _pack(pk.astype(BF16))
        return post

    def g_unit(c, n):
        cols = slice(n * gw, (n + 1) * gw)
        g = jnp.dot(packed(pk_v, c * rc, rc), packed(xp_v, 0, S, cols), preferred_element_type=F32)

        def post():
            g_v[c * rc // 2:(c + 1) * rc // 2, cols] = _pack(tie(g).astype(BF16))
        return post

    def kv_unit(j):
        q = slice(j * L, (j + 1) * L)
        kv = jnp.dot(packed(g_v, j * L, L), wv_v[:, q], preferred_element_type=F32)

        def post():
            same_head = (lax.broadcasted_iota(jnp.int32, (L, L), 0) // dh
                         == lax.broadcasted_iota(jnp.int32, (L, L), 1) // dh)
            kvm = jnp.where(same_head, kv, 0.0).astype(BF16)
            m = jnp.dot(kvm, wo_v[q, :], preferred_element_type=F32)
            m_v[j * L // 2:(j + 1) * L // 2, :] = _pack(m.astype(BF16))
        return post

    sel = {}

    def block_of(i):
        return lax.rem(sel["blk"] + 1 + i, nb)

    def q_unit(i, c, t):
        r = slice(c * rc, (c + 1) * rc)
        q = lax.dot_general(packed(wqt_v, c * rc, rc), packed(xp_v, block_of(i) * tb + t * tw, tw), NT,
                            preferred_element_type=F32)

        def post():
            pq = _phi(tie(q))
            z = jnp.tile(z_v[r, :], (1, tw // L))
            den = jnp.sum((pq * z).reshape(rc // dh, dh, tw), axis=1, keepdims=True) + 1e-6
            o = (pq.reshape(rc // dh, dh, tw) * (1.0 / den)).reshape(rc, tw)
            lo = (i % 2) * tb + t * tw
            on_v[lo // 2:(lo + tw) // 2, r] = _pack(o.T.astype(BF16))
        return post

    def out_unit(i, n):
        cols = slice(n * L, (n + 1) * L)
        a = jnp.dot(packed(on_v, (i % 2) * tb, tb), _unpack(m_v[:, cols]), preferred_element_type=F32)

        def post():
            lo = block_of(i) * tb
            gate = gate_v[pl.ds(pl.multiple_of(lo, tb), tb), :]
            bx = packed(xp_v, lo, tb, cols).astype(F32)
            upd = bx * 0.0
            if i == nb - 1:
                y = jnp.sum(y_v[:, cols], axis=0, keepdims=True) * sel["w"]
                is_sel = lax.broadcasted_iota(jnp.int32, (tb, L), 0) + lo == sel["idx"]
                upd = upd + jnp.where(is_sel, y, 0.0)
            o_v[i * tb:(i + 1) * tb, cols] = (gate * tie(a) + (1.0 - gate) * (bx + upd)).astype(BF16)
            if i == nb - 1:
                cp_o(i, block_of(i), n).start()
            elif n == D // L - 1:
                cp_o(i, block_of(i)).start()
        return post

    def repack(i):
        xp = _pack(x_v[i * L:(i + 1) * L, :])
        xp_v[i * L // 2:(i + 1) * L // 2, :] = xp
        return digest(xp[0:8])

    def transpose_w(src, dst, j):
        wt = _pack(src[:, j * L:(j + 1) * L].T)
        dst[j * L // 2:(j + 1) * L // 2, :] = wt
        return digest(wt)

    def route(lo, n):
        xf = packed(xp_v, lo, n).astype(F32)
        gl = jnp.sum(xf * w_g, axis=-1, keepdims=True)
        gate = jnp.broadcast_to(_sigmoid(gl), (n, L))
        gate_v[lo:lo + n, :] = gate
        sc = jnp.sum(xf * w_r, axis=-1, keepdims=True)
        sc = jnp.broadcast_to(sc.astype(BF16).astype(F32), (n, L))
        best, besti = best_v[...], besti_v[...]
        for k in range(n // 8):
            s8 = sc[k * 8:(k + 1) * 8, :]
            take = (s8 > best) | ((s8 == best) & (besti == BIG))
            best = jnp.where(take, s8, best)
            besti = jnp.where(take, lax.broadcasted_iota(jnp.int32, (8, L), 0) + (lo + k * 8), besti)
        best_v[...] = best
        besti_v[...] = besti
        return digest(gate, besti)

    def select():
        best, besti = best_v[...], besti_v[...]
        m = jnp.max(best, axis=0, keepdims=True)
        mi = jnp.min(jnp.where(best == m, besti, BIG), axis=0, keepdims=True)
        none = mi == BIG
        sel["w"] = _sigmoid(jnp.where(none, jnp.nan, m))
        sel["idx"] = jnp.where(none, 0, mi)[0, 0]
        sel["blk"] = sel["idx"] // tb

    def gather():
        base = pl.multiple_of((sel["idx"] // 16) * 16, 16)
        slab = x_v[pl.ds(base, 16), :].astype(F32)
        pick = lax.broadcasted_iota(jnp.int32, (16, 1), 0) == sel["idx"] - base
        xs = jnp.sum(jnp.where(pick, slab, 0.0), axis=0, keepdims=True)
        xb_v[...] = jnp.broadcast_to(xs, (L, D)).T

    def ffn_up(j, k, kr=256):
        f, r = slice(j * L, (j + 1) * L), slice(k * kr, (k + 1) * kr)
        xb = xb_v[r, :]
        parts = []
        for w_v, h_v in ((wg_v, hg_v), (wu_v, hu_v)):
            part = jnp.sum((w_v[r, f].astype(F32) * xb).reshape(kr // 8, 8, L), axis=0)
            parts.append(part if k == 0 else h_v[:, f] + part)
            h_v[:, f] = parts[-1]
        return digest(*parts)

    def ffn_act(j):
        f = slice(j * L, (j + 1) * L)
        hg = jnp.sum(hg_v[:, f], axis=0, keepdims=True)
        hu = jnp.sum(hu_v[:, f], axis=0, keepdims=True)
        hb = jnp.broadcast_to(hg * _sigmoid(hg) * hu, (L, L)).T
        hb_v[f, :] = hb
        return digest(hb)

    def ffn_down(j, n, nw=512):
        f, cols = slice(j * L, (j + 1) * L), slice(n * nw, (n + 1) * nw)
        hb = jnp.tile(hb_v[f, :], (1, nw // L))
        part = jnp.sum((wd_v[f, cols].astype(F32) * hb).reshape(L // 8, 8, nw), axis=0)
        part = part if j == 0 else y_v[:, cols] + part
        y_v[:, cols] = part
        return digest(part)

    P = functools.partial
    units, before, after = [], {}, {}
    units += [P(k_unit, c, t) for c in range(nc) for t in range(2)]
    units += [P(k_unit, c, t) for t in range(2, nl) for c in range(nc)]
    units += [P(g_unit, c, n) for c in range(nc) for n in range(D // gw)]
    q_units = lambda i: [P(q_unit, i, c, t) for t in range(tb // tw) for c in range(nc)]
    first_q = q_units(0)
    for j in range(D // L):
        units += [P(kv_unit, j)] + first_q[j * len(first_q) // (D // L):(j + 1) * len(first_q) // (D // L)]
    for i in range(nb):
        if i + 1 < nb:
            units += q_units(i + 1)
        units += [P(out_unit, i, n) for n in range(D // L)]
    cost = {k_unit: rc * tw * D, g_unit: rc * gw * S, kv_unit: 2 * L * L * D,
            q_unit: rc * tw * D, out_unit: tb * L * D}
    clock = [0]
    for unit in units:
        clock.append(clock[-1] + cost[unit.func] / (S * D * D))

    def at(time):
        return max(u for u in range(len(units)) if clock[u] <= time)

    def spread(jobs, t0, t1):
        for n, job in enumerate(jobs):
            after.setdefault(at(t0 + (t1 - t0) * n / len(jobs)), []).append(job)

    assert xc == tw and nc == 4 and nl == 8
    xs = lambda *ids: [cp for i in ids for cp in cp_x(i)]
    wkt = lambda c: [P(transpose_w, wk_v, wkt_v, j) for j in range(c * rc // L, (c + 1) * rc // L)]
    start(*cp_k(0), *xs(0, 1))()
    best_v[...] = jnp.full(best_v.shape, -jnp.inf, F32)
    besti_v[...] = jnp.full(besti_v.shape, BIG, jnp.int32)
    before[0] = [wait(*cp_k(0), *xs(0, 1))] + wkt(0)
    if boot == 0:
        before[0].insert(1, start(*cp_k(1), *cp_k(2), *cp_k(3)))
    else:
        for c in range(1, nc):
            cp_k(c)[0].start(priority=boot - 1)
    before[2] = [wait(*cp_k(1), *cp_k(2), *cp_k(3)), start(*xs(2, 3))] + wkt(1)
    after[2], after[3] = wkt(2), wkt(3)
    before[6] = [wait(*xs(2, 3)), start(*xs(4, 5, 6, 7))]
    spread([P(repack, i) for i in (4, 5, 6, 7, 0, 1, 2, 3)], clock[6], clock[10])
    before[12] = [wait(*xs(4, 5, 6, 7)), start(*cp_qvo())]
    spread([P(repack, i) for i in range(8, 16)], clock[12], clock[20])
    spread([P(route, lo, 32) for lo in range(0, S, 32)], t_route, t_sel)
    before.setdefault(at(t_dma[0]), []).append(start(*cp_up(0)))
    before.setdefault(at(t_dma[1]), []).append(start(*cp_up(1)))
    before.setdefault(at(t_dma[2]), []).append(start(*cp_d()))
    u_sel = at(t_sel)
    after.setdefault(u_sel, []).append(select)
    after.setdefault(u_sel + 1, []).append(gather)
    assert at(t_up) >= u_sel + 2
    before.setdefault(at(t_up), []).append(wait(*cp_up(0)))
    ups = lambda j0, j1: [job for j in range(j0, j1)
                          for job in [P(ffn_up, j, k) for k in range(D // 256)] + [P(ffn_act, j)]]
    spread(ups(0, fh // L), t_up, t_mid)
    before.setdefault(at(t_mid), []).append(wait(*cp_up(1)))
    spread(ups(fh // L, F // L), t_mid, t_down)
    before.setdefault(at(1.55), []).append(wait(*cp_qvo()))
    spread([P(transpose_w, wq_v, wqt_v, j) for j in range(D // L)], 1.55, 1.95)
    before.setdefault(at(t_down), []).append(wait(*cp_d()))
    spread([P(ffn_down, j, n) for j in range(F // L) for n in range(D // 512)],
           t_down, clock[len(units) - D // L - 2])

    posts = []
    for u, unit in enumerate(units):
        for job in before.get(u, []):
            job()
        posts.append(unit())
        if len(posts) > skew:
            posts.pop(0)()
        for job in after.get(u, []):
            token = job()
            if token is not None and pin:
                tokens.append(token)
    for post in posts:
        post()
    for i in range(nb - 1):
        cp_o(i, 0).wait()
    for n in range(D // L):
        cp_o(nb - 1, 0, n).wait()


def _build(rc=256, tw=256, tb=256, xc=256, skew=1, t_sel=1.55, t_mid=2.4, t_down=3.1, pin=1, t_up=1.7, boot=2, ns=1, gw=128, t_route=0.6, t_dma=(0.8, 1.4, 2.0), flags=None):
    def run(A_x, A_wqkv, A_wo, B_x, B_w_r, B_w_gate, B_w_up, B_w_down, gate_w):
        B, S, D = A_x.shape
        F = B_w_gate.shape[1]
        hbm = pl.BlockSpec(memory_space=pl.ANY)
        vec = pl.BlockSpec(memory_space=pltpu.VMEM)
        vmem, dma = pltpu.VMEM, pltpu.SemaphoreType.DMA
        out = pl.pallas_call(
            functools.partial(_kernel, rc=rc, tw=tw, tb=tb, xc=xc, skew=skew,
                              t_sel=t_sel, t_mid=t_mid, t_down=t_down, pin=pin, t_up=t_up, boot=boot, ns=ns, gw=gw, t_route=t_route, t_dma=t_dma),
            out_shape=jax.ShapeDtypeStruct((S, D), BF16),
            in_specs=[hbm, hbm, hbm, vec, hbm, hbm, hbm, vec],
            out_specs=hbm,
            scratch_shapes=[
                vmem((S, D), BF16),
                vmem((D, D), BF16), vmem((D, D), BF16),
                vmem((D, D), BF16), vmem((D, D), BF16),
                vmem((D, F), BF16), vmem((D, F), BF16), vmem((F, D), BF16),
                vmem((S // 2, D), U32),
                vmem((D // 2, D), U32), vmem((D // 2, D), U32),
                vmem((D // 2, S), U32),
                vmem((D // 2, D), U32), vmem((D // 2, D), U32),
                vmem((tb, D), U32),
                vmem((D, 128), F32), vmem((S, 128), F32),
                vmem((8, 128), F32), vmem((8, 128), jnp.int32),
                vmem((D, 128), F32),
                vmem((8, F), F32), vmem((8, F), F32), vmem((F, 128), F32),
                vmem((8, D), F32),
                vmem((S, D), BF16),
                dma((S // xc,)), dma((4,)), dma((D // rc,)), dma((S // tb + D // 128 - 1,)),
            ],
            compiler_params=pltpu.CompilerParams(
                vmem_limit_bytes=110 * 1024 * 1024, flags=flags),
        )(A_x.reshape(S, D), A_wqkv, A_wo, B_w_r.reshape(D // 128, 128),
          B_w_gate, B_w_up, B_w_down, gate_w.reshape(D // 128, 128))
        return out.reshape(B, S, D)
    return run


@jax.jit
def pallas_gated_mix__linear_attn_block__moe_arch_mod__prompt_kernel(
    A_x: jax.Array,
    A_wqkv: jax.Array,
    A_wo: jax.Array,
    B_x: jax.Array,
    B_w_r: jax.Array,
    B_w_gate: jax.Array,
    B_w_up: jax.Array,
    B_w_down: jax.Array,
    gate_w: jax.Array,
):
    return _build()(A_x, A_wqkv, A_wo, B_x, B_w_r, B_w_gate, B_w_up, B_w_down, gate_w)
```

```python
import functools

import jax
import jax.numpy as jnp
from jax import lax
import jax.experimental.pallas as pl
import jax.experimental.pallas.tpu as pltpu

F32 = jnp.float32
BF16 = jnp.bfloat16
U32 = jnp.uint32
HEADS = 32
BIG = 1 << 30
NT = (((1,), (1,)), ((), ()))
TN = (((0,), (0,)), ((), ()))


def _phi(t):
    return jnp.where(t > 0, t + 1.0, jnp.exp(t)) + 1e-6


def _sigmoid(t):
    return 1.0 / (1.0 + jnp.exp(-t))


def _pack(v):
    return pltpu.bitcast(v, jnp.uint32)


def _unpack(v):
    return pltpu.bitcast(v, BF16)


def _kernel(x_hbm, wqkv_hbm, wo_hbm, wr_ref, wg_hbm, wu_hbm, wd_hbm, gw_ref,
            out_hbm,
            x_v, wq_v, wk_v, wv_v, wo_v, wg_v, wu_v, wd_v,
            xp_v, wqt_v, wkt_v, pk_v, g_v, m_v, on_v, z_v, gate_v, best_v, besti_v,
            xb_v, hg_v, hu_v, hb_v, y_v, o_v,
            sem_x, sem_w, sem_k, sem_o, *, t_up, t_q, boot, ns, gw, lead, rc, tw, tb, xc, skew, t_sel, t_mid, t_down):
    S, D = x_v.shape
    F = wg_v.shape[1]
    L = 128
    nc = D // rc
    nl = S // tw
    nb = S // tb
    dh = D // HEADS
    fh = F // 2

    def copies(src, dst, sem, rows, cols, shift, n):
        (r0, nr), (c0, ncol) = rows, cols
        return [pltpu.make_async_copy(src.at[pl.ds(r0 + k * nr // n, nr // n), pl.ds(c0 + shift, ncol)],
                                      dst.at[pl.ds(r0 + k * nr // n, nr // n), pl.ds(c0, ncol)], sem)
                for k in range(n)]

    cp_x = lambda i: copies(x_hbm, x_v, sem_x.at[i], (i * xc, xc), (0, D), 0, ns)
    cp_k = lambda c: copies(wqkv_hbm, wk_v, sem_k.at[c], (0, D), (c * rc, rc), D, ns)
    cp_qvo = lambda: (copies(wqkv_hbm, wq_v, sem_w.at[0], (0, D), (0, D), 0, 2)
                      + copies(wqkv_hbm, wv_v, sem_w.at[0], (0, D), (0, D), 2 * D, 2)
                      + copies(wo_hbm, wo_v, sem_w.at[0], (0, D), (0, D), 0, 2))
    cp_up = lambda j: (copies(wg_hbm, wg_v, sem_w.at[1 + j], (0, D), (j * fh, fh), 0, 2)
                       + copies(wu_hbm, wu_v, sem_w.at[1 + j], (0, D), (j * fh, fh), 0, 2))
    cp_d = lambda: copies(wd_hbm, wd_v, sem_w.at[3], (0, F), (0, D), 0, 4)

    def cp_o(i, t, n=None):
        cols = pl.ds(0, D) if n is None else pl.ds(n * L, L)
        return pltpu.make_async_copy(o_v.at[pl.ds(i * tb, tb), cols],
                                     out_hbm.at[pl.ds(pl.multiple_of(t * tb, tb), tb), cols],
                                     sem_o.at[i + (n or 0)])

    def start(*cps):
        return lambda: [cp.start() for cp in cps] and None

    def wait(*cps):
        return lambda: [cp.wait() for cp in cps] and None

    def packed(ref, lo, n, cols=slice(None)):
        if isinstance(lo, int):
            return _unpack(ref[lo // 2:(lo + n) // 2, cols])
        return _unpack(ref[pl.ds(pl.multiple_of(lo // 2, n // 2), n // 2), cols])

    tokens = []
    w_g, w_r = gw_ref[...].astype(F32), wr_ref[...].astype(F32)
    never = (pltpu.bitcast(w_g, jnp.int32) & 0xFFFF) != 0
    w_g, w_r = (jnp.concatenate([w[j:j + 1, :] for j in range(D // L)], axis=1) for w in (w_g, w_r))

    def digest(*vals):
        acc = None
        for v in vals:
            v = v if v.dtype == jnp.int32 else pltpu.bitcast(v, jnp.int32)
            for i in range(v.shape[0] // 8):
                for j in range(v.shape[1] // L):
                    e = v[i * 8:(i + 1) * 8, j * L:(j + 1) * L]
                    acc = e if acc is None else acc ^ e
        return acc

    def tie(v):
        if not tokens:
            return v
        head = jnp.where(never, pltpu.bitcast(digest(*tokens), v.dtype), v[0:8, 0:L])
        tokens.clear()
        if v.shape[1] > L:
            head = jnp.concatenate([head, v[0:8, L:]], axis=1)
        return jnp.concatenate([head, v[8:]], axis=0)

    def k_unit(c, t):
        r = slice(c * rc, (c + 1) * rc)
        xt = x_v[t * tw:(t + 1) * tw, :] if t < 2 else packed(xp_v, t * tw, tw)
        more = 8 if c == nc - 1 else 0
        w = _unpack(tie(wkt_v[c * rc // 2:(c + 1) * rc // 2 + more, :]))
        kt = lax.dot_general(w, xt, NT, preferred_element_type=F32)

        def post():
            if more:
                route(t * tw, kt[rc:rc + 8], kt[rc + 8:])
            pk = _phi(kt[:rc])
            zs = pk[:, 0:L]
            for j in range(1, tw // L):
                zs = zs + pk[:, j * L:(j + 1) * L]
            if t > 0:
                zs = zs + z_v[r, :]
            if t == nl - 1:
                zs = jnp.broadcast_to(jnp.sum(zs, axis=-1, keepdims=True), zs.shape)
            z_v[r, :] = zs
            pk_v[c * rc // 2:(c + 1) * rc // 2, t * tw:(t + 1) * tw] = _pack(pk.astype(BF16))
        return post

    def g_unit(c, n):
        cols = slice(n * gw, (n + 1) * gw)
        g = jnp.dot(packed(pk_v, c * rc, rc), packed(xp_v, 0, S, cols), preferred_element_type=F32)

        def post():
            g_v[c * rc // 2:(c + 1) * rc // 2, cols] = _pack(tie(g).astype(BF16))
        return post

    def kv_unit(j):
        q = slice(j * L, (j + 1) * L)
        kv = jnp.dot(packed(g_v, j * L, L), wv_v[:, q], preferred_element_type=F32)

        def post():
            same_head = (lax.broadcasted_iota(jnp.int32, (L, L), 0) // dh
                         == lax.broadcasted_iota(jnp.int32, (L, L), 1) // dh)
            kvm = jnp.where(same_head, kv, 0.0).astype(BF16)
            m = jnp.dot(kvm, wo_v[q, :], preferred_element_type=F32)
            m_v[j * L // 2:(j + 1) * L // 2, :] = _pack(m.astype(BF16))
        return post

    sel = {}

    def block_of(i):
        return lax.rem(sel["blk"] + 1 + i, nb)

    def q_unit(i, c, t):
        r = slice(c * rc, (c + 1) * rc)
        q = lax.dot_general(packed(wqt_v, c * rc, rc), packed(xp_v, block_of(i) * tb + t * tw, tw), NT,
                            preferred_element_type=F32)

        def post():
            pq = _phi(tie(q))
            z = jnp.tile(z_v[r, :], (1, tw // L))
            den = jnp.sum((pq * z).reshape(rc // dh, dh, tw), axis=1, keepdims=True) + 1e-6
            o = (pq.reshape(rc // dh, dh, tw) * (1.0 / den)).reshape(rc, tw)
            lo = (i % 2) * tb + t * tw
            on_v[lo // 2:(lo + tw) // 2, r] = _pack(o.T.astype(BF16))
        return post

    def out_unit(i, n):
        cols = slice(n * L, (n + 1) * L)
        a = jnp.dot(packed(on_v, (i % 2) * tb, tb), _unpack(m_v[:, cols]), preferred_element_type=F32)

        def post():
            lo = block_of(i) * tb
            gate = gate_v[pl.ds(pl.multiple_of(lo, tb), tb), :]
            bx = packed(xp_v, lo, tb, cols).astype(F32)
            upd = bx * 0.0
            if i == nb - 1:
                y = jnp.sum(y_v[:, cols], axis=0, keepdims=True) * sel["w"]
                is_sel = lax.broadcasted_iota(jnp.int32, (tb, L), 0) + lo == sel["idx"]
                upd = upd + jnp.where(is_sel, y, 0.0)
            o_v[i * tb:(i + 1) * tb, cols] = (gate * tie(a) + (1.0 - gate) * (bx + upd)).astype(BF16)
            if i == nb - 1:
                cp_o(i, block_of(i), n).start()
            elif n == D // L - 1:
                cp_o(i, block_of(i)).start()
        return post

    def repack(i):
        xp = _pack(x_v[i * L:(i + 1) * L, :])
        xp_v[i * L // 2:(i + 1) * L // 2, :] = xp
        return digest(xp)

    def transpose_w(src, dst, j):
        wt = _pack(src[:, j * L:(j + 1) * L].T)
        dst[j * L // 2:(j + 1) * L // 2, :] = wt
        return digest(wt)

    def route(lo, score, logit):
        score = score.astype(BF16).astype(F32)
        gate = _sigmoid(logit)
        best, besti = best_v[...], besti_v[...]
        for k in range(tw // L):
            s8 = score[:, k * L:(k + 1) * L]
            take = (s8 > best) | ((s8 == best) & (besti == BIG))
            best = jnp.where(take, s8, best)
            besti = jnp.where(take, lax.broadcasted_iota(jnp.int32, (8, L), 1) + (lo + k * L), besti)
            gate_v[lo + k * L:lo + (k + 1) * L, :] = jnp.tile(gate[:, k * L:(k + 1) * L], (L // 8, 1)).T
        best_v[...] = best
        besti_v[...] = besti

    def select():
        best, besti = best_v[...], besti_v[...]
        m = jnp.max(best[0:1], axis=1, keepdims=True)
        mi = jnp.min(jnp.where(best[0:1] == m, besti[0:1], BIG), axis=1, keepdims=True)
        none = mi == BIG
        sel["w"] = _sigmoid(jnp.where(none, jnp.nan, m))
        sel["idx"] = jnp.where(none, 0, mi)[0, 0]
        sel["blk"] = sel["idx"] // tb

    def gather():
        base = pl.multiple_of((sel["idx"] // 16) * 16, 16)
        slab = x_v[pl.ds(base, 16), :].astype(F32)
        pick = lax.broadcasted_iota(jnp.int32, (16, 1), 0) == sel["idx"] - base
        xs = jnp.sum(jnp.where(pick, slab, 0.0), axis=0, keepdims=True)
        xb_v[...] = jnp.broadcast_to(xs, (L, D)).T

    def ffn_up(j, k, kr=256):
        f, r = slice(j * L, (j + 1) * L), slice(k * kr, (k + 1) * kr)
        xb = xb_v[r, :]
        parts = []
        for w_v, h_v in ((wg_v, hg_v), (wu_v, hu_v)):
            part = jnp.sum((w_v[r, f].astype(F32) * xb).reshape(kr // 8, 8, L), axis=0)
            parts.append(part if k == 0 else h_v[:, f] + part)
            h_v[:, f] = parts[-1]
        return digest(*parts)

    def ffn_act(j):
        f = slice(j * L, (j + 1) * L)
        hg = jnp.sum(hg_v[:, f], axis=0, keepdims=True)
        hu = jnp.sum(hu_v[:, f], axis=0, keepdims=True)
        hb = jnp.broadcast_to(hg * _sigmoid(hg) * hu, (L, L)).T
        hb_v[f, :] = hb
        return digest(hb)

    def ffn_down(j, n, nw=512):
        f, cols = slice(j * L, (j + 1) * L), slice(n * nw, (n + 1) * nw)
        hb = jnp.tile(hb_v[f, :], (1, nw // L))
        part = jnp.sum((wd_v[f, cols].astype(F32) * hb).reshape(L // 8, 8, nw), axis=0)
        part = part if j == 0 else y_v[:, cols] + part
        y_v[:, cols] = part
        return digest(part)

    P = functools.partial
    units, before, after = [], {}, {}
    units += [P(k_unit, c, t) for c in range(nc) for t in range(2)]
    units += [P(k_unit, c, t) for t in range(2, nl) for c in range(nc)]
    units += [P(g_unit, c, n) for c in range(nc) for n in range(D // gw)]
    q_units = lambda i: [P(q_unit, i, c, t) for t in range(tb // tw) for c in range(nc)]
    first_q = q_units(0)
    for j in range(D // L):
        units += [P(kv_unit, j)] + first_q[j * len(first_q) // (D // L):(j + 1) * len(first_q) // (D // L)]
    for i in range(nb):
        if i + 1 < nb:
            units += q_units(i + 1)
        units += [P(out_unit, i, n) for n in range(D // L)]
    cost = {k_unit: rc * tw * D, g_unit: rc * gw * S, kv_unit: 2 * L * L * D,
            q_unit: rc * tw * D, out_unit: tb * L * D}
    clock = [0]
    for unit in units:
        clock.append(clock[-1] + cost[unit.func] / (S * D * D))

    def at(time):
        return max(u for u in range(len(units)) if clock[u] <= time)

    def spread(jobs, t0, t1):
        for n, job in enumerate(jobs):
            after.setdefault(at(t0 + (t1 - t0) * n / len(jobs)), []).append(job)

    assert xc == tw and nc == 4 and nl == 8
    xs = lambda *ids: [cp for i in ids for cp in cp_x(i)]
    wkt = lambda c: [P(transpose_w, wk_v, wkt_v, j) for j in range(c * rc // L, (c + 1) * rc // L)]
    start(*cp_k(0), *xs(0, 1))()
    best_v[...] = jnp.full(best_v.shape, -jnp.inf, F32)
    besti_v[...] = jnp.full(besti_v.shape, BIG, jnp.int32)
    wkt_v[D // 2:, :] = _pack(jnp.concatenate(
        [jnp.broadcast_to(w_r, (8, D)), jnp.broadcast_to(w_g, (8, D))], axis=0).astype(BF16))
    before[0] = [wait(*cp_k(0), *xs(0, 1))] + wkt(0)
    if boot == 0:
        before[0].insert(1, start(*cp_k(1), *cp_k(2), *cp_k(3)))
    else:
        for c in range(1, nc):
            cp_k(c)[0].start(priority=boot - 1)
    before[2] = [wait(*cp_k(1), *cp_k(2), *cp_k(3)), start(*xs(2, 3))] + wkt(1)
    after[2], after[3] = wkt(2), wkt(3)
    before[6] = [wait(*xs(2, 3)), start(*xs(4, 5, 6, 7))]
    spread([P(repack, i) for i in (4, 5, 6, 7, 0, 1, 2, 3)], clock[6], clock[10])
    before[12] = [wait(*xs(4, 5, 6, 7)), start(*cp_qvo())]
    spread([P(repack, i) for i in range(8, 16)], clock[12], clock[20])
    before.setdefault(at(t_q - lead), []).append(start(*cp_up(0)))
    before.setdefault(at(t_up - lead), []).append(start(*cp_up(1)))
    before.setdefault(at(t_mid - lead), []).append(start(*cp_d()))
    u_sel = at(t_sel)
    after.setdefault(u_sel, []).append(select)
    after.setdefault(u_sel + 1, []).append(gather)
    assert at(t_up) >= u_sel + 2
    before.setdefault(at(t_up), []).append(wait(*cp_up(0)))
    ups = lambda j0, j1: [job for j in range(j0, j1)
                          for job in [P(ffn_up, j, k) for k in range(D // 256)] + [P(ffn_act, j)]]
    spread(ups(0, fh // L), t_up, t_mid)
    before.setdefault(at(t_mid), []).append(wait(*cp_up(1)))
    spread(ups(fh // L, F // L), t_mid, t_down)
    before.setdefault(at(t_q), []).append(wait(*cp_qvo()))
    spread([P(transpose_w, wq_v, wqt_v, j) for j in range(D // L)], t_q, t_up)
    before.setdefault(at(t_down), []).append(wait(*cp_d()))
    spread([P(ffn_down, j, n) for j in range(F // L) for n in range(D // 512)],
           t_down, clock[len(units) - D // L - 2])

    posts = []
    for u, unit in enumerate(units):
        for job in before.get(u, []):
            job()
        posts.append(unit())
        if len(posts) > skew:
            posts.pop(0)()
        for job in after.get(u, []):
            token = job()
            if token is not None:
                tokens.append(token)
    for post in posts:
        post()
    for i in range(nb - 1):
        cp_o(i, 0).wait()
    for n in range(D // L):
        cp_o(nb - 1, 0, n).wait()


def _build(rc=256, tw=256, tb=256, xc=256, skew=1, t_sel=1.05, t_mid=2.3, t_down=3.0, t_up=1.65, t_q=1.0, boot=2, ns=1, gw=128, lead=0.05, flags=None):
    def run(A_x, A_wqkv, A_wo, B_x, B_w_r, B_w_gate, B_w_up, B_w_down, gate_w):
        B, S, D = A_x.shape
        F = B_w_gate.shape[1]
        hbm = pl.BlockSpec(memory_space=pl.ANY)
        vec = pl.BlockSpec(memory_space=pltpu.VMEM)
        vmem, dma = pltpu.VMEM, pltpu.SemaphoreType.DMA
        out = pl.pallas_call(
            functools.partial(_kernel, rc=rc, tw=tw, tb=tb, xc=xc, skew=skew,
                              t_sel=t_sel, t_mid=t_mid, t_down=t_down, t_up=t_up, t_q=t_q, boot=boot, ns=ns, gw=gw, lead=lead),
            out_shape=jax.ShapeDtypeStruct((S, D), BF16),
            in_specs=[hbm, hbm, hbm, vec, hbm, hbm, hbm, vec],
            out_specs=hbm,
            scratch_shapes=[
                vmem((S, D), BF16),
                vmem((D, D), BF16), vmem((D, D), BF16),
                vmem((D, D), BF16), vmem((D, D), BF16),
                vmem((D, F), BF16), vmem((D, F), BF16), vmem((F, D), BF16),
                vmem((S // 2, D), U32),
                vmem((D // 2, D), U32), vmem((D // 2 + 8, D), U32),
                vmem((D // 2, S), U32),
                vmem((D // 2, D), U32), vmem((D // 2, D), U32),
                vmem((tb, D), U32),
                vmem((D, 128), F32), vmem((S, 128), F32),
                vmem((8, 128), F32), vmem((8, 128), jnp.int32),
                vmem((D, 128), F32),
                vmem((8, F), F32), vmem((8, F), F32), vmem((F, 128), F32),
                vmem((8, D), F32),
                vmem((S, D), BF16),
                dma((S // xc,)), dma((4,)), dma((D // rc,)), dma((S // tb + D // 128 - 1,)),
            ],
            compiler_params=pltpu.CompilerParams(
                vmem_limit_bytes=110 * 1024 * 1024, flags=flags),
        )(A_x.reshape(S, D), A_wqkv, A_wo, B_w_r.reshape(D // 128, 128),
          B_w_gate, B_w_up, B_w_down, gate_w.reshape(D // 128, 128))
        return out.reshape(B, S, D)
    return run


@jax.jit
def pallas_gated_mix__linear_attn_block__moe_arch_mod__prompt_kernel(
    A_x: jax.Array,
    A_wqkv: jax.Array,
    A_wo: jax.Array,
    B_x: jax.Array,
    B_w_r: jax.Array,
    B_w_gate: jax.Array,
    B_w_up: jax.Array,
    B_w_down: jax.Array,
    gate_w: jax.Array,
):
    return _build()(A_x, A_wqkv, A_wo, B_x, B_w_r, B_w_gate, B_w_up, B_w_down, gate_w)
```

```python
import functools

import jax
import jax.numpy as jnp
from jax import lax
import jax.experimental.pallas as pl
import jax.experimental.pallas.tpu as pltpu

F32 = jnp.float32
BF16 = jnp.bfloat16
U32 = jnp.uint32
HEADS = 32
BIG = 1 << 30
NT = (((1,), (1,)), ((), ()))
TN = (((0,), (0,)), ((), ()))


def _phi(t):
    return jnp.where(t > 0, t + 1.0, jnp.exp(t)) + 1e-6


def _sigmoid(t):
    return 1.0 / (1.0 + jnp.exp(-t))


def _pack(v):
    return pltpu.bitcast(v, jnp.uint32)


def _unpack(v):
    return pltpu.bitcast(v, BF16)


def _kernel(x_hbm, wqkv_hbm, wo_hbm, wr_ref, wg_hbm, wu_hbm, wd_hbm, gw_ref,
            out_hbm,
            x_v, wq_v, wk_v, wv_v, wo_v, wg_v, wu_v, wd_v,
            xp_v, wqt_v, wkt_v, pk_v, g_v, m_v, on_v, z_v, gate_v, best_v, besti_v,
            xb_v, hg_v, hu_v, hb_v, y_v, o_v,
            sem_x, sem_w, sem_k, sem_o, *, t_up, t_q, boot, ns, gw, lead, rc, tw, tb, xc, skew, t_sel, t_mid, t_down):
    S, D = x_v.shape
    F = wg_v.shape[1]
    L = 128
    nc = D // rc
    nl = S // tw
    nb = S // tb
    dh = D // HEADS
    fh = F // 2

    def copies(src, dst, sem, rows, cols, shift, n):
        (r0, nr), (c0, ncol) = rows, cols
        return [pltpu.make_async_copy(src.at[pl.ds(r0 + k * nr // n, nr // n), pl.ds(c0 + shift, ncol)],
                                      dst.at[pl.ds(r0 + k * nr // n, nr // n), pl.ds(c0, ncol)], sem)
                for k in range(n)]

    cp_x = lambda i: copies(x_hbm, x_v, sem_x.at[i], (i * xc, xc), (0, D), 0, ns if i == 0 else 1)
    cp_k = lambda c: copies(wqkv_hbm, wk_v, sem_k.at[c], (0, D), (c * rc, rc), D, ns if c == 0 else 1)
    cp_qvo = lambda: (copies(wqkv_hbm, wq_v, sem_w.at[0], (0, D), (0, D), 0, 2)
                      + copies(wqkv_hbm, wv_v, sem_w.at[0], (0, D), (0, D), 2 * D, 2)
                      + copies(wo_hbm, wo_v, sem_w.at[0], (0, D), (0, D), 0, 2))
    cp_up = lambda j: (copies(wg_hbm, wg_v, sem_w.at[1 + j], (0, D), (j * fh, fh), 0, 2)
                       + copies(wu_hbm, wu_v, sem_w.at[1 + j], (0, D), (j * fh, fh), 0, 2))
    cp_d = lambda: copies(wd_hbm, wd_v, sem_w.at[3], (0, F), (0, D), 0, 4)

    def cp_o(i, t, n=None):
        cols = pl.ds(0, D) if n is None else pl.ds(n * L, L)
        return pltpu.make_async_copy(o_v.at[pl.ds(i * tb, tb), cols],
                                     out_hbm.at[pl.ds(pl.multiple_of(t * tb, tb), tb), cols],
                                     sem_o.at[i + (n or 0)])

    def start(*cps):
        return lambda: [cp.start() for cp in cps] and None

    def wait(*cps):
        return lambda: [cp.wait() for cp in cps] and None

    def packed(ref, lo, n, cols=slice(None)):
        if isinstance(lo, int):
            return _unpack(ref[lo // 2:(lo + n) // 2, cols])
        return _unpack(ref[pl.ds(pl.multiple_of(lo // 2, n // 2), n // 2), cols])

    tokens = []
    w_g, w_r = gw_ref[...].astype(F32), wr_ref[...].astype(F32)
    never = (pltpu.bitcast(w_g, jnp.int32) & 0xFFFF) != 0
    w_g, w_r = (jnp.concatenate([w[j:j + 1, :] for j in range(D // L)], axis=1) for w in (w_g, w_r))

    def digest(*vals):
        acc = None
        for v in vals:
            v = v if v.dtype == jnp.int32 else pltpu.bitcast(v, jnp.int32)
            for i in range(v.shape[0] // 8):
                for j in range(v.shape[1] // L):
                    e = v[i * 8:(i + 1) * 8, j * L:(j + 1) * L]
                    acc = e if acc is None else acc ^ e
        return acc

    def tie(v):
        if not tokens:
            return v
        head = jnp.where(never, pltpu.bitcast(digest(*tokens), v.dtype), v[0:8, 0:L])
        tokens.clear()
        if v.shape[1] > L:
            head = jnp.concatenate([head, v[0:8, L:]], axis=1)
        return jnp.concatenate([head, v[8:]], axis=0)

    def k_unit(c, t):
        r = slice(c * rc, (c + 1) * rc)
        xt = x_v[t * tw:(t + 1) * tw, :] if t < 2 else packed(xp_v, t * tw, tw)
        more = 8 if c == nc - 1 else 0
        w = _unpack(tie(wkt_v[c * rc // 2:(c + 1) * rc // 2 + more, :]))
        kt = lax.dot_general(w, xt, NT, preferred_element_type=F32)

        def post():
            if more:
                route(t * tw, kt[rc:rc + 8], kt[rc + 8:])
            pk = _phi(kt[:rc])
            zs = pk[:, 0:L]
            for j in range(1, tw // L):
                zs = zs + pk[:, j * L:(j + 1) * L]
            if t > 0:
                zs = zs + z_v[r, :]
            if t == nl - 1:
                zs = jnp.broadcast_to(jnp.sum(zs, axis=-1, keepdims=True), zs.shape)
            z_v[r, :] = zs
            pk_v[c * rc // 2:(c + 1) * rc // 2, t * tw:(t + 1) * tw] = _pack(pk.astype(BF16))
        return post

    def g_unit(c, n):
        cols = slice(n * gw, (n + 1) * gw)
        g = jnp.dot(packed(pk_v, c * rc, rc), packed(xp_v, 0, S, cols), preferred_element_type=F32)

        def post():
            g_v[c * rc // 2:(c + 1) * rc // 2, cols] = _pack(tie(g).astype(BF16))
        return post

    def kv_unit(j):
        q = slice(j * L, (j + 1) * L)
        kv = jnp.dot(packed(g_v, j * L, L), wv_v[:, q], preferred_element_type=F32)

        def post():
            same_head = (lax.broadcasted_iota(jnp.int32, (L, L), 0) // dh
                         == lax.broadcasted_iota(jnp.int32, (L, L), 1) // dh)
            kvm = jnp.where(same_head, kv, 0.0).astype(BF16)
            m = jnp.dot(kvm, wo_v[q, :], preferred_element_type=F32)
            m_v[j * L // 2:(j + 1) * L // 2, :] = _pack(m.astype(BF16))
        return post

    sel = {}

    def block_of(i):
        return lax.rem(sel["blk"] + 1 + i, nb)

    def q_unit(i, c, t):
        r = slice(c * rc, (c + 1) * rc)
        q = lax.dot_general(packed(wqt_v, c * rc, rc), packed(xp_v, block_of(i) * tb + t * tw, tw), NT,
                            preferred_element_type=F32)

        def post():
            pq = _phi(tie(q))
            z = jnp.tile(z_v[r, :], (1, tw // L))
            den = jnp.sum((pq * z).reshape(rc // dh, dh, tw), axis=1, keepdims=True) + 1e-6
            o = (pq.reshape(rc // dh, dh, tw) * (1.0 / den)).reshape(rc, tw)
            lo = (i % 2) * tb + t * tw
            on_v[lo // 2:(lo + tw) // 2, r] = _pack(o.T.astype(BF16))
        return post

    def out_unit(i, n):
        cols = slice(n * L, (n + 1) * L)
        a = jnp.dot(packed(on_v, (i % 2) * tb, tb), _unpack(m_v[:, cols]), preferred_element_type=F32)

        def post():
            lo = block_of(i) * tb
            gate = gate_v[pl.ds(pl.multiple_of(lo, tb), tb), :]
            bx = packed(xp_v, lo, tb, cols).astype(F32)
            upd = bx * 0.0
            if i == nb - 1:
                y = jnp.sum(y_v[:, cols], axis=0, keepdims=True) * sel["w"]
                is_sel = lax.broadcasted_iota(jnp.int32, (tb, L), 0) + lo == sel["idx"]
                upd = upd + jnp.where(is_sel, y, 0.0)
            o_v[i * tb:(i + 1) * tb, cols] = (gate * tie(a) + (1.0 - gate) * (bx + upd)).astype(BF16)
            if i == nb - 1:
                cp_o(i, block_of(i), n).start()
            elif n == D // L - 1:
                cp_o(i, block_of(i)).start()
        return post

    def repack(i):
        xp = _pack(x_v[i * L:(i + 1) * L, :])
        xp_v[i * L // 2:(i + 1) * L // 2, :] = xp
        return digest(xp)

    def transpose_w(src, dst, j):
        wt = _pack(src[:, j * L:(j + 1) * L].T)
        dst[j * L // 2:(j + 1) * L // 2, :] = wt
        return digest(wt)

    def route(lo, score, logit):
        score = score.astype(BF16).astype(F32)
        gate = _sigmoid(logit)
        best, besti = best_v[...], besti_v[...]
        for k in range(tw // L):
            s8 = score[:, k * L:(k + 1) * L]
            take = (s8 > best) | ((s8 == best) & (besti == BIG))
            best = jnp.where(take, s8, best)
            besti = jnp.where(take, lax.broadcasted_iota(jnp.int32, (8, L), 1) + (lo + k * L), besti)
            gate_v[lo + k * L:lo + (k + 1) * L, :] = jnp.tile(gate[:, k * L:(k + 1) * L], (L // 8, 1)).T
        best_v[...] = best
        besti_v[...] = besti

    def select():
        best, besti = best_v[...], besti_v[...]
        m = jnp.max(best[0:1], axis=1, keepdims=True)
        mi = jnp.min(jnp.where(best[0:1] == m, besti[0:1], BIG), axis=1, keepdims=True)
        none = mi == BIG
        sel["w"] = _sigmoid(jnp.where(none, jnp.nan, m))
        sel["idx"] = jnp.where(none, 0, mi)[0, 0]
        sel["blk"] = sel["idx"] // tb

    def gather():
        base = pl.multiple_of((sel["idx"] // 16) * 16, 16)
        slab = x_v[pl.ds(base, 16), :].astype(F32)
        pick = lax.broadcasted_iota(jnp.int32, (16, 1), 0) == sel["idx"] - base
        xs = jnp.sum(jnp.where(pick, slab, 0.0), axis=0, keepdims=True)
        xb_v[...] = jnp.broadcast_to(xs, (L, D)).T

    def ffn_up(j, k, kr=256):
        f, r = slice(j * L, (j + 1) * L), slice(k * kr, (k + 1) * kr)
        xb = xb_v[r, :]
        parts = []
        for w_v, h_v in ((wg_v, hg_v), (wu_v, hu_v)):
            part = jnp.sum((w_v[r, f].astype(F32) * xb).reshape(kr // 8, 8, L), axis=0)
            parts.append(part if k == 0 else h_v[:, f] + part)
            h_v[:, f] = parts[-1]
        return digest(*parts)

    def ffn_act(j):
        f = slice(j * L, (j + 1) * L)
        hg = jnp.sum(hg_v[:, f], axis=0, keepdims=True)
        hu = jnp.sum(hu_v[:, f], axis=0, keepdims=True)
        hb = jnp.broadcast_to(hg * _sigmoid(hg) * hu, (L, L)).T
        hb_v[f, :] = hb
        return digest(hb)

    def ffn_down(j, n, nw=512):
        f, cols = slice(j * L, (j + 1) * L), slice(n * nw, (n + 1) * nw)
        hb = jnp.tile(hb_v[f, :], (1, nw // L))
        part = jnp.sum((wd_v[f, cols].astype(F32) * hb).reshape(L // 8, 8, nw), axis=0)
        part = part if j == 0 else y_v[:, cols] + part
        y_v[:, cols] = part
        return digest(part)

    P = functools.partial
    units, before, after = [], {}, {}
    units += [P(k_unit, c, t) for c in range(nc) for t in range(2)]
    units += [P(k_unit, c, t) for t in range(2, nl) for c in range(nc)]
    units += [P(g_unit, c, n) for c in range(nc) for n in range(D // gw)]
    q_units = lambda i: [P(q_unit, i, c, t) for t in range(tb // tw) for c in range(nc)]
    first_q = q_units(0)
    for j in range(D // L):
        units += [P(kv_unit, j)] + first_q[j * len(first_q) // (D // L):(j + 1) * len(first_q) // (D // L)]
    for i in range(nb):
        if i + 1 < nb:
            units += q_units(i + 1)
        units += [P(out_unit, i, n) for n in range(D // L)]
    cost = {k_unit: rc * tw * D, g_unit: rc * gw * S, kv_unit: 2 * L * L * D,
            q_unit: rc * tw * D, out_unit: tb * L * D}
    clock = [0]
    for unit in units:
        clock.append(clock[-1] + cost[unit.func] / (S * D * D))

    def at(time):
        return max(u for u in range(len(units)) if clock[u] <= time)

    def spread(jobs, t0, t1):
        for n, job in enumerate(jobs):
            after.setdefault(at(t0 + (t1 - t0) * n / len(jobs)), []).append(job)

    assert xc == tw and nc == 4 and nl == 8
    xs = lambda *ids: [cp for i in ids for cp in cp_x(i)]
    wkt = lambda c: [P(transpose_w, wk_v, wkt_v, j) for j in range(c * rc // L, (c + 1) * rc // L)]
    start(*cp_k(0), *xs(0))()
    best_v[...] = jnp.full(best_v.shape, -jnp.inf, F32)
    besti_v[...] = jnp.full(besti_v.shape, BIG, jnp.int32)
    wkt_v[D // 2:, :] = _pack(jnp.concatenate(
        [jnp.broadcast_to(w_r, (8, D)), jnp.broadcast_to(w_g, (8, D))], axis=0).astype(BF16))
    for cp in xs(1) + cp_k(1):
        cp.start(priority=boot)
    before[0] = [wait(*cp_k(0), *xs(0)), start(*cp_k(2), *cp_k(3))] + wkt(0)
    before[1] = [wait(*xs(1), *cp_k(1))]
    after[1] = wkt(1)
    before[3] = [wait(*cp_k(2), *cp_k(3)), start(*xs(2, 3))]
    after[3], after[4] = wkt(2), wkt(3)
    before[6] = [wait(*xs(2, 3)), start(*xs(4, 5, 6, 7))]
    spread([P(repack, i) for i in (4, 5, 6, 7, 0, 1, 2, 3)], clock[6], clock[10])
    before[12] = [wait(*xs(4, 5, 6, 7)), start(*cp_qvo())]
    spread([P(repack, i) for i in range(8, 16)], clock[12], clock[20])
    before.setdefault(at(t_q - lead), []).append(start(*cp_up(0)))
    before.setdefault(at(t_up - lead), []).append(start(*cp_up(1)))
    before.setdefault(at(t_mid - lead), []).append(start(*cp_d()))
    u_sel = at(t_sel)
    after.setdefault(u_sel, []).append(select)
    after.setdefault(u_sel + 1, []).append(gather)
    assert at(t_up) >= u_sel + 2
    before.setdefault(at(t_up), []).append(wait(*cp_up(0)))
    ups = lambda j0, j1: [job for j in range(j0, j1)
                          for job in [P(ffn_up, j, k) for k in range(D // 256)] + [P(ffn_act, j)]]
    spread(ups(0, fh // L), t_up, t_mid)
    before.setdefault(at(t_mid), []).append(wait(*cp_up(1)))
    spread(ups(fh // L, F // L), t_mid, t_down)
    before.setdefault(at(t_q), []).append(wait(*cp_qvo()))
    spread([P(transpose_w, wq_v, wqt_v, j) for j in range(D // L)], t_q, t_up)
    before.setdefault(at(t_down), []).append(wait(*cp_d()))
    spread([P(ffn_down, j, n) for j in range(F // L) for n in range(D // 512)],
           t_down, clock[len(units) - D // L - 2])

    posts = []
    for u, unit in enumerate(units):
        for job in before.get(u, []):
            job()
        posts.append(unit())
        if len(posts) > skew:
            posts.pop(0)()
        for job in after.get(u, []):
            token = job()
            if token is not None:
                tokens.append(token)
    for post in posts:
        post()
    for i in range(nb - 1):
        cp_o(i, 0).wait()
    for n in range(D // L):
        cp_o(nb - 1, 0, n).wait()


def _build(rc=256, tw=256, tb=256, xc=256, skew=1, t_sel=1.05, t_mid=2.3, t_down=3.0, t_up=1.65, t_q=1.0, boot=0, ns=4, gw=128, lead=0.05, flags=None):
    def run(A_x, A_wqkv, A_wo, B_x, B_w_r, B_w_gate, B_w_up, B_w_down, gate_w):
        B, S, D = A_x.shape
        F = B_w_gate.shape[1]
        hbm = pl.BlockSpec(memory_space=pl.ANY)
        vec = pl.BlockSpec(memory_space=pltpu.VMEM)
        vmem, dma = pltpu.VMEM, pltpu.SemaphoreType.DMA
        out = pl.pallas_call(
            functools.partial(_kernel, rc=rc, tw=tw, tb=tb, xc=xc, skew=skew,
                              t_sel=t_sel, t_mid=t_mid, t_down=t_down, t_up=t_up, t_q=t_q, boot=boot, ns=ns, gw=gw, lead=lead),
            out_shape=jax.ShapeDtypeStruct((S, D), BF16),
            in_specs=[hbm, hbm, hbm, vec, hbm, hbm, hbm, vec],
            out_specs=hbm,
            scratch_shapes=[
                vmem((S, D), BF16),
                vmem((D, D), BF16), vmem((D, D), BF16),
                vmem((D, D), BF16), vmem((D, D), BF16),
                vmem((D, F), BF16), vmem((D, F), BF16), vmem((F, D), BF16),
                vmem((S // 2, D), U32),
                vmem((D // 2, D), U32), vmem((D // 2 + 8, D), U32),
                vmem((D // 2, S), U32),
                vmem((D // 2, D), U32), vmem((D // 2, D), U32),
                vmem((tb, D), U32),
                vmem((D, 128), F32), vmem((S, 128), F32),
                vmem((8, 128), F32), vmem((8, 128), jnp.int32),
                vmem((D, 128), F32),
                vmem((8, F), F32), vmem((8, F), F32), vmem((F, 128), F32),
                vmem((8, D), F32),
                vmem((S, D), BF16),
                dma((S // xc,)), dma((4,)), dma((D // rc,)), dma((S // tb + D // 128 - 1,)),
            ],
            compiler_params=pltpu.CompilerParams(
                vmem_limit_bytes=110 * 1024 * 1024, flags=flags),
        )(A_x.reshape(S, D), A_wqkv, A_wo, B_w_r.reshape(D // 128, 128),
          B_w_gate, B_w_up, B_w_down, gate_w.reshape(D // 128, 128))
        return out.reshape(B, S, D)
    return run


@jax.jit
def pallas_gated_mix__linear_attn_block__moe_arch_mod__prompt_kernel(
    A_x: jax.Array,
    A_wqkv: jax.Array,
    A_wo: jax.Array,
    B_x: jax.Array,
    B_w_r: jax.Array,
    B_w_gate: jax.Array,
    B_w_up: jax.Array,
    B_w_down: jax.Array,
    gate_w: jax.Array,
):
    return _build()(A_x, A_wqkv, A_wo, B_x, B_w_r, B_w_gate, B_w_up, B_w_down, gate_w)
```

```python
import functools

import jax
import jax.numpy as jnp
from jax import lax
import jax.experimental.pallas as pl
import jax.experimental.pallas.tpu as pltpu

F32 = jnp.float32
BF16 = jnp.bfloat16
U32 = jnp.uint32
HEADS = 32
BIG = 1 << 30
NT = (((1,), (1,)), ((), ()))
TN = (((0,), (0,)), ((), ()))


def _phi(t):
    return jnp.where(t > 0, t + 1.0, jnp.exp(t)) + 1e-6


def _sigmoid(t):
    return 1.0 / (1.0 + jnp.exp(-t))


def _pack(v):
    return pltpu.bitcast(v, jnp.uint32)


def _unpack(v):
    return pltpu.bitcast(v, BF16)


def _kernel(x_hbm, wqkv_hbm, wo_hbm, wr_hbm, wg_hbm, wu_hbm, wd_hbm, gw_hbm,
            out_hbm,
            x_v, vec_v, wq_v, wk_v, wv_v, wo_v, wg_v, wu_v, wd_v,
            xp_v, xq_v, wqt_v, wkt_v, pk_v, g_v, m_v, on_v, z_v, gate_v, best_v, besti_v,
            xb_v, hg_v, hu_v, hb_v, y_v, o_v,
            sem_s, sem_x, sem_w, sem_k, sem_o, *, t_up, t_q, rq, ns, lead, rc, tw, tb, xc, skew, t_sel, t_mid, t_down):
    S, D = x_v.shape
    F = wg_v.shape[1]
    L = 128
    nc = D // rc
    nl = S // tw
    nb = S // tb
    dh = D // HEADS
    fh = F // 2

    def copies(src, dst, sem, rows, cols, shift, n):
        (r0, nr), (c0, ncol) = rows, cols
        return [pltpu.make_async_copy(src.at[pl.ds(r0 + k * nr // n, nr // n), pl.ds(c0 + shift, ncol)],
                                      dst.at[pl.ds(r0 + k * nr // n, nr // n), pl.ds(c0, ncol)], sem)
                for k in range(n)]

    cp_x = lambda i: copies(x_hbm, x_v, sem_x.at[i], (i * xc, xc), (0, D), 0, ns if i == 0 else 1)
    cp_k = lambda c: copies(wqkv_hbm, wk_v, sem_k.at[c], (0, D), (c * rc, rc), D, ns if c == 0 else 1)
    cp_qvo = lambda: (copies(wqkv_hbm, wq_v, sem_w.at[0], (0, D), (0, D), 0, 2)
                      + copies(wqkv_hbm, wv_v, sem_w.at[0], (0, D), (0, D), 2 * D, 2)
                      + copies(wo_hbm, wo_v, sem_w.at[0], (0, D), (0, D), 0, 2))
    cp_up = lambda j: (copies(wg_hbm, wg_v, sem_w.at[1 + j], (0, D), (j * fh, fh), 0, 2)
                       + copies(wu_hbm, wu_v, sem_w.at[1 + j], (0, D), (j * fh, fh), 0, 2))
    cp_d = lambda: copies(wd_hbm, wd_v, sem_w.at[3], (0, F), (0, D), 0, 4)

    def cp_o(i, t, n=None):
        cols = pl.ds(0, D) if n is None else pl.ds(n * L, L)
        return pltpu.make_async_copy(o_v.at[pl.ds(i * tb, tb), cols],
                                     out_hbm.at[pl.ds(pl.multiple_of(t * tb, tb), tb), cols],
                                     sem_o.at[i + (n or 0)])

    def start(*cps):
        return lambda: [cp.start() for cp in cps] and None

    def wait(*cps):
        return lambda: [cp.wait() for cp in cps] and None

    def packed(ref, lo, n):
        if isinstance(lo, int):
            return _unpack(ref[lo // 2:(lo + n) // 2, :])
        return _unpack(ref[pl.ds(pl.multiple_of(lo // 2, n // 2), n // 2), :])

    tokens = []
    start(*cp_k(0), *cp_x(0))()
    small = [pltpu.make_async_copy(src, vec_v.at[j], sem_s.at[j]) for j, src in enumerate((wr_hbm, gw_hbm))]
    start(*small, *cp_x(1), *cp_k(1))()
    wait(*small)()
    w_r, w_g = vec_v[0].astype(F32), vec_v[1].astype(F32)
    never = (pltpu.bitcast(w_g, jnp.int32) & 0xFFFF) != 0
    w_g, w_r = (jnp.concatenate([w[j:j + 1, :] for j in range(D // L)], axis=1) for w in (w_g, w_r))

    def digest(*vals):
        acc = None
        for v in vals:
            v = v if v.dtype == jnp.int32 else pltpu.bitcast(v, jnp.int32)
            for i in range(v.shape[0] // 8):
                for j in range(v.shape[1] // L):
                    e = v[i * 8:(i + 1) * 8, j * L:(j + 1) * L]
                    acc = e if acc is None else acc ^ e
        return acc

    def tie(v):
        if not tokens:
            return v
        head = jnp.where(never, pltpu.bitcast(digest(*tokens), v.dtype), v[0:8, 0:L])
        tokens.clear()
        if v.shape[1] > L:
            head = jnp.concatenate([head, v[0:8, L:]], axis=1)
        return jnp.concatenate([head, v[8:]], axis=0)

    def k_unit(c, t):
        r = slice(c * rc, (c + 1) * rc)
        if t < 2:
            xt = x_v[t * tw:(t + 1) * tw, :]
        else:
            xt = jnp.concatenate([packed(xp_v.at[n], t * tw, tw) for n in range(D // L)], axis=1)
        more = 8 if c == nc - 1 else 0
        w = _unpack(tie(wkt_v[c * rc // 2:(c + 1) * rc // 2 + more, :]))
        kt = lax.dot_general(w, xt, NT, preferred_element_type=F32)

        def post():
            if more:
                route(t * tw, kt[rc:rc + 8], kt[rc + 8:])
            tokens.append(besti_v[...])
            pk = _phi(tie(kt[:rc]))
            zs = pk[:, 0:L]
            for j in range(1, tw // L):
                zs = zs + pk[:, j * L:(j + 1) * L]
            if t > 0:
                zs = zs + z_v[r, :]
            if t == nl - 1:
                zs = jnp.broadcast_to(jnp.sum(zs, axis=-1, keepdims=True), zs.shape)
            z_v[r, :] = zs
            pk_v[c * rc // 2:(c + 1) * rc // 2, t * tw:(t + 1) * tw] = _pack(pk.astype(BF16))
        return post

    def g_unit(c, n):
        cols = slice(n * L, (n + 1) * L)
        g = jnp.dot(packed(pk_v, c * rc, rc), packed(xp_v.at[n], 0, S), preferred_element_type=F32)

        def post():
            g_v[c * rc // 2:(c + 1) * rc // 2, cols] = _pack(tie(g).astype(BF16))
        return post

    def kv_unit(j):
        q = slice(j * L, (j + 1) * L)
        kv = jnp.dot(packed(g_v, j * L, L), wv_v[:, q], preferred_element_type=F32)

        def post():
            same_head = (lax.broadcasted_iota(jnp.int32, (L, L), 0) // dh
                         == lax.broadcasted_iota(jnp.int32, (L, L), 1) // dh)
            kvm = jnp.where(same_head, kv, 0.0).astype(BF16)
            m = jnp.dot(kvm, wo_v[q, :], preferred_element_type=F32)
            m_v[j * L // 2:(j + 1) * L // 2, :] = _pack(m.astype(BF16))
        return post

    sel = {}

    def block_of(i):
        return lax.rem(sel["blk"] + 1 + i, nb)

    def q_unit(i, c):
        r = slice(c * rq, (c + 1) * rq)
        q = lax.dot_general(packed(wqt_v, c * rq, rq), packed(xq_v, block_of(i) * tb, tb), NT,
                            preferred_element_type=F32)

        def post():
            pq = _phi(tie(q))
            z = jnp.tile(z_v[r, :], (1, tb // L))
            den = jnp.sum((pq * z).reshape(rq // dh, dh, tb), axis=1, keepdims=True) + 1e-6
            o = (pq.reshape(rq // dh, dh, tb) * (1.0 / den)).reshape(rq, tb)
            pairs = pltpu.pack_elementwise([o[:, :L], o[:, L:]], packed_dtype=BF16)
            on_v[(i % 2) * L:(i % 2 + 1) * L, r] = pltpu.bitcast(pairs, U32).T
        return post

    def out_unit(i, n):
        cols = slice(n * L, (n + 1) * L)
        a = jnp.dot(packed(on_v, (i % 2) * tb, tb), _unpack(m_v[:, cols]), preferred_element_type=F32)

        def post():
            lo = block_of(i) * tb
            gate = gate_v[pl.ds(pl.multiple_of(lo, tb), tb), :]
            bx = packed(xp_v.at[n], lo, tb).astype(F32)
            upd = bx * 0.0
            if i == nb - 1:
                y = jnp.sum(y_v[:, cols], axis=0, keepdims=True) * sel["w"]
                is_sel = lax.broadcasted_iota(jnp.int32, (tb, L), 0) + lo == sel["idx"]
                upd = upd + jnp.where(is_sel, y, 0.0)
            o_v[i * tb:(i + 1) * tb, cols] = (gate * tie(a) + (1.0 - gate) * (bx + upd)).astype(BF16)
            if i == nb - 1:
                cp_o(i, block_of(i), n).start()
            elif n == D // L - 1:
                cp_o(i, block_of(i)).start()
        return post

    def repack(i):
        xp = _pack(x_v[i * L:(i + 1) * L, :])
        for n in range(D // L):
            xp_v[n, i * L // 2:(i + 1) * L // 2, :] = xp[:, n * L:(n + 1) * L]
        return digest(xp)

    def split_parity(t):
        lo, n = t * tw // 2, tw // 4
        a, b = (jnp.concatenate([xp_v[k, pl.ds(lo + first, n, stride=2), :] for k in range(D // L)], axis=1)
                for first in (0, 1))
        even = (a & jnp.uint32(0xFFFF)) | (b << 16)
        odd = (a >> 16) | (b & jnp.uint32(0xFFFF0000))
        xq_v[lo:lo + n, :] = even
        xq_v[lo + n:lo + 2 * n, :] = odd
        return digest(even ^ odd)

    def transpose_w(src, dst, j):
        wt = _pack(src[:, j * L:(j + 1) * L].T)
        dst[j * L // 2:(j + 1) * L // 2, :] = wt
        return digest(wt)

    def route(lo, score, logit):
        score = score.astype(BF16).astype(F32)
        gate = _sigmoid(logit)
        best, besti = best_v[...], besti_v[...]
        for k in range(tw // L):
            s8 = score[:, k * L:(k + 1) * L]
            take = (s8 > best) | ((s8 == best) & (besti == BIG))
            best = jnp.where(take, s8, best)
            besti = jnp.where(take, lax.broadcasted_iota(jnp.int32, (8, L), 1) + (lo + k * L), besti)
            gate_v[lo + k * L:lo + (k + 1) * L, :] = jnp.tile(gate[:, k * L:(k + 1) * L], (L // 8, 1)).T
        best_v[...] = best
        besti_v[...] = besti

    def select():
        best, besti = best_v[...], besti_v[...]
        m = jnp.max(best[0:1], axis=1, keepdims=True)
        mi = jnp.min(jnp.where(best[0:1] == m, besti[0:1], BIG), axis=1, keepdims=True)
        none = mi == BIG
        sel["w"] = _sigmoid(jnp.where(none, jnp.nan, m))
        sel["idx"] = jnp.where(none, 0, mi)[0, 0]
        sel["blk"] = sel["idx"] // tb

    def gather():
        base = pl.multiple_of((sel["idx"] // 16) * 16, 16)
        slab = x_v[pl.ds(base, 16), :].astype(F32)
        pick = lax.broadcasted_iota(jnp.int32, (16, 1), 0) == sel["idx"] - base
        xs = jnp.sum(jnp.where(pick, slab, 0.0), axis=0, keepdims=True)
        xb_v[...] = jnp.broadcast_to(xs, (L, D)).T

    def ffn_up(j, k, kr=256):
        f, r = slice(j * L, (j + 1) * L), slice(k * kr, (k + 1) * kr)
        xb = xb_v[r, :]
        parts = []
        for w_v, h_v in ((wg_v, hg_v), (wu_v, hu_v)):
            part = jnp.sum((w_v[r, f].astype(F32) * xb).reshape(kr // 8, 8, L), axis=0)
            parts.append(part if k == 0 else h_v[:, f] + part)
            h_v[:, f] = parts[-1]
        return digest(*parts)

    def ffn_act(j):
        f = slice(j * L, (j + 1) * L)
        hg = jnp.sum(hg_v[:, f], axis=0, keepdims=True)
        hu = jnp.sum(hu_v[:, f], axis=0, keepdims=True)
        hb = jnp.broadcast_to(hg * _sigmoid(hg) * hu, (L, L)).T
        hb_v[f, :] = hb
        return digest(hb)

    def ffn_down(j, n, nw=512):
        f, cols = slice(j * L, (j + 1) * L), slice(n * nw, (n + 1) * nw)
        hb = jnp.tile(hb_v[f, :], (1, nw // L))
        part = jnp.sum((wd_v[f, cols].astype(F32) * hb).reshape(L // 8, 8, nw), axis=0)
        part = part if j == 0 else y_v[:, cols] + part
        y_v[:, cols] = part
        return digest(part)

    P = functools.partial
    units, before, after = [], {}, {}
    units += [P(k_unit, c, t) for c in range(nc) for t in range(2)]
    units += [P(k_unit, c, t) for t in range(2, nl) for c in range(nc)]
    units += [P(g_unit, c, n) for c in range(nc) for n in range(D // L)]
    q_units = lambda i: [P(q_unit, i, c) for c in range(D // rq)]
    first_q = q_units(0)
    for j in range(D // L):
        units += [P(kv_unit, j)] + first_q[j * len(first_q) // (D // L):(j + 1) * len(first_q) // (D // L)]
    for i in range(nb):
        if i + 1 < nb:
            units += q_units(i + 1)
        units += [P(out_unit, i, n) for n in range(D // L)]
    cost = {k_unit: rc * tw * D, g_unit: rc * L * S, kv_unit: 2 * L * L * D,
            q_unit: rq * tb * D, out_unit: tb * L * D}
    clock = [0]
    for unit in units:
        clock.append(clock[-1] + cost[unit.func] / (S * D * D))

    def at(time):
        return max(u for u in range(len(units)) if clock[u] <= time)

    def spread(jobs, t0, t1):
        for n, job in enumerate(jobs):
            after.setdefault(at(t0 + (t1 - t0) * n / len(jobs)), []).append(job)

    assert xc == tw == tb == 2 * L and nc == 4 and nl == 8
    xs = lambda *ids: [cp for i in ids for cp in cp_x(i)]
    wkt = lambda c: [P(transpose_w, wk_v, wkt_v, j) for j in range(c * rc // L, (c + 1) * rc // L)]
    best_v[...] = jnp.full(best_v.shape, -jnp.inf, F32)
    besti_v[...] = jnp.full(besti_v.shape, BIG, jnp.int32)
    wkt_v[D // 2:, :] = _pack(jnp.concatenate(
        [jnp.broadcast_to(w_r, (8, D)), jnp.broadcast_to(w_g, (8, D))], axis=0).astype(BF16))
    before[0] = [wait(*cp_k(0), *xs(0)), start(*cp_k(2), *cp_k(3))] + wkt(0)
    before[1] = [wait(*xs(1), *cp_k(1))]
    after[1] = wkt(1)
    before[3] = [wait(*cp_k(2), *cp_k(3)), start(*xs(2, 3))]
    after[3], after[4] = wkt(2), wkt(3)
    before[6] = [wait(*xs(2, 3)), start(*xs(4, 5, 6, 7))]
    spread([P(repack, i) for i in (4, 5, 6, 7, 0, 1, 2, 3)], clock[6], clock[10])
    before[12] = [wait(*xs(4, 5, 6, 7)), start(*cp_qvo())]
    spread([P(repack, i) for i in range(8, 16)], clock[12], clock[20])
    spread([P(split_parity, t) for t in range(nl)], 0.7, t_q)
    before.setdefault(at(t_q - lead), []).append(start(*cp_up(0)))
    before.setdefault(at(t_up - lead), []).append(start(*cp_up(1)))
    before.setdefault(at(t_mid - lead), []).append(start(*cp_d()))
    u_sel = at(t_sel)
    after.setdefault(u_sel, []).append(select)
    after.setdefault(u_sel + 1, []).append(gather)
    assert at(t_up) >= u_sel + 2
    before.setdefault(at(t_up), []).append(wait(*cp_up(0)))
    ups = lambda j0, j1: [job for j in range(j0, j1)
                          for job in [P(ffn_up, j, k) for k in range(D // 256)] + [P(ffn_act, j)]]
    spread(ups(0, fh // L), t_up, t_mid)
    before.setdefault(at(t_mid), []).append(wait(*cp_up(1)))
    spread(ups(fh // L, F // L), t_mid, t_down)
    before.setdefault(at(t_q), []).append(wait(*cp_qvo()))
    spread([P(transpose_w, wq_v, wqt_v, j) for j in range(D // L)], t_q, t_up)
    before.setdefault(at(t_down), []).append(wait(*cp_d()))
    spread([P(ffn_down, j, n) for j in range(F // L) for n in range(D // 512)],
           t_down, clock[len(units) - D // L - 2])

    posts = []
    for u, unit in enumerate(units):
        for job in before.get(u, []):
            job()
        posts.append(unit())
        if len(posts) > skew:
            posts.pop(0)()
        for job in after.get(u, []):
            token = job()
            if token is not None:
                tokens.append(token)
    for post in posts:
        post()
    for i in range(nb - 1):
        cp_o(i, 0).wait()
    for n in range(D // L):
        cp_o(nb - 1, 0, n).wait()


def _build(rc=256, tw=256, tb=256, xc=256, skew=1, t_sel=1.05, t_mid=2.3, t_down=3.0, t_up=1.65, t_q=1.0, rq=128, ns=4, lead=0.05, flags=None):
    def run(A_x, A_wqkv, A_wo, B_x, B_w_r, B_w_gate, B_w_up, B_w_down, gate_w):
        B, S, D = A_x.shape
        F = B_w_gate.shape[1]
        hbm = pl.BlockSpec(memory_space=pl.ANY)
        vmem, dma = pltpu.VMEM, pltpu.SemaphoreType.DMA
        out = pl.pallas_call(
            functools.partial(_kernel, rc=rc, tw=tw, tb=tb, xc=xc, skew=skew,
                              t_sel=t_sel, t_mid=t_mid, t_down=t_down, t_up=t_up, t_q=t_q, rq=rq, ns=ns, lead=lead),
            out_shape=jax.ShapeDtypeStruct((S, D), BF16),
            in_specs=[hbm] * 8,
            out_specs=hbm,
            scratch_shapes=[
                vmem((S, D), BF16),
                vmem((2, D // 128, 128), BF16),
                vmem((D, D), BF16), vmem((D, D), BF16),
                vmem((D, D), BF16), vmem((D, D), BF16),
                vmem((D, F), BF16), vmem((D, F), BF16), vmem((F, D), BF16),
                vmem((D // 128, S // 2, 128), U32), vmem((S // 2, D), U32),
                vmem((D // 2, D), U32), vmem((D // 2 + 8, D), U32),
                vmem((D // 2, S), U32),
                vmem((D // 2, D), U32), vmem((D // 2, D), U32),
                vmem((tb, D), U32),
                vmem((D, 128), F32), vmem((S, 128), F32),
                vmem((8, 128), F32), vmem((8, 128), jnp.int32),
                vmem((D, 128), F32),
                vmem((8, F), F32), vmem((8, F), F32), vmem((F, 128), F32),
                vmem((8, D), F32),
                vmem((S, D), BF16),
                dma((2,)), dma((S // xc,)), dma((4,)), dma((D // rc,)), dma((S // tb + D // 128 - 1,)),
            ],
            compiler_params=pltpu.CompilerParams(
                vmem_limit_bytes=110 * 1024 * 1024, flags=flags),
        )(A_x.reshape(S, D), A_wqkv, A_wo, B_w_r.reshape(D // 128, 128),
          B_w_gate, B_w_up, B_w_down, gate_w.reshape(D // 128, 128))
        return out.reshape(B, S, D)
    return run


@jax.jit
def pallas_gated_mix__linear_attn_block__moe_arch_mod__prompt_kernel(
    A_x: jax.Array,
    A_wqkv: jax.Array,
    A_wo: jax.Array,
    B_x: jax.Array,
    B_w_r: jax.Array,
    B_w_gate: jax.Array,
    B_w_up: jax.Array,
    B_w_down: jax.Array,
    gate_w: jax.Array,
):
    return _build()(A_x, A_wqkv, A_wo, B_x, B_w_r, B_w_gate, B_w_up, B_w_down, gate_w)
```

```python
import functools

import jax
import jax.numpy as jnp
from jax import lax
import jax.experimental.pallas as pl
import jax.experimental.pallas.tpu as pltpu

F32 = jnp.float32
BF16 = jnp.bfloat16
U32 = jnp.uint32
HEADS = 32
BIG = 1 << 30
FLAGS = {"XLA_TPU_EVENLY_DISTRIBUTE_CRITICAL_NODES": True}
NT = (((1,), (1,)), ((), ()))
TN = (((0,), (0,)), ((), ()))


def _phi(t):
    return jnp.where(t > 0, t + 1.0, jnp.exp(t)) + 1e-6


def _sigmoid(t):
    return 1.0 / (1.0 + jnp.exp(-t))


def _pack(v):
    return pltpu.bitcast(v, jnp.uint32)


def _unpack(v):
    return pltpu.bitcast(v, BF16)


def _kernel(x_hbm, wqkv_hbm, wo_hbm, wr_hbm, wg_hbm, wu_hbm, wd_hbm, gw_hbm,
            out_hbm,
            x_v, vec_v, wq_v, wk_v, wv_v, wo_v, wg_v, wu_v, wd_v,
            xp_v, xq_v, wqt_v, wkt_v, pk_v, g_v, m_v, on_v, z_v, gate_v, best_v, besti_v,
            xb_v, hg_v, hu_v, hb_v, y_v, o_v,
            sem_s, sem_x, sem_w, sem_k, sem_o, *, t_up, t_q, rq, ns, lead, rc, tw, tb, xc, skew, t_sel, t_mid, t_down):
    S, D = x_v.shape
    F = wg_v.shape[1]
    L = 128
    nc = D // rc
    nl = S // tw
    nb = S // tb
    dh = D // HEADS
    fh = F // 2

    def copies(src, dst, sem, rows, cols, shift, n):
        (r0, nr), (c0, ncol) = rows, cols
        return [pltpu.make_async_copy(src.at[pl.ds(r0 + k * nr // n, nr // n), pl.ds(c0 + shift, ncol)],
                                      dst.at[pl.ds(r0 + k * nr // n, nr // n), pl.ds(c0, ncol)], sem)
                for k in range(n)]

    cp_x = lambda i: copies(x_hbm, x_v, sem_x.at[i], (i * xc, xc), (0, D), 0, ns if i == 0 else 1)
    cp_k = lambda c: copies(wqkv_hbm, wk_v, sem_k.at[c], (0, D), (c * rc, rc), D, ns if c == 0 else 1)
    cp_qvo = lambda: (copies(wqkv_hbm, wq_v, sem_w.at[0], (0, D), (0, D), 0, 2)
                      + copies(wqkv_hbm, wv_v, sem_w.at[0], (0, D), (0, D), 2 * D, 2)
                      + copies(wo_hbm, wo_v, sem_w.at[0], (0, D), (0, D), 0, 2))
    cp_up = lambda j: (copies(wg_hbm, wg_v, sem_w.at[1 + j], (0, D), (j * fh, fh), 0, 2)
                       + copies(wu_hbm, wu_v, sem_w.at[1 + j], (0, D), (j * fh, fh), 0, 2))
    cp_d = lambda: copies(wd_hbm, wd_v, sem_w.at[3], (0, F), (0, D), 0, 4)

    def cp_o(i, t, n=None):
        cols = pl.ds(0, D) if n is None else pl.ds(n * L, L)
        return pltpu.make_async_copy(o_v.at[pl.ds(i * tb, tb), cols],
                                     out_hbm.at[pl.ds(pl.multiple_of(t * tb, tb), tb), cols],
                                     sem_o.at[i + (n or 0)])

    def start(*cps):
        return lambda: [cp.start() for cp in cps] and None

    def wait(*cps):
        return lambda: [cp.wait() for cp in cps] and None

    def packed(ref, lo, n):
        if isinstance(lo, int):
            return _unpack(ref[lo // 2:(lo + n) // 2, :])
        return _unpack(ref[pl.ds(pl.multiple_of(lo // 2, n // 2), n // 2), :])

    tokens = []
    start(*cp_k(0), *cp_x(0))()
    small = [pltpu.make_async_copy(src, vec_v.at[j], sem_s.at[j]) for j, src in enumerate((wr_hbm, gw_hbm))]
    start(*small, *cp_x(1), *cp_k(1))()
    wait(*small)()
    w_r, w_g = vec_v[0].astype(F32), vec_v[1].astype(F32)
    never = (pltpu.bitcast(w_g, jnp.int32) & 0xFFFF) != 0
    w_g, w_r = (jnp.concatenate([w[j:j + 1, :] for j in range(D // L)], axis=1) for w in (w_g, w_r))

    def digest(*vals):
        acc = None
        for v in vals:
            v = v if v.dtype == jnp.int32 else pltpu.bitcast(v, jnp.int32)
            for i in range(v.shape[0] // 8):
                for j in range(v.shape[1] // L):
                    e = v[i * 8:(i + 1) * 8, j * L:(j + 1) * L]
                    acc = e if acc is None else acc ^ e
        return acc

    def tie(v):
        if not tokens:
            return v
        head = jnp.where(never, pltpu.bitcast(digest(*tokens), v.dtype), v[0:8, 0:L])
        tokens.clear()
        if v.shape[1] > L:
            head = jnp.concatenate([head, v[0:8, L:]], axis=1)
        return jnp.concatenate([head, v[8:]], axis=0)

    def k_unit(c, t):
        r = slice(c * rc, (c + 1) * rc)
        if t < 3:
            xt = x_v[t * tw:(t + 1) * tw, :]
        else:
            xt = jnp.concatenate([packed(xp_v.at[n], t * tw, tw) for n in range(D // L)], axis=1)
        more = 8 if c == nc - 1 else 0
        w = _unpack(tie(wkt_v[c * rc // 2:(c + 1) * rc // 2 + more, :]))
        kt = lax.dot_general(w, xt, NT, preferred_element_type=F32)

        def post():
            if more:
                route(t * tw, kt[rc:rc + 8], kt[rc + 8:])
            tokens.append(besti_v[...])
            pk = _phi(tie(kt[:rc]))
            zs = pk[:, 0:L]
            for j in range(1, tw // L):
                zs = zs + pk[:, j * L:(j + 1) * L]
            if t > 0:
                zs = zs + z_v[r, :]
            if t == nl - 1:
                zs = jnp.broadcast_to(jnp.sum(zs, axis=-1, keepdims=True), zs.shape)
            z_v[r, :] = zs
            pk_v[c * rc // 2:(c + 1) * rc // 2, t * tw:(t + 1) * tw] = _pack(pk.astype(BF16))
        return post

    def g_unit(c, n):
        cols = slice(n * L, (n + 1) * L)
        g = jnp.dot(packed(pk_v, c * rc, rc), packed(xp_v.at[n], 0, S), preferred_element_type=F32)

        def post():
            g_v[c * rc // 2:(c + 1) * rc // 2, cols] = _pack(tie(g).astype(BF16))
        return post

    def kv_unit(j):
        q = slice(j * L, (j + 1) * L)
        kv = jnp.dot(packed(g_v, j * L, L), wv_v[:, q], preferred_element_type=F32)

        def post():
            same_head = (lax.broadcasted_iota(jnp.int32, (L, L), 0) // dh
                         == lax.broadcasted_iota(jnp.int32, (L, L), 1) // dh)
            kvs[j] = jnp.where(same_head, kv, 0.0).astype(BF16)
        return post

    def m_unit(j):
        m = jnp.dot(kvs.pop(j), wo_v[j * L:(j + 1) * L, :], preferred_element_type=F32)

        def post():
            m_v[j * L // 2:(j + 1) * L // 2, :] = _pack(m.astype(BF16))
        return post

    kvs, sel = {}, {}

    def block_of(i):
        return lax.rem(sel["blk"] + 1 + i, nb)

    def q_unit(i, c):
        r = slice(c * rq, (c + 1) * rq)
        q = lax.dot_general(packed(wqt_v, c * rq, rq), packed(xq_v, block_of(i) * tb, tb), NT,
                            preferred_element_type=F32)

        def post():
            pq = _phi(tie(q))
            z = jnp.tile(z_v[r, :], (1, tb // L))
            den = jnp.sum((pq * z).reshape(rq // dh, dh, tb), axis=1, keepdims=True) + 1e-6
            o = (pq.reshape(rq // dh, dh, tb) * (1.0 / den)).reshape(rq, tb)
            pairs = pltpu.pack_elementwise([o[:, :L], o[:, L:]], packed_dtype=BF16)
            on_v[(i % 2) * L:(i % 2 + 1) * L, r] = pltpu.bitcast(pairs, U32).T
        return post

    def out_unit(i, n):
        cols = slice(n * L, (n + 1) * L)
        a = jnp.dot(packed(on_v, (i % 2) * tb, tb), _unpack(m_v[:, cols]), preferred_element_type=F32)

        def post():
            lo = block_of(i) * tb
            gate = gate_v[pl.ds(pl.multiple_of(lo, tb), tb), :]
            bx = packed(xp_v.at[n], lo, tb).astype(F32)
            upd = bx * 0.0
            if i == nb - 1:
                y = jnp.sum(y_v[:, cols], axis=0, keepdims=True) * sel["w"]
                is_sel = lax.broadcasted_iota(jnp.int32, (tb, L), 0) + lo == sel["idx"]
                upd = upd + jnp.where(is_sel, y, 0.0)
            o_v[i * tb:(i + 1) * tb, cols] = (gate * tie(a) + (1.0 - gate) * (bx + upd)).astype(BF16)
            if i == nb - 1:
                cp_o(i, block_of(i), n).start()
            elif n == D // L - 1:
                cp_o(i, block_of(i)).start()
        return post

    def repack(i):
        xp = _pack(x_v[i * L:(i + 1) * L, :])
        for n in range(D // L):
            xp_v[n, i * L // 2:(i + 1) * L // 2, :] = xp[:, n * L:(n + 1) * L]
        return digest(xp)

    def split_parity(t):
        lo, n = t * tw // 2, tw // 4
        a, b = (jnp.concatenate([xp_v[k, pl.ds(lo + first, n, stride=2), :] for k in range(D // L)], axis=1)
                for first in (0, 1))
        even = (a & jnp.uint32(0xFFFF)) | (b << 16)
        odd = (a >> 16) | (b & jnp.uint32(0xFFFF0000))
        xq_v[lo:lo + n, :] = even
        xq_v[lo + n:lo + 2 * n, :] = odd
        return digest(even ^ odd)

    def transpose_w(src, dst, j):
        wt = _pack(src[:, j * L:(j + 1) * L].T)
        dst[j * L // 2:(j + 1) * L // 2, :] = wt
        return digest(wt)

    def route(lo, score, logit):
        score = score.astype(BF16).astype(F32)
        gate = _sigmoid(logit)
        best, besti = best_v[...], besti_v[...]
        for k in range(tw // L):
            s8 = score[:, k * L:(k + 1) * L]
            take = (s8 > best) | ((s8 == best) & (besti == BIG))
            best = jnp.where(take, s8, best)
            besti = jnp.where(take, lax.broadcasted_iota(jnp.int32, (8, L), 1) + (lo + k * L), besti)
            gate_v[lo + k * L:lo + (k + 1) * L, :] = jnp.tile(gate[:, k * L:(k + 1) * L], (L // 8, 1)).T
        best_v[...] = best
        besti_v[...] = besti

    def select():
        best, besti = best_v[...], besti_v[...]
        m = jnp.max(best[0:1], axis=1, keepdims=True)
        mi = jnp.min(jnp.where(best[0:1] == m, besti[0:1], BIG), axis=1, keepdims=True)
        none = mi == BIG
        sel["w"] = _sigmoid(jnp.where(none, jnp.nan, m))
        sel["idx"] = jnp.where(none, 0, mi)[0, 0]
        sel["blk"] = sel["idx"] // tb

    def gather():
        base = pl.multiple_of((sel["idx"] // 16) * 16, 16)
        slab = x_v[pl.ds(base, 16), :].astype(F32)
        pick = lax.broadcasted_iota(jnp.int32, (16, 1), 0) == sel["idx"] - base
        xs = jnp.sum(jnp.where(pick, slab, 0.0), axis=0, keepdims=True)
        xb_v[...] = jnp.broadcast_to(xs, (L, D)).T

    def ffn_up(j, k, kr=256):
        f, r = slice(j * L, (j + 1) * L), slice(k * kr, (k + 1) * kr)
        xb = xb_v[r, :]
        parts = []
        for w_v, h_v in ((wg_v, hg_v), (wu_v, hu_v)):
            part = jnp.sum((w_v[r, f].astype(F32) * xb).reshape(kr // 8, 8, L), axis=0)
            parts.append(part if k == 0 else h_v[:, f] + part)
            h_v[:, f] = parts[-1]
        return digest(*parts)

    def ffn_act(j):
        f = slice(j * L, (j + 1) * L)
        hg = jnp.sum(hg_v[:, f], axis=0, keepdims=True)
        hu = jnp.sum(hu_v[:, f], axis=0, keepdims=True)
        hb = jnp.broadcast_to(hg * _sigmoid(hg) * hu, (L, L)).T
        hb_v[f, :] = hb
        return digest(hb)

    def ffn_down(j, n, nw=512):
        f, cols = slice(j * L, (j + 1) * L), slice(n * nw, (n + 1) * nw)
        hb = jnp.tile(hb_v[f, :], (1, nw // L))
        part = jnp.sum((wd_v[f, cols].astype(F32) * hb).reshape(L // 8, 8, nw), axis=0)
        part = part if j == 0 else y_v[:, cols] + part
        y_v[:, cols] = part
        return digest(part)

    P = functools.partial
    units, before, after = [], {}, {}
    units += [P(k_unit, c, t) for c in range(nc) for t in range(2)]
    units += [P(k_unit, c, t) for t in range(2, nl) for c in range(nc)]
    units += [P(g_unit, c, n) for c in range(nc) for n in range(D // L)]
    q_units = lambda i: [P(q_unit, i, c) for c in range(D // rq)]
    small_units = [P(kv_unit, j) for j in range(D // L)]
    for j in range(D // L):
        small_units.insert(2 * j + 2, P(m_unit, j))
    first_q = q_units(0)
    step = len(small_units) // len(first_q)
    for j, unit in enumerate(first_q):
        units += small_units[j * step:(j + 1) * step] + [unit]
    for i in range(nb):
        if i + 1 < nb:
            units += q_units(i + 1)
        units += [P(out_unit, i, n) for n in range(D // L)]
    cost = {k_unit: rc * tw * D, g_unit: rc * L * S, kv_unit: L * L * D, m_unit: L * L * D,
            q_unit: rq * tb * D, out_unit: tb * L * D}
    clock = [0]
    for unit in units:
        clock.append(clock[-1] + cost[unit.func] / (S * D * D))

    def at(time):
        return max(u for u in range(len(units)) if clock[u] <= time)

    def spread(jobs, t0, t1):
        for n, job in enumerate(jobs):
            after.setdefault(at(t0 + (t1 - t0) * n / len(jobs)), []).append(job)

    assert xc == tw == tb == 2 * L and nc == 4 and nl == 8
    xs = lambda *ids: [cp for i in ids for cp in cp_x(i)]
    wkt = lambda c: [P(transpose_w, wk_v, wkt_v, j) for j in range(c * rc // L, (c + 1) * rc // L)]
    best_v[...] = jnp.full(best_v.shape, -jnp.inf, F32)
    besti_v[...] = jnp.full(besti_v.shape, BIG, jnp.int32)
    wkt_v[D // 2:, :] = _pack(jnp.concatenate(
        [jnp.broadcast_to(w_r, (8, D)), jnp.broadcast_to(w_g, (8, D))], axis=0).astype(BF16))
    before[0] = [wait(*cp_k(0), *xs(0)), start(*cp_k(2), *cp_k(3))] + wkt(0)
    before[1] = [wait(*xs(1), *cp_k(1))]
    after[1] = wkt(1)
    before[3] = [wait(*cp_k(2), *cp_k(3)), start(*xs(2, 3))]
    after[3], after[4] = wkt(2), wkt(3)
    before[6] = [wait(*xs(2, 3)), start(*xs(4, 5, 6, 7))]
    spread([P(repack, i) for i in (6, 7, 4, 5, 0, 1, 2, 3)], clock[6], clock[12])
    before[12] = [wait(*xs(4, 5, 6, 7)), start(*cp_qvo())]
    spread([P(repack, i) for i in range(8, 16)], clock[12], clock[20])
    spread([P(split_parity, t) for t in range(nl)], 0.7, t_q)
    before.setdefault(at(t_q - lead), []).append(start(*cp_up(0)))
    before.setdefault(at(t_up - lead), []).append(start(*cp_up(1)))
    before.setdefault(at(t_mid - lead), []).append(start(*cp_d()))
    u_sel = at(t_sel)
    after.setdefault(u_sel, []).append(select)
    after.setdefault(u_sel + 1, []).append(gather)
    assert at(t_up) >= u_sel + 2
    before.setdefault(at(t_up), []).append(wait(*cp_up(0)))
    ups = lambda j0, j1: [job for j in range(j0, j1)
                          for job in [P(ffn_up, j, k) for k in range(D // 256)] + [P(ffn_act, j)]]
    spread(ups(0, fh // L), t_up, t_mid)
    before.setdefault(at(t_mid), []).append(wait(*cp_up(1)))
    spread(ups(fh // L, F // L), t_mid, t_down)
    before.setdefault(at(t_q), []).append(wait(*cp_qvo()))
    spread([P(transpose_w, wq_v, wqt_v, j) for j in range(D // L)], t_q, t_up)
    before.setdefault(at(t_down), []).append(wait(*cp_d()))
    spread([P(ffn_down, j, n) for j in range(F // L) for n in range(D // 512)],
           t_down, clock[len(units) - D // L - 2])

    posts = []
    for u, unit in enumerate(units):
        for job in before.get(u, []):
            job()
        posts.append(unit())
        if len(posts) > skew:
            posts.pop(0)()
        for job in after.get(u, []):
            token = job()
            if token is not None:
                tokens.append(token)
    for post in posts:
        post()
    for i in range(nb - 1):
        cp_o(i, block_of(i)).wait()
    for n in range(D // L):
        cp_o(nb - 1, block_of(nb - 1), n).wait()


def _build(rc=256, tw=256, tb=256, xc=256, skew=1, t_sel=1.05, t_mid=2.3, t_down=3.0, t_up=1.65, t_q=1.0, rq=128, ns=4, lead=0.05, flags=FLAGS):
    def run(A_x, A_wqkv, A_wo, B_x, B_w_r, B_w_gate, B_w_up, B_w_down, gate_w):
        B, S, D = A_x.shape
        F = B_w_gate.shape[1]
        hbm = pl.BlockSpec(memory_space=pl.ANY)
        vmem, dma = pltpu.VMEM, pltpu.SemaphoreType.DMA
        out = pl.pallas_call(
            functools.partial(_kernel, rc=rc, tw=tw, tb=tb, xc=xc, skew=skew,
                              t_sel=t_sel, t_mid=t_mid, t_down=t_down, t_up=t_up, t_q=t_q, rq=rq, ns=ns, lead=lead),
            out_shape=jax.ShapeDtypeStruct((S, D), BF16),
            in_specs=[hbm] * 8,
            out_specs=hbm,
            scratch_shapes=[
                vmem((S, D), BF16),
                vmem((2, D // 128, 128), BF16),
                vmem((D, D), BF16), vmem((D, D), BF16),
                vmem((D, D), BF16), vmem((D, D), BF16),
                vmem((D, F), BF16), vmem((D, F), BF16), vmem((F, D), BF16),
                vmem((D // 128, S // 2 + 8, 128), U32), vmem((S // 2, D), U32),
                vmem((D // 2, D), U32), vmem((D // 2 + 8, D), U32),
                vmem((D // 2, S), U32),
                vmem((D // 2, D), U32), vmem((D // 2, D), U32),
                vmem((tb, D), U32),
                vmem((D, 128), F32), vmem((S, 128), F32),
                vmem((8, 128), F32), vmem((8, 128), jnp.int32),
                vmem((D, 128), F32),
                vmem((8, F), F32), vmem((8, F), F32), vmem((F, 128), F32),
                vmem((8, D), F32),
                vmem((S, D), BF16),
                dma((2,)), dma((S // xc,)), dma((4,)), dma((D // rc,)), dma((S // tb + D // 128 - 1,)),
            ],
            compiler_params=pltpu.CompilerParams(
                vmem_limit_bytes=110 * 1024 * 1024, flags=flags),
        )(A_x.reshape(S, D), A_wqkv, A_wo, B_w_r.reshape(D // 128, 128),
          B_w_gate, B_w_up, B_w_down, gate_w.reshape(D // 128, 128))
        return out.reshape(B, S, D)
    return run


@jax.jit
def pallas_gated_mix__linear_attn_block__moe_arch_mod__prompt_kernel(
    A_x: jax.Array,
    A_wqkv: jax.Array,
    A_wo: jax.Array,
    B_x: jax.Array,
    B_w_r: jax.Array,
    B_w_gate: jax.Array,
    B_w_up: jax.Array,
    B_w_down: jax.Array,
    gate_w: jax.Array,
):
    return _build()(A_x, A_wqkv, A_wo, B_x, B_w_r, B_w_gate, B_w_up, B_w_down, gate_w)
```

```python
import functools

import jax
import jax.numpy as jnp
from jax import lax
import jax.experimental.pallas as pl
import jax.experimental.pallas.tpu as pltpu

F32 = jnp.float32
BF16 = jnp.bfloat16
U32 = jnp.uint32
HEADS = 32
BIG = 1 << 30
FLAGS = {"XLA_TPU_EVENLY_DISTRIBUTE_CRITICAL_NODES": True}
NT = (((1,), (1,)), ((), ()))
TN = (((0,), (0,)), ((), ()))


def _phi(t):
    return jnp.where(t > 0, t + 1.0, jnp.exp(t)) + 1e-6


def _sigmoid(t):
    return 1.0 / (1.0 + jnp.exp(-t))


def _pack(v):
    return pltpu.bitcast(v, jnp.uint32)


def _unpack(v):
    return pltpu.bitcast(v, BF16)


def _kernel(x_hbm, wqkv_hbm, wo_hbm, wr_hbm, wg_hbm, wu_hbm, wd_hbm, gw_hbm,
            out_hbm,
            x_v, vec_v, wq_v, wk_v, wv_v, wo_v, wg_v, wu_v, wd_v,
            xp_v, xq_v, wqt_v, wkt_v, pk_v, g_v, m_v, on_v, z_v, gate_v, best_v, besti_v,
            xb_v, hg_v, hu_v, hb_v, y_v, o_v,
            sem_s, sem_x, sem_w, sem_k, sem_o,
            rc=256, rk=128, rq=128, tw=256, tb=256, xc=256, kr=256, nw=512, ns=4, skew=1,
            lead=0.05, t_q=1.0, t_sel=1.05, t_up=1.65, t_mid=2.3, t_down=3.0):
    S, D = x_v.shape
    F = wg_v.shape[1]
    L = 128
    nc = D // rc
    nl = S // tw
    nb = S // tb
    dh = D // HEADS
    fh = F // 2

    def copies(src, dst, sem, rows, cols, shift, n):
        (r0, nr), (c0, ncol) = rows, cols
        return [pltpu.make_async_copy(src.at[pl.ds(r0 + k * nr // n, nr // n), pl.ds(c0 + shift, ncol)],
                                      dst.at[pl.ds(r0 + k * nr // n, nr // n), pl.ds(c0, ncol)], sem)
                for k in range(n)]

    cp_x = lambda i: copies(x_hbm, x_v, sem_x.at[i], (i * xc, xc), (0, D), 0, ns if i == 0 else 1)
    cp_k = lambda c: copies(wqkv_hbm, wk_v, sem_k.at[c], (0, D), (c * rc, rc), D, ns if c == 0 else 1)
    cp_qvo = lambda: (copies(wqkv_hbm, wq_v, sem_w.at[0], (0, D), (0, D), 0, 2)
                      + copies(wqkv_hbm, wv_v, sem_w.at[0], (0, D), (0, D), 2 * D, 2)
                      + copies(wo_hbm, wo_v, sem_w.at[0], (0, D), (0, D), 0, 2))
    cp_up = lambda j: (copies(wg_hbm, wg_v, sem_w.at[1 + j], (0, D), (j * fh, fh), 0, 2)
                       + copies(wu_hbm, wu_v, sem_w.at[1 + j], (0, D), (j * fh, fh), 0, 2))
    cp_d = lambda: copies(wd_hbm, wd_v, sem_w.at[3], (0, F), (0, D), 0, 4)

    def cp_o(i, t, n=None):
        cols = pl.ds(0, D) if n is None else pl.ds(n * L, L)
        return pltpu.make_async_copy(o_v.at[pl.ds(i * tb, tb), cols],
                                     out_hbm.at[pl.ds(pl.multiple_of(t * tb, tb), tb), cols],
                                     sem_o.at[i + (n or 0)])

    def start(*cps):
        return lambda: [cp.start() for cp in cps] and None

    def wait(*cps):
        return lambda: [cp.wait() for cp in cps] and None

    def packed(ref, lo, n):
        if isinstance(lo, int):
            return _unpack(ref[lo // 2:(lo + n) // 2, :])
        return _unpack(ref[pl.ds(pl.multiple_of(lo // 2, n // 2), n // 2), :])

    tokens = []
    start(*cp_k(0), *cp_x(0))()
    small = [pltpu.make_async_copy(src, vec_v.at[j], sem_s.at[j]) for j, src in enumerate((wr_hbm, gw_hbm))]
    start(*small, *cp_x(1), *cp_k(1))()
    wait(*small)()
    w_r, w_g = vec_v[0].astype(F32), vec_v[1].astype(F32)
    never = (pltpu.bitcast(w_g, jnp.int32) & 0xFFFF) != 0
    w_g, w_r = (jnp.concatenate([w[j:j + 1, :] for j in range(D // L)], axis=1) for w in (w_g, w_r))

    def digest(*vals):
        acc = None
        for v in vals:
            v = v if v.dtype == jnp.int32 else pltpu.bitcast(v, jnp.int32)
            for i in range(v.shape[0] // 8):
                for j in range(v.shape[1] // L):
                    e = v[i * 8:(i + 1) * 8, j * L:(j + 1) * L]
                    acc = e if acc is None else acc ^ e
        return acc

    def tie(v):
        if not tokens:
            return v
        head = jnp.where(never, pltpu.bitcast(digest(*tokens), v.dtype), v[0:8, 0:L])
        tokens.clear()
        if v.shape[1] > L:
            head = jnp.concatenate([head, v[0:8, L:]], axis=1)
        return jnp.concatenate([head, v[8:]], axis=0)

    def k_unit(c, t):
        r = slice(c * rk, (c + 1) * rk)
        if t < 3:
            xt = x_v[t * tw:(t + 1) * tw, :]
        else:
            xt = jnp.concatenate([packed(xp_v.at[n], t * tw, tw) for n in range(D // L)], axis=1)
        more = 8 if c == D // rk - 1 else 0
        w = _unpack(tie(wkt_v[c * rk // 2:(c + 1) * rk // 2 + more, :]))
        kt = lax.dot_general(w, xt, NT, preferred_element_type=F32)

        def post():
            if more:
                route(t * tw, kt[rk:rk + 8], kt[rk + 8:])
            tokens.append(besti_v[...])
            pk = _phi(tie(kt[:rk]))
            zs = pk[:, 0:L]
            for j in range(1, tw // L):
                zs = zs + pk[:, j * L:(j + 1) * L]
            if t > 0:
                zs = zs + z_v[r, :]
            if t == nl - 1:
                zs = jnp.broadcast_to(jnp.sum(zs, axis=-1, keepdims=True), zs.shape)
            z_v[r, :] = zs
            pk_v[c * rk // 2:(c + 1) * rk // 2, t * tw:(t + 1) * tw] = _pack(pk.astype(BF16))
        return post

    def g_unit(c, n):
        cols = slice(n * L, (n + 1) * L)
        g = jnp.dot(packed(pk_v, c * rc, rc), packed(xp_v.at[n], 0, S), preferred_element_type=F32)

        def post():
            g_v[c * rc // 2:(c + 1) * rc // 2, cols] = _pack(tie(g).astype(BF16))
        return post

    def kv_unit(j):
        q = slice(j * L, (j + 1) * L)
        kv = jnp.dot(packed(g_v, j * L, L), wv_v[:, q], preferred_element_type=F32)

        def post():
            same_head = (lax.broadcasted_iota(jnp.int32, (L, L), 0) // dh
                         == lax.broadcasted_iota(jnp.int32, (L, L), 1) // dh)
            kvs[j] = jnp.where(same_head, kv, 0.0).astype(BF16)
        return post

    def m_unit(j):
        m = jnp.dot(kvs.pop(j), wo_v[j * L:(j + 1) * L, :], preferred_element_type=F32)

        def post():
            m_v[j * L // 2:(j + 1) * L // 2, :] = _pack(m.astype(BF16))
        return post

    kvs, sel = {}, {}

    def block_of(i):
        return lax.rem(sel["blk"] + 1 + i, nb)

    def q_unit(i, c):
        r = slice(c * rq, (c + 1) * rq)
        q = lax.dot_general(packed(wqt_v, c * rq, rq), packed(xq_v, block_of(i) * tb, tb), NT,
                            preferred_element_type=F32)

        def post():
            pq = _phi(tie(q))
            z = jnp.tile(z_v[r, :], (1, tb // L))
            den = jnp.sum((pq * z).reshape(rq // dh, dh, tb), axis=1, keepdims=True) + 1e-6
            o = (pq.reshape(rq // dh, dh, tb) * (1.0 / den)).reshape(rq, tb)
            pairs = pltpu.pack_elementwise([o[:, :L], o[:, L:]], packed_dtype=BF16)
            on_v[(i % 2) * L:(i % 2 + 1) * L, r] = pltpu.bitcast(pairs, U32).T
        return post

    def out_unit(i, n):
        cols = slice(n * L, (n + 1) * L)
        a = jnp.dot(packed(on_v, (i % 2) * tb, tb), _unpack(m_v[:, cols]), preferred_element_type=F32)

        def post():
            lo = block_of(i) * tb
            gate = gate_v[pl.ds(pl.multiple_of(lo, tb), tb), :]
            bx = packed(xp_v.at[n], lo, tb).astype(F32)
            upd = bx * 0.0
            if i == nb - 1:
                y = jnp.sum(y_v[:, cols], axis=0, keepdims=True) * sel["w"]
                is_sel = lax.broadcasted_iota(jnp.int32, (tb, L), 0) + lo == sel["idx"]
                upd = upd + jnp.where(is_sel, y, 0.0)
            o_v[i * tb:(i + 1) * tb, cols] = (gate * tie(a) + (1.0 - gate) * (bx + upd)).astype(BF16)
            if i == nb - 1:
                cp_o(i, block_of(i), n).start()
            elif n == D // L - 1:
                cp_o(i, block_of(i)).start()
        return post

    def repack(i):
        xp = _pack(x_v[i * L:(i + 1) * L, :])
        for n in range(D // L):
            xp_v[n, i * L // 2:(i + 1) * L // 2, :] = xp[:, n * L:(n + 1) * L]
        return digest(xp)

    def split_parity(t):
        lo, n = t * tw // 2, tw // 4
        a, b = (jnp.concatenate([xp_v[k, pl.ds(lo + first, n, stride=2), :] for k in range(D // L)], axis=1)
                for first in (0, 1))
        even = (a & jnp.uint32(0xFFFF)) | (b << 16)
        odd = (a >> 16) | (b & jnp.uint32(0xFFFF0000))
        xq_v[lo:lo + n, :] = even
        xq_v[lo + n:lo + 2 * n, :] = odd
        return digest(even ^ odd)

    def transpose_w(src, dst, j):
        wt = _pack(src[:, j * L:(j + 1) * L].T)
        dst[j * L // 2:(j + 1) * L // 2, :] = wt
        return digest(wt)

    def route(lo, score, logit):
        score = score.astype(BF16).astype(F32)
        gate = _sigmoid(logit)
        best, besti = best_v[...], besti_v[...]
        for k in range(tw // L):
            s8 = score[:, k * L:(k + 1) * L]
            take = (s8 > best) | ((s8 == best) & (besti == BIG))
            best = jnp.where(take, s8, best)
            besti = jnp.where(take, lax.broadcasted_iota(jnp.int32, (8, L), 1) + (lo + k * L), besti)
            gate_v[lo + k * L:lo + (k + 1) * L, :] = jnp.tile(gate[:, k * L:(k + 1) * L], (L // 8, 1)).T
        best_v[...] = best
        besti_v[...] = besti

    def select():
        best, besti = best_v[...], besti_v[...]
        m = jnp.max(best[0:1], axis=1, keepdims=True)
        mi = jnp.min(jnp.where(best[0:1] == m, besti[0:1], BIG), axis=1, keepdims=True)
        none = mi == BIG
        sel["w"] = _sigmoid(jnp.where(none, jnp.nan, m))
        sel["idx"] = jnp.where(none, 0, mi)[0, 0]
        sel["blk"] = sel["idx"] // tb

    def gather():
        base = pl.multiple_of((sel["idx"] // 16) * 16, 16)
        slab = x_v[pl.ds(base, 16), :].astype(F32)
        pick = lax.broadcasted_iota(jnp.int32, (16, 1), 0) == sel["idx"] - base
        xs = jnp.sum(jnp.where(pick, slab, 0.0), axis=0, keepdims=True)
        xb_v[...] = jnp.broadcast_to(xs, (L, D)).T

    def ffn_up(j, k):
        f, r = slice(j * L, (j + 1) * L), slice(k * kr, (k + 1) * kr)
        xb = xb_v[r, :]
        parts = []
        for w_v, h_v in ((wg_v, hg_v), (wu_v, hu_v)):
            part = jnp.sum((w_v[r, f].astype(F32) * xb).reshape(kr // 8, 8, L), axis=0)
            parts.append(part if k == 0 else h_v[:, f] + part)
            h_v[:, f] = parts[-1]
        return digest(*parts)

    def ffn_act(j):
        f = slice(j * L, (j + 1) * L)
        hg = jnp.sum(hg_v[:, f], axis=0, keepdims=True)
        hu = jnp.sum(hu_v[:, f], axis=0, keepdims=True)
        hb = jnp.broadcast_to(hg * _sigmoid(hg) * hu, (L, L)).T
        hb_v[f, :] = hb
        return digest(hb)

    def ffn_down(j, n):
        f, cols = slice(j * L, (j + 1) * L), slice(n * nw, (n + 1) * nw)
        hb = jnp.tile(hb_v[f, :], (1, nw // L))
        part = jnp.sum((wd_v[f, cols].astype(F32) * hb).reshape(L // 8, 8, nw), axis=0)
        part = part if j == 0 else y_v[:, cols] + part
        y_v[:, cols] = part
        return digest(part)

    P = functools.partial
    units, before, after = [], {}, {}
    ks = rc // rk
    units += [P(k_unit, c * ks + h, t) for c in range(nc) for t in range(2) for h in range(ks)]
    units += [P(k_unit, c, t) for t in range(2, nl) for c in range(nc * ks)]
    units += [P(g_unit, c, n) for c in range(nc) for n in range(D // L)]
    q_units = lambda i: [P(q_unit, i, c) for c in range(D // rq)]
    small_units = [P(kv_unit, j) for j in range(D // L)]
    for j in range(D // L):
        small_units.insert(2 * j + 2, P(m_unit, j))
    first_q = q_units(0)
    step = len(small_units) // len(first_q)
    for j, unit in enumerate(first_q):
        units += small_units[j * step:(j + 1) * step] + [unit]
    for i in range(nb):
        if i + 1 < nb:
            units += q_units(i + 1)
        units += [P(out_unit, i, n) for n in range(D // L)]
    cost = {k_unit: rk * tw * D, g_unit: rc * L * S, kv_unit: L * L * D, m_unit: L * L * D,
            q_unit: rq * tb * D, out_unit: tb * L * D}
    clock = [0]
    for unit in units:
        clock.append(clock[-1] + cost[unit.func] / (S * D * D))

    def at(time):
        return max(u for u in range(len(units)) if clock[u] <= time + 1e-9)

    def spread(jobs, t0, t1):
        for n, job in enumerate(jobs):
            after.setdefault(at(t0 + (t1 - t0) * n / len(jobs)), []).append(job)

    assert xc == tw == tb == 2 * L and nc == 4 and nl == 8
    xs = lambda *ids: [cp for i in ids for cp in cp_x(i)]
    wkt = lambda c: [P(transpose_w, wk_v, wkt_v, j) for j in range(c * rc // L, (c + 1) * rc // L)]
    best_v[...] = jnp.full(best_v.shape, -jnp.inf, F32)
    besti_v[...] = jnp.full(besti_v.shape, BIG, jnp.int32)
    wkt_v[D // 2:, :] = _pack(jnp.concatenate(
        [jnp.broadcast_to(w_r, (8, D)), jnp.broadcast_to(w_g, (8, D))], axis=0).astype(BF16))
    before[0] = [wait(*cp_k(0), *xs(0)), start(*cp_k(2), *cp_k(3))] + wkt(0)
    before[ks] = [wait(*xs(1), *cp_k(1))]
    spread(wkt(1), clock[ks], clock[2 * ks])
    before[3 * ks] = [wait(*cp_k(2), *cp_k(3)), start(*xs(2, 3))]
    spread(wkt(2) + wkt(3), clock[3 * ks], clock[5 * ks])
    before[6 * ks] = [wait(*xs(2, 3)), start(*xs(4, 5, 6, 7))]
    spread([P(repack, i) for i in (6, 7, 4, 5, 0, 1, 2, 3)], clock[6 * ks], clock[12 * ks])
    before[12 * ks] = [wait(*xs(4, 5, 6, 7)), start(*cp_qvo())]
    spread([P(repack, i) for i in range(8, 16)], clock[12 * ks], clock[20 * ks])
    spread([P(split_parity, t) for t in range(nl)], 0.7, t_q)
    before.setdefault(at(t_q - lead), []).append(start(*cp_up(0)))
    before.setdefault(at(t_up - lead), []).append(start(*cp_up(1)))
    before.setdefault(at(t_mid - lead), []).append(start(*cp_d()))
    u_sel = at(t_sel)
    after.setdefault(u_sel, []).append(select)
    after.setdefault(u_sel + 1, []).append(gather)
    assert at(t_up) >= u_sel + 2
    before.setdefault(at(t_up), []).append(wait(*cp_up(0)))
    ups = lambda j0, j1: [job for j in range(j0, j1)
                          for job in [P(ffn_up, j, k) for k in range(D // kr)] + [P(ffn_act, j)]]
    spread(ups(0, fh // L), t_up, t_mid)
    before.setdefault(at(t_mid), []).append(wait(*cp_up(1)))
    spread(ups(fh // L, F // L), t_mid, t_down)
    before.setdefault(at(t_q), []).append(wait(*cp_qvo()))
    spread([P(transpose_w, wq_v, wqt_v, j) for j in range(D // L)], t_q, t_up)
    before.setdefault(at(t_down), []).append(wait(*cp_d()))
    spread([P(ffn_down, j, n) for j in range(F // L) for n in range(D // nw)],
           t_down, clock[len(units) - D // L - 2])

    posts = []
    for u, unit in enumerate(units):
        for job in before.get(u, []):
            job()
        posts.append(unit())
        if len(posts) > skew:
            posts.pop(0)()
        for job in after.get(u, []):
            token = job()
            if token is not None:
                tokens.append(token)
    for post in posts:
        post()
    for i in range(nb - 1):
        cp_o(i, block_of(i)).wait()
    for n in range(D // L):
        cp_o(nb - 1, block_of(nb - 1), n).wait()


def _build(flags=FLAGS, **tuning):
    def run(A_x, A_wqkv, A_wo, B_x, B_w_r, B_w_gate, B_w_up, B_w_down, gate_w):
        B, S, D = A_x.shape
        F = B_w_gate.shape[1]
        hbm = pl.BlockSpec(memory_space=pl.ANY)
        vmem, dma = pltpu.VMEM, pltpu.SemaphoreType.DMA
        out = pl.pallas_call(
            functools.partial(_kernel, **tuning),
            out_shape=jax.ShapeDtypeStruct((S, D), BF16),
            in_specs=[hbm] * 8,
            out_specs=hbm,
            scratch_shapes=[
                vmem((S, D), BF16),
                vmem((2, D // 128, 128), BF16),
                vmem((D, D), BF16), vmem((D, D), BF16),
                vmem((D, D), BF16), vmem((D, D), BF16),
                vmem((D, F), BF16), vmem((D, F), BF16), vmem((F, D), BF16),
                vmem((D // 128, S // 2 + 8, 128), U32), vmem((S // 2, D), U32),
                vmem((D // 2, D), U32), vmem((D // 2 + 8, D), U32),
                vmem((D // 2, S), U32),
                vmem((D // 2, D), U32), vmem((D // 2, D), U32),
                vmem((256, D), U32),
                vmem((D, 128), F32), vmem((S, 128), F32),
                vmem((8, 128), F32), vmem((8, 128), jnp.int32),
                vmem((D, 128), F32),
                vmem((8, F), F32), vmem((8, F), F32), vmem((F, 128), F32),
                vmem((8, D), F32),
                vmem((S, D), BF16),
                dma((2,)), dma((S // 256,)), dma((4,)), dma((D // 256,)), dma((S // 256 + D // 128 - 1,)),
            ],
            compiler_params=pltpu.CompilerParams(
                vmem_limit_bytes=110 * 1024 * 1024, flags=flags),
        )(A_x.reshape(S, D), A_wqkv, A_wo, B_w_r.reshape(D // 128, 128),
          B_w_gate, B_w_up, B_w_down, gate_w.reshape(D // 128, 128))
        return out.reshape(B, S, D)
    return run


@jax.jit
def pallas_gated_mix__linear_attn_block__moe_arch_mod__prompt_kernel(
    A_x: jax.Array,
    A_wqkv: jax.Array,
    A_wo: jax.Array,
    B_x: jax.Array,
    B_w_r: jax.Array,
    B_w_gate: jax.Array,
    B_w_up: jax.Array,
    B_w_down: jax.Array,
    gate_w: jax.Array,
):
    return _build()(A_x, A_wqkv, A_wo, B_x, B_w_r, B_w_gate, B_w_up, B_w_down, gate_w)
```

```python
import functools

import jax
import jax.numpy as jnp
from jax import lax
import jax.experimental.pallas as pl
import jax.experimental.pallas.tpu as pltpu

F32 = jnp.float32
BF16 = jnp.bfloat16
U32 = jnp.uint32
HEADS = 32
BIG = 1 << 30
FLAGS = {"XLA_TPU_EVENLY_DISTRIBUTE_CRITICAL_NODES": True}
NT = (((1,), (1,)), ((), ()))
TN = (((0,), (0,)), ((), ()))


def _phi(t):
    return jnp.where(t > 0, t + 1.0, jnp.exp(t)) + 1e-6


def _sigmoid(t):
    return 1.0 / (1.0 + jnp.exp(-t))


def _pack(v):
    return pltpu.bitcast(v, jnp.uint32)


def _unpack(v):
    return pltpu.bitcast(v, BF16)


def _kernel(x_hbm, wqkv_hbm, wo_hbm, wr_hbm, wg_hbm, wu_hbm, wd_hbm, gw_hbm,
            out_hbm,
            x_v, vec_v, wq_v, wk_v, wv_v, wo_v, wg_v, wu_v, wd_v,
            xp_v, xq_v, wqt_v, wkt_v, pk_v, g_v, m_v, on_v, z_v, gate_v, best_v, besti_v,
            xb_v, hg_v, hu_v, hb_v, y_v, o_v,
            sem_s, sem_x, sem_w, sem_k, sem_o,
            rc=256, rk=128, rq=128, tw=256, tb=256, xc=256, kr=256, nw=512, ns=4, skew=1,
            lead=0.05, t_q=1.0, t_sel=1.05, t_up=1.65, t_mid=2.3, t_down=3.0):
    S, D = x_v.shape
    F = wg_v.shape[1]
    L = 128
    nc = D // rc
    nl = S // tw
    nb = S // tb
    dh = D // HEADS
    fh = F // 2

    def copies(src, dst, sem, rows, cols, shift, n):
        (r0, nr), (c0, ncol) = rows, cols
        return [pltpu.make_async_copy(src.at[pl.ds(r0 + k * nr // n, nr // n), pl.ds(c0 + shift, ncol)],
                                      dst.at[pl.ds(r0 + k * nr // n, nr // n), pl.ds(c0, ncol)], sem)
                for k in range(n)]

    cp_x = lambda i: copies(x_hbm, x_v, sem_x.at[i], (i * xc, xc), (0, D), 0, ns if i == 0 else 1)
    cp_k = lambda c: copies(wqkv_hbm, wk_v, sem_k.at[c], (0, D), (c * rc, rc), D, ns if c == 0 else 1)
    cp_qvo = lambda: (copies(wqkv_hbm, wq_v, sem_w.at[0], (0, D), (0, D), 0, 2)
                      + copies(wqkv_hbm, wv_v, sem_w.at[0], (0, D), (0, D), 2 * D, 2)
                      + copies(wo_hbm, wo_v, sem_w.at[0], (0, D), (0, D), 0, 2))
    cp_up = lambda j: (copies(wg_hbm, wg_v, sem_w.at[1 + j], (0, D), (j * fh, fh), 0, 2)
                       + copies(wu_hbm, wu_v, sem_w.at[1 + j], (0, D), (j * fh, fh), 0, 2))
    cp_d = lambda: copies(wd_hbm, wd_v, sem_w.at[3], (0, F), (0, D), 0, 4)

    def cp_o(i, t, n=None):
        cols = pl.ds(0, D) if n is None else pl.ds(n * L, L)
        return pltpu.make_async_copy(o_v.at[pl.ds(i * tb, tb), cols],
                                     out_hbm.at[pl.ds(pl.multiple_of(t * tb, tb), tb), cols],
                                     sem_o.at[i + (n or 0)])

    def start(*cps):
        return lambda: [cp.start() for cp in cps] and None

    def wait(*cps):
        return lambda: [cp.wait() for cp in cps] and None

    def packed(ref, lo, n):
        if isinstance(lo, int):
            return _unpack(ref[lo // 2:(lo + n) // 2, :])
        return _unpack(ref[pl.ds(pl.multiple_of(lo // 2, n // 2), n // 2), :])

    tokens = []
    start(*cp_k(0), *cp_x(0))()
    small = [pltpu.make_async_copy(src, vec_v.at[j], sem_s.at[j]) for j, src in enumerate((wr_hbm, gw_hbm))]
    start(*small, *cp_x(1), *cp_k(1))()
    wait(*small)()
    w_r, w_g = vec_v[0].astype(F32), vec_v[1].astype(F32)
    never = (pltpu.bitcast(w_g, jnp.int32) & 0xFFFF) != 0
    w_g, w_r = (jnp.concatenate([w[j:j + 1, :] for j in range(D // L)], axis=1) for w in (w_g, w_r))

    def digest(*vals):
        acc = None
        for v in vals:
            v = v if v.dtype == jnp.int32 else pltpu.bitcast(v, jnp.int32)
            for i in range(v.shape[0] // 8):
                for j in range(v.shape[1] // L):
                    e = v[i * 8:(i + 1) * 8, j * L:(j + 1) * L]
                    acc = e if acc is None else acc ^ e
        return acc

    def tie(v):
        if not tokens:
            return v
        head = jnp.where(never, pltpu.bitcast(digest(*tokens), v.dtype), v[0:8, 0:L])
        tokens.clear()
        if v.shape[1] > L:
            head = jnp.concatenate([head, v[0:8, L:]], axis=1)
        return jnp.concatenate([head, v[8:]], axis=0)

    def k_unit(c, t):
        r = slice(c * rk, (c + 1) * rk)
        if t < 3:
            xt = x_v[t * tw:(t + 1) * tw, :]
        else:
            xt = jnp.concatenate([packed(xp_v.at[n], t * tw, tw) for n in range(D // L)], axis=1)
        more = 8 if c == D // rk - 1 else 0
        w = _unpack(tie(wkt_v[c * rk // 2:(c + 1) * rk // 2 + more, :]))
        kt = lax.dot_general(w, xt, NT, preferred_element_type=F32)

        def post():
            if more:
                route(t * tw, kt[rk:rk + 8], kt[rk + 8:])
            tokens.append(besti_v[...])
            pk = _phi(tie(kt[:rk]))
            zs = pk[:, 0:L]
            for j in range(1, tw // L):
                zs = zs + pk[:, j * L:(j + 1) * L]
            if t > 0:
                zs = zs + z_v[r, :]
            if t == nl - 1:
                zs = jnp.broadcast_to(jnp.sum(zs, axis=-1, keepdims=True), zs.shape)
            z_v[r, :] = zs
            pk_v[c * rk // 2:(c + 1) * rk // 2, t * tw:(t + 1) * tw] = _pack(pk.astype(BF16))
        return post

    def g_unit(c, n):
        cols = slice(n * L, (n + 1) * L)
        g = jnp.dot(packed(pk_v, c * rc, rc), packed(xp_v.at[n], 0, S), preferred_element_type=F32)

        def post():
            g_v[c * rc // 2:(c + 1) * rc // 2, cols] = _pack(tie(g).astype(BF16))
        return post

    def kv_unit(j):
        q = slice(j * L, (j + 1) * L)
        kv = jnp.dot(packed(g_v, j * L, L), wv_v[:, q], preferred_element_type=F32)

        def post():
            same_head = (lax.broadcasted_iota(jnp.int32, (L, L), 0) // dh
                         == lax.broadcasted_iota(jnp.int32, (L, L), 1) // dh)
            kvs[j] = jnp.where(same_head, kv, 0.0).astype(BF16)
        return post

    def m_unit(j):
        m = jnp.dot(kvs.pop(j), wo_v[j * L:(j + 1) * L, :], preferred_element_type=F32)

        def post():
            m_v[j * L // 2:(j + 1) * L // 2, :] = _pack(m.astype(BF16))
        return post

    kvs, sel = {}, {}

    def block_of(i):
        return lax.rem(sel["blk"] + 1 + i, nb)

    def q_unit(i, c):
        r = slice(c * rq, (c + 1) * rq)
        q = lax.dot_general(packed(wqt_v, c * rq, rq), packed(xq_v, block_of(i) * tb, tb), NT,
                            preferred_element_type=F32)

        def post():
            pq = _phi(tie(q))
            z = jnp.tile(z_v[r, :], (1, tb // L))
            den = jnp.sum((pq * z).reshape(rq // dh, dh, tb), axis=1, keepdims=True) + 1e-6
            o = (pq.reshape(rq // dh, dh, tb) * (1.0 / den)).reshape(rq, tb)
            pairs = pltpu.pack_elementwise([o[:, :L], o[:, L:]], packed_dtype=BF16)
            on_v[(i % 2) * L:(i % 2 + 1) * L, r] = pltpu.bitcast(pairs, U32).T
        return post

    def out_unit(i, n):
        cols = slice(n * L, (n + 1) * L)
        a = jnp.dot(packed(on_v, (i % 2) * tb, tb), _unpack(m_v[:, cols]), preferred_element_type=F32)

        def post():
            lo = block_of(i) * tb
            gate = gate_v[pl.ds(pl.multiple_of(lo, tb), tb), :]
            bx = packed(xp_v.at[n], lo, tb).astype(F32)
            upd = bx * 0.0
            if i == nb - 1:
                y = jnp.sum(y_v[:, cols], axis=0, keepdims=True) * sel["w"]
                is_sel = lax.broadcasted_iota(jnp.int32, (tb, L), 0) + lo == sel["idx"]
                upd = upd + jnp.where(is_sel, y, 0.0)
            o_v[i * tb:(i + 1) * tb, cols] = (gate * tie(a) + (1.0 - gate) * (bx + upd)).astype(BF16)
            if i == nb - 1:
                cp_o(i, block_of(i), n).start()
            elif n == D // L - 1:
                cp_o(i, block_of(i)).start()
        return post

    def repack(i):
        xp = _pack(x_v[i * L:(i + 1) * L, :])
        for n in range(D // L):
            xp_v[n, i * L // 2:(i + 1) * L // 2, :] = xp[:, n * L:(n + 1) * L]
        return digest(xp)

    def split_parity(t):
        lo, n = t * tw // 2, tw // 4
        a, b = (jnp.concatenate([xp_v[k, pl.ds(lo + first, n, stride=2), :] for k in range(D // L)], axis=1)
                for first in (0, 1))
        even = (a & jnp.uint32(0xFFFF)) | (b << 16)
        odd = (a >> 16) | (b & jnp.uint32(0xFFFF0000))
        xq_v[lo:lo + n, :] = even
        xq_v[lo + n:lo + 2 * n, :] = odd
        return digest(even ^ odd)

    def transpose_w(src, dst, j):
        wt = _pack(src[:, j * L:(j + 1) * L].T)
        dst[j * L // 2:(j + 1) * L // 2, :] = wt
        return digest(wt)

    def route(lo, score, logit):
        score = score.astype(BF16).astype(F32)
        gate = _sigmoid(logit)
        best, besti = best_v[...], besti_v[...]
        for k in range(tw // L):
            s8 = score[:, k * L:(k + 1) * L]
            take = (s8 > best) | ((s8 == best) & (besti == BIG))
            best = jnp.where(take, s8, best)
            besti = jnp.where(take, lax.broadcasted_iota(jnp.int32, (8, L), 1) + (lo + k * L), besti)
            gate_v[lo + k * L:lo + (k + 1) * L, :] = jnp.tile(gate[:, k * L:(k + 1) * L], (L // 8, 1)).T
        best_v[...] = best
        besti_v[...] = besti

    def select():
        best, besti = best_v[...], besti_v[...]
        m = jnp.max(best[0:1], axis=1, keepdims=True)
        mi = jnp.min(jnp.where(best[0:1] == m, besti[0:1], BIG), axis=1, keepdims=True)
        none = mi == BIG
        sel["w"] = _sigmoid(jnp.where(none, jnp.nan, m))
        sel["idx"] = jnp.where(none, 0, mi)[0, 0]
        sel["blk"] = sel["idx"] // tb

    def gather():
        base = pl.multiple_of((sel["idx"] // 16) * 16, 16)
        slab = x_v[pl.ds(base, 16), :].astype(F32)
        pick = lax.broadcasted_iota(jnp.int32, (16, 1), 0) == sel["idx"] - base
        xs = jnp.sum(jnp.where(pick, slab, 0.0), axis=0, keepdims=True)
        xb_v[...] = jnp.broadcast_to(xs, (L, D)).T

    def ffn_up(j, k):
        f, r = slice(j * L, (j + 1) * L), slice(k * kr, (k + 1) * kr)
        xb = xb_v[r, :]
        parts = []
        for w_v, h_v in ((wg_v, hg_v), (wu_v, hu_v)):
            part = jnp.sum((w_v[r, f].astype(F32) * xb).reshape(kr // 8, 8, L), axis=0)
            parts.append(part if k == 0 else h_v[:, f] + part)
            h_v[:, f] = parts[-1]
        return digest(*parts)

    def ffn_act(j):
        f = slice(j * L, (j + 1) * L)
        hg = jnp.sum(hg_v[:, f], axis=0, keepdims=True)
        hu = jnp.sum(hu_v[:, f], axis=0, keepdims=True)
        hb = jnp.broadcast_to(hg * _sigmoid(hg) * hu, (L, L)).T
        hb_v[f, :] = hb
        return digest(hb)

    def ffn_down(j, n):
        f, cols = slice(j * L, (j + 1) * L), slice(n * nw, (n + 1) * nw)
        hb = jnp.tile(hb_v[f, :], (1, nw // L))
        part = jnp.sum((wd_v[f, cols].astype(F32) * hb).reshape(L // 8, 8, nw), axis=0)
        part = part if j == 0 else y_v[:, cols] + part
        y_v[:, cols] = part
        return digest(part)

    P = functools.partial
    units, before, after = [], {}, {}
    ks = rc // rk
    units += [P(k_unit, c * ks + h, t) for c in range(nc) for t in range(2) for h in range(ks)]
    units += [P(k_unit, c, t) for t in range(2, nl) for c in range(nc * ks)]
    units += [P(g_unit, c, n) for c in range(nc) for n in range(D // L)]
    q_units = lambda i: [P(q_unit, i, c) for c in range(D // rq)]
    small_units = [P(kv_unit, j) for j in range(D // L)]
    for j in range(D // L):
        small_units.insert(2 * j + 2, P(m_unit, j))
    first_q = q_units(0)
    step = len(small_units) // len(first_q)
    for j, unit in enumerate(first_q):
        units += small_units[j * step:(j + 1) * step] + [unit]
    for i in range(nb):
        if i + 1 < nb:
            units += q_units(i + 1)
        units += [P(out_unit, i, n) for n in range(D // L)]
    cost = {k_unit: rk * tw * D, g_unit: rc * L * S, kv_unit: L * L * D, m_unit: L * L * D,
            q_unit: rq * tb * D, out_unit: tb * L * D}
    clock = [0]
    for unit in units:
        clock.append(clock[-1] + cost[unit.func] / (S * D * D))

    def at(time):
        return max(u for u in range(len(units)) if clock[u] <= time + 1e-9)

    def spread(jobs, t0, t1):
        for n, job in enumerate(jobs):
            after.setdefault(at(t0 + (t1 - t0) * n / len(jobs)), []).append(job)

    assert xc == tw == tb == rc == 2 * rk == 2 * L and nc == 4 and nl == 8
    xs = lambda *ids: [cp for i in ids for cp in cp_x(i)]
    wkt = lambda c: [P(transpose_w, wk_v, wkt_v, j) for j in range(c * rc // L, (c + 1) * rc // L)]
    best_v[...] = jnp.full(best_v.shape, -jnp.inf, F32)
    besti_v[...] = jnp.full(besti_v.shape, BIG, jnp.int32)
    wkt_v[D // 2:, :] = _pack(jnp.concatenate(
        [jnp.broadcast_to(w_r, (8, D)), jnp.broadcast_to(w_g, (8, D))], axis=0).astype(BF16))
    before[0] = [wait(*cp_k(0), *xs(0)), start(*cp_k(2), *cp_k(3))] + wkt(0)[:1]
    after[0] = wkt(0)[1:]
    before[ks] = [wait(*xs(1), *cp_k(1))]
    spread(wkt(1), clock[ks], clock[2 * ks])
    before[6] = [start(*xs(2, 3))]
    before[7] = [wait(*cp_k(2), *cp_k(3))]
    spread(wkt(2) + wkt(3), clock[7], clock[11])
    before[6 * ks] = [wait(*xs(2, 3)), start(*xs(4, 5, 6, 7))]
    spread([P(repack, i) for i in (6, 7, 4, 5, 0, 1, 2, 3)], clock[6 * ks], clock[12 * ks])
    before[12 * ks] = [wait(*xs(4, 5, 6, 7)), start(*cp_qvo())]
    spread([P(repack, i) for i in range(8, 16)], clock[12 * ks], clock[20 * ks])
    spread([P(split_parity, t) for t in range(nl)], 0.7, t_q)
    before.setdefault(at(t_q - lead), []).append(start(*cp_up(0)))
    before.setdefault(at(t_up - lead), []).append(start(*cp_up(1)))
    before.setdefault(at(t_mid - lead), []).append(start(*cp_d()))
    u_sel = at(t_sel)
    after.setdefault(u_sel, []).append(select)
    after.setdefault(u_sel + 1, []).append(gather)
    assert at(t_up) >= u_sel + 2
    before.setdefault(at(t_up), []).append(wait(*cp_up(0)))
    ups = lambda j0, j1: [job for j in range(j0, j1)
                          for job in [P(ffn_up, j, k) for k in range(D // kr)] + [P(ffn_act, j)]]
    spread(ups(0, fh // L), t_up, t_mid)
    before.setdefault(at(t_mid), []).append(wait(*cp_up(1)))
    spread(ups(fh // L, F // L), t_mid, t_down)
    before.setdefault(at(t_q), []).append(wait(*cp_qvo()))
    spread([P(transpose_w, wq_v, wqt_v, j) for j in range(D // L)], t_q, t_up)
    before.setdefault(at(t_down), []).append(wait(*cp_d()))
    spread([P(ffn_down, j, n) for j in range(F // L) for n in range(D // nw)],
           t_down, clock[len(units) - D // L - 2])

    posts = []
    for u, unit in enumerate(units):
        for job in before.get(u, []):
            job()
        posts.append(unit())
        if len(posts) > skew:
            posts.pop(0)()
        for job in after.get(u, []):
            token = job()
            if token is not None:
                tokens.append(token)
    for post in posts:
        post()
    for i in range(nb - 1):
        cp_o(i, block_of(i)).wait()
    for n in range(D // L):
        cp_o(nb - 1, block_of(nb - 1), n).wait()


def _build(flags=FLAGS, **tuning):
    def run(A_x, A_wqkv, A_wo, B_x, B_w_r, B_w_gate, B_w_up, B_w_down, gate_w):
        B, S, D = A_x.shape
        F = B_w_gate.shape[1]
        hbm = pl.BlockSpec(memory_space=pl.ANY)
        vmem, dma = pltpu.VMEM, pltpu.SemaphoreType.DMA
        out = pl.pallas_call(
            functools.partial(_kernel, **tuning),
            out_shape=jax.ShapeDtypeStruct((S, D), BF16),
            in_specs=[hbm] * 8,
            out_specs=hbm,
            scratch_shapes=[
                vmem((S, D), BF16),
                vmem((2, D // 128, 128), BF16),
                vmem((D, D), BF16), vmem((D, D), BF16),
                vmem((D, D), BF16), vmem((D, D), BF16),
                vmem((D, F), BF16), vmem((D, F), BF16), vmem((F, D), BF16),
                vmem((D // 128, S // 2 + 8, 128), U32), vmem((S // 2, D), U32),
                vmem((D // 2, D), U32), vmem((D // 2 + 8, D), U32),
                vmem((D // 2, S), U32),
                vmem((D // 2, D), U32), vmem((D // 2, D), U32),
                vmem((256, D), U32),
                vmem((D, 128), F32), vmem((S, 128), F32),
                vmem((8, 128), F32), vmem((8, 128), jnp.int32),
                vmem((D, 128), F32),
                vmem((8, F), F32), vmem((8, F), F32), vmem((F, 128), F32),
                vmem((8, D), F32),
                vmem((S, D), BF16),
                dma((2,)), dma((S // 256,)), dma((4,)), dma((D // 256,)), dma((S // 256 + D // 128 - 1,)),
            ],
            compiler_params=pltpu.CompilerParams(
                vmem_limit_bytes=110 * 1024 * 1024, flags=flags),
        )(A_x.reshape(S, D), A_wqkv, A_wo, B_w_r.reshape(D // 128, 128),
          B_w_gate, B_w_up, B_w_down, gate_w.reshape(D // 128, 128))
        return out.reshape(B, S, D)
    return run


@jax.jit
def pallas_gated_mix__linear_attn_block__moe_arch_mod__prompt_kernel(
    A_x: jax.Array,
    A_wqkv: jax.Array,
    A_wo: jax.Array,
    B_x: jax.Array,
    B_w_r: jax.Array,
    B_w_gate: jax.Array,
    B_w_up: jax.Array,
    B_w_down: jax.Array,
    gate_w: jax.Array,
):
    return _build()(A_x, A_wqkv, A_wo, B_x, B_w_r, B_w_gate, B_w_up, B_w_down, gate_w)
```

```python
import functools

import jax
import jax.numpy as jnp
from jax import lax
import jax.experimental.pallas as pl
import jax.experimental.pallas.tpu as pltpu

F32 = jnp.float32
BF16 = jnp.bfloat16
U32 = jnp.uint32
HEADS = 32
BIG = 1 << 30
FLAGS = {"XLA_TPU_EVENLY_DISTRIBUTE_CRITICAL_NODES": True}
NT = (((1,), (1,)), ((), ()))
TN = (((0,), (0,)), ((), ()))


def _phi(t):
    return jnp.where(t > 0, t + 1.0, jnp.exp(t)) + 1e-6


def _sigmoid(t):
    return 1.0 / (1.0 + jnp.exp(-t))


def _pack(v):
    return pltpu.bitcast(v, jnp.uint32)


def _unpack(v):
    return pltpu.bitcast(v, BF16)


def _kernel(x_hbm, wqkv_hbm, wo_hbm, wr_hbm, wg_hbm, wu_hbm, wd_hbm, gw_hbm,
            out_hbm,
            x_v, vec_v, wq_v, wk_v, wv_v, wo_v, wg_v, wu_v, wd_v,
            xp_v, xq_v, wqt_v, wkt_v, pk_v, g_v, m_v, on_v, z_v, gate_v, best_v, besti_v,
            xb_v, hg_v, hu_v, hb_v, y_v, o_v,
            sem_s, sem_x, sem_w, sem_k, sem_o,
            rc=256, rk=128, rq=128, tw=256, tb=256, xc=256, kr=256, nw=512, ns=4, skew=1,
            lead=0.05, t_sel=1.05, t_up=1.72, t_mid=2.35, t_down=3.1):
    S, D = x_v.shape
    F = wg_v.shape[1]
    L = 128
    nc = D // rc
    nl = S // tw
    nb = S // tb
    dh = D // HEADS
    fh = F // 2

    def copies(src, dst, sem, rows, cols, shift, n):
        (r0, nr), (c0, ncol) = rows, cols
        return [pltpu.make_async_copy(src.at[pl.ds(r0 + k * nr // n, nr // n), pl.ds(c0 + shift, ncol)],
                                      dst.at[pl.ds(r0 + k * nr // n, nr // n), pl.ds(c0, ncol)], sem)
                for k in range(n)]

    cp_x = lambda i: copies(x_hbm, x_v, sem_x.at[i], (i * xc, xc), (0, D), 0, ns if i == 0 else 1)
    cp_k = lambda c: copies(wqkv_hbm, wk_v, sem_k.at[c], (0, D), (c * rc, rc), D, ns if c == 0 else 1)
    cp_qvo = lambda: (copies(wqkv_hbm, wq_v, sem_w.at[0], (0, D), (0, D), 0, 2)
                      + copies(wqkv_hbm, wv_v, sem_w.at[0], (0, D), (0, D), 2 * D, 2)
                      + copies(wo_hbm, wo_v, sem_w.at[0], (0, D), (0, D), 0, 2))
    cp_up = lambda j: (copies(wg_hbm, wg_v, sem_w.at[1 + j], (0, D), (j * fh, fh), 0, 2)
                       + copies(wu_hbm, wu_v, sem_w.at[1 + j], (0, D), (j * fh, fh), 0, 2))
    cp_d = lambda: copies(wd_hbm, wd_v, sem_w.at[3], (0, F), (0, D), 0, 4)

    def cp_o(i, t, n=None):
        cols = pl.ds(0, D) if n is None else pl.ds(n * L, L)
        return pltpu.make_async_copy(o_v.at[pl.ds(i * tb, tb), cols],
                                     out_hbm.at[pl.ds(pl.multiple_of(t * tb, tb), tb), cols],
                                     sem_o.at[i + (n or 0)])

    def start(*cps):
        return lambda: [cp.start() for cp in cps] and None

    def wait(*cps):
        return lambda: [cp.wait() for cp in cps] and None

    def packed(ref, lo, n):
        if isinstance(lo, int):
            return _unpack(ref[lo // 2:(lo + n) // 2, :])
        return _unpack(ref[pl.ds(pl.multiple_of(lo // 2, n // 2), n // 2), :])

    tokens = []
    start(*cp_k(0), *cp_x(0))()
    small = [pltpu.make_async_copy(src, vec_v.at[j], sem_s.at[j]) for j, src in enumerate((wr_hbm, gw_hbm))]
    start(*small, *cp_x(1), *cp_k(1))()
    wait(*small)()
    w_r, w_g = vec_v[0].astype(F32), vec_v[1].astype(F32)
    never = (pltpu.bitcast(w_g, jnp.int32) & 0xFFFF) != 0
    w_g, w_r = (jnp.concatenate([w[j:j + 1, :] for j in range(D // L)], axis=1) for w in (w_g, w_r))

    def digest(*vals):
        acc = None
        for v in vals:
            v = v if v.dtype == jnp.int32 else pltpu.bitcast(v, jnp.int32)
            for i in range(v.shape[0] // 8):
                for j in range(v.shape[1] // L):
                    e = v[i * 8:(i + 1) * 8, j * L:(j + 1) * L]
                    acc = e if acc is None else acc ^ e
        return acc

    def tie(v):
        if not tokens:
            return v
        head = jnp.where(never, pltpu.bitcast(digest(*tokens), v.dtype), v[0:8, 0:L])
        tokens.clear()
        if v.shape[1] > L:
            head = jnp.concatenate([head, v[0:8, L:]], axis=1)
        return jnp.concatenate([head, v[8:]], axis=0)

    def k_unit(c, t):
        r = slice(c * rk, (c + 1) * rk)
        if t < 3:
            xt = x_v[t * tw:(t + 1) * tw, :]
        else:
            xt = jnp.concatenate([packed(xp_v.at[n], t * tw, tw) for n in range(D // L)], axis=1)
        more = 8 if c == D // rk - 1 else 0
        w = _unpack(tie(wkt_v[c * rk // 2:(c + 1) * rk // 2 + more, :]))
        kt = lax.dot_general(w, xt, NT, preferred_element_type=F32)

        def post():
            if more:
                route(t * tw, kt[rk:rk + 8], kt[rk + 8:])
            tokens.append(besti_v[...])
            pk = _phi(tie(kt[:rk]))
            zs = pk[:, 0:L]
            for j in range(1, tw // L):
                zs = zs + pk[:, j * L:(j + 1) * L]
            if t > 0:
                zs = zs + z_v[r, :]
            if t == nl - 1:
                zs = jnp.broadcast_to(jnp.sum(zs, axis=-1, keepdims=True), zs.shape)
            z_v[r, :] = zs
            pk_v[c * rk // 2:(c + 1) * rk // 2, t * tw:(t + 1) * tw] = _pack(pk.astype(BF16))
        return post

    def g_unit(c, n):
        cols = slice(n * L, (n + 1) * L)
        g = jnp.dot(packed(pk_v, c * rc, rc), packed(xp_v.at[n], 0, S), preferred_element_type=F32)

        def post():
            g_v[c * rc // 2:(c + 1) * rc // 2, cols] = _pack(tie(g).astype(BF16))
        return post

    def kv_unit(j):
        q = slice(j * L, (j + 1) * L)
        kv = jnp.dot(packed(g_v, j * L, L), wv_v[:, q], preferred_element_type=F32)

        def post():
            same_head = (lax.broadcasted_iota(jnp.int32, (L, L), 0) // dh
                         == lax.broadcasted_iota(jnp.int32, (L, L), 1) // dh)
            kvs[j] = jnp.where(same_head, kv, 0.0).astype(BF16)
        return post

    def m_unit(j):
        m = jnp.dot(kvs.pop(j), wo_v[j * L:(j + 1) * L, :], preferred_element_type=F32)

        def post():
            m_v[j * L // 2:(j + 1) * L // 2, :] = _pack(m.astype(BF16))
        return post

    kvs, sel = {}, {}

    def block_of(i):
        return lax.rem(sel["blk"] + 1 + i, nb)

    def q_unit(i, c):
        r = slice(c * rq, (c + 1) * rq)
        q = lax.dot_general(packed(wqt_v, c * rq, rq), packed(xq_v, block_of(i) * tb, tb), NT,
                            preferred_element_type=F32)

        def post():
            pq = _phi(tie(q))
            z = jnp.tile(z_v[r, :], (1, tb // L))
            den = jnp.sum((pq * z).reshape(rq // dh, dh, tb), axis=1, keepdims=True) + 1e-6
            o = (pq.reshape(rq // dh, dh, tb) * (1.0 / den)).reshape(rq, tb)
            pairs = pltpu.pack_elementwise([o[:, :L], o[:, L:]], packed_dtype=BF16)
            on_v[(i % 2) * L:(i % 2 + 1) * L, r] = pltpu.bitcast(pairs, U32).T
        return post

    def out_unit(i, n):
        cols = slice(n * L, (n + 1) * L)
        a = jnp.dot(packed(on_v, (i % 2) * tb, tb), _unpack(m_v[:, cols]), preferred_element_type=F32)

        def post():
            lo = block_of(i) * tb
            gate = gate_v[pl.ds(pl.multiple_of(lo, tb), tb), :]
            bx = packed(xp_v.at[n], lo, tb).astype(F32)
            upd = bx * 0.0
            if i == nb - 1:
                y = jnp.sum(y_v[:, cols], axis=0, keepdims=True) * sel["w"]
                is_sel = lax.broadcasted_iota(jnp.int32, (tb, L), 0) + lo == sel["idx"]
                upd = upd + jnp.where(is_sel, y, 0.0)
            o_v[i * tb:(i + 1) * tb, cols] = (gate * tie(a) + (1.0 - gate) * (bx + upd)).astype(BF16)
            if i == nb - 1:
                cp_o(i, block_of(i), n).start()
            elif n == D // L - 1:
                cp_o(i, block_of(i)).start()
        return post

    def repack(i):
        xp = _pack(x_v[i * L:(i + 1) * L, :])
        for n in range(D // L):
            xp_v[n, i * L // 2:(i + 1) * L // 2, :] = xp[:, n * L:(n + 1) * L]
        return digest(xp)

    def split_parity(t):
        lo, n = t * tw // 2, tw // 4
        a, b = (jnp.concatenate([xp_v[k, pl.ds(lo + first, n, stride=2), :] for k in range(D // L)], axis=1)
                for first in (0, 1))
        even = (a & jnp.uint32(0xFFFF)) | (b << 16)
        odd = (a >> 16) | (b & jnp.uint32(0xFFFF0000))
        xq_v[lo:lo + n, :] = even
        xq_v[lo + n:lo + 2 * n, :] = odd
        return digest(even ^ odd)

    def transpose_w(src, dst, j):
        wt = _pack(src[:, j * L:(j + 1) * L].T)
        dst[j * L // 2:(j + 1) * L // 2, :] = wt
        return digest(wt)

    def route(lo, score, logit):
        score = score.astype(BF16).astype(F32)
        gate = _sigmoid(logit)
        best, besti = best_v[...], besti_v[...]
        for k in range(tw // L):
            s8 = score[:, k * L:(k + 1) * L]
            take = (s8 > best) | ((s8 == best) & (besti == BIG))
            best = jnp.where(take, s8, best)
            besti = jnp.where(take, lax.broadcasted_iota(jnp.int32, (8, L), 1) + (lo + k * L), besti)
            gate_v[lo + k * L:lo + (k + 1) * L, :] = jnp.tile(gate[:, k * L:(k + 1) * L], (L // 8, 1)).T
        best_v[...] = best
        besti_v[...] = besti

    def select():
        best, besti = best_v[...], besti_v[...]
        m = jnp.max(best[0:1], axis=1, keepdims=True)
        mi = jnp.min(jnp.where(best[0:1] == m, besti[0:1], BIG), axis=1, keepdims=True)
        none = mi == BIG
        sel["w"] = _sigmoid(jnp.where(none, jnp.nan, m))
        sel["idx"] = jnp.where(none, 0, mi)[0, 0]
        sel["blk"] = sel["idx"] // tb

    def gather():
        base = pl.multiple_of((sel["idx"] // 16) * 16, 16)
        slab = x_v[pl.ds(base, 16), :].astype(F32)
        pick = lax.broadcasted_iota(jnp.int32, (16, 1), 0) == sel["idx"] - base
        xs = jnp.sum(jnp.where(pick, slab, 0.0), axis=0, keepdims=True)
        xb_v[...] = jnp.broadcast_to(xs, (L, D)).T

    def ffn_up(j, k):
        f, r = slice(j * L, (j + 1) * L), slice(k * kr, (k + 1) * kr)
        xb = xb_v[r, :]
        parts = []
        for w_v, h_v in ((wg_v, hg_v), (wu_v, hu_v)):
            part = jnp.sum((w_v[r, f].astype(F32) * xb).reshape(kr // 8, 8, L), axis=0)
            parts.append(part if k == 0 else h_v[:, f] + part)
            h_v[:, f] = parts[-1]
        return digest(*parts)

    def ffn_act(j):
        f = slice(j * L, (j + 1) * L)
        hg = jnp.sum(hg_v[:, f], axis=0, keepdims=True)
        hu = jnp.sum(hu_v[:, f], axis=0, keepdims=True)
        hb = jnp.broadcast_to(hg * _sigmoid(hg) * hu, (L, L)).T
        hb_v[f, :] = hb
        return digest(hb)

    def ffn_down(j, n):
        f, cols = slice(j * L, (j + 1) * L), slice(n * nw, (n + 1) * nw)
        hb = jnp.tile(hb_v[f, :], (1, nw // L))
        part = jnp.sum((wd_v[f, cols].astype(F32) * hb).reshape(L // 8, 8, nw), axis=0)
        part = part if j == 0 else y_v[:, cols] + part
        y_v[:, cols] = part
        return digest(part)

    P = functools.partial
    units, before, after = [], {}, {}
    ks = rc // rk
    units += [P(k_unit, c * ks + h, t) for c in range(nc) for t in range(2) for h in range(ks)]
    units += [P(k_unit, c, t) for t in range(2, nl) for c in range(nc * ks)]
    units += [P(g_unit, c, n) for c in range(nc) for n in range(D // L)]
    q_units = lambda i: [P(q_unit, i, c) for c in range(D // rq)]
    small_units = [P(kv_unit, j) for j in range(D // L)]
    for j in range(D // L):
        small_units.insert(2 * j + 2, P(m_unit, j))
    first_q = q_units(0)
    step = len(small_units) // len(first_q)
    for j, unit in enumerate(first_q):
        units += small_units[j * step:(j + 1) * step] + [unit]
    for i in range(nb):
        if i + 1 < nb:
            units += q_units(i + 1)
        units += [P(out_unit, i, n) for n in range(D // L)]
    cost = {k_unit: rk * tw * D, g_unit: rc * L * S, kv_unit: L * L * D, m_unit: L * L * D,
            q_unit: rq * tb * D, out_unit: tb * L * D}
    clock = [0]
    for unit in units:
        clock.append(clock[-1] + cost[unit.func] / (S * D * D))

    def at(time):
        return max(u for u in range(len(units)) if clock[u] <= time + 1e-9)

    def spread(jobs, t0, t1):
        for n, job in enumerate(jobs):
            after.setdefault(at(t0 + (t1 - t0) * n / len(jobs)), []).append(job)

    assert xc == tw == tb == rc == 2 * rk == 2 * L and nc == 4 and nl == 8
    xs = lambda *ids: [cp for i in ids for cp in cp_x(i)]
    wkt = lambda c: [P(transpose_w, wk_v, wkt_v, j) for j in range(c * rc // L, (c + 1) * rc // L)]
    best_v[...] = jnp.full(best_v.shape, -jnp.inf, F32)
    besti_v[...] = jnp.full(besti_v.shape, BIG, jnp.int32)
    wkt_v[D // 2:, :] = _pack(jnp.concatenate(
        [jnp.broadcast_to(w_r, (8, D)), jnp.broadcast_to(w_g, (8, D))], axis=0).astype(BF16))
    before[0] = [wait(*cp_k(0), *xs(0)), start(*cp_k(2), *cp_k(3))] + wkt(0)[:1]
    after[0] = wkt(0)[1:]
    before[ks] = [wait(*xs(1), *cp_k(1))]
    spread(wkt(1), clock[ks], clock[2 * ks])
    before[6] = [start(*xs(2, 3))]
    before[7] = [wait(*cp_k(2), *cp_k(3))]
    spread(wkt(2) + wkt(3), clock[7], clock[11])
    before[6 * ks] = [wait(*xs(2, 3)), start(*xs(4, 5, 6, 7))]
    spread([P(repack, i) for i in (6, 7, 4, 5, 0, 1, 2, 3)], clock[6 * ks], clock[12 * ks])
    before[12 * ks] = [wait(*xs(4, 5, 6, 7)), start(*cp_qvo(), *cp_up(0))]
    spread([P(repack, i) for i in range(8, 16)], clock[12 * ks], clock[20 * ks])
    spread([P(split_parity, t) for t in range(nl)], 1.1, 1.6)
    before.setdefault(at(t_up - lead), []).append(start(*cp_up(1)))
    before.setdefault(at(t_mid - lead), []).append(start(*cp_d()))
    u_sel = at(t_sel)
    after.setdefault(u_sel, []).append(select)
    after.setdefault(u_sel + 1, []).append(gather)
    assert at(t_up) >= u_sel + 2
    before.setdefault(at(t_up), []).append(wait(*cp_qvo(), *cp_up(0)))
    ups = lambda j0, j1: [job for j in range(j0, j1)
                          for job in [P(ffn_up, j, k) for k in range(D // kr)] + [P(ffn_act, j)]]
    spread(ups(0, fh // L), t_up, t_mid)
    before.setdefault(at(t_mid), []).append(wait(*cp_up(1)))
    spread(ups(fh // L, F // L), t_mid, t_down)
    spread([P(transpose_w, wq_v, wqt_v, j) for j in range(D // L)], t_up, 1.97)
    before.setdefault(at(t_down), []).append(wait(*cp_d()))
    spread([P(ffn_down, j, n) for j in range(F // L) for n in range(D // nw)],
           t_down, clock[len(units) - D // L - 2])

    posts = []
    for u, unit in enumerate(units):
        for job in before.get(u, []):
            job()
        posts.append(unit())
        if len(posts) > skew:
            posts.pop(0)()
        for job in after.get(u, []):
            token = job()
            if token is not None:
                tokens.append(token)
    for post in posts:
        post()
    for i in range(nb - 1):
        cp_o(i, block_of(i)).wait()
    for n in range(D // L):
        cp_o(nb - 1, block_of(nb - 1), n).wait()


def _build(flags=FLAGS, **tuning):
    def run(A_x, A_wqkv, A_wo, B_x, B_w_r, B_w_gate, B_w_up, B_w_down, gate_w):
        B, S, D = A_x.shape
        F = B_w_gate.shape[1]
        hbm = pl.BlockSpec(memory_space=pl.ANY)
        vmem, dma = pltpu.VMEM, pltpu.SemaphoreType.DMA
        out = pl.pallas_call(
            functools.partial(_kernel, **tuning),
            out_shape=jax.ShapeDtypeStruct((S, D), BF16),
            in_specs=[hbm] * 8,
            out_specs=hbm,
            scratch_shapes=[
                vmem((S, D), BF16),
                vmem((2, D // 128, 128), BF16),
                vmem((D, D), BF16), vmem((D, D), BF16),
                vmem((D, D), BF16), vmem((D, D), BF16),
                vmem((D, F), BF16), vmem((D, F), BF16), vmem((F, D), BF16),
                vmem((D // 128, S // 2 + 8, 128), U32), vmem((S // 2, D), U32),
                vmem((D // 2, D), U32), vmem((D // 2 + 8, D), U32),
                vmem((D // 2, S), U32),
                vmem((D // 2, D), U32), vmem((D // 2, D), U32),
                vmem((256, D), U32),
                vmem((D, 128), F32), vmem((S, 128), F32),
                vmem((8, 128), F32), vmem((8, 128), jnp.int32),
                vmem((D, 128), F32),
                vmem((8, F), F32), vmem((8, F), F32), vmem((F, 128), F32),
                vmem((8, D), F32),
                vmem((S, D), BF16),
                dma((2,)), dma((S // 256,)), dma((4,)), dma((D // 256,)), dma((S // 256 + D // 128 - 1,)),
            ],
            compiler_params=pltpu.CompilerParams(
                vmem_limit_bytes=110 * 1024 * 1024, flags=flags),
        )(A_x.reshape(S, D), A_wqkv, A_wo, B_w_r.reshape(D // 128, 128),
          B_w_gate, B_w_up, B_w_down, gate_w.reshape(D // 128, 128))
        return out.reshape(B, S, D)
    return run


@jax.jit
def pallas_gated_mix__linear_attn_block__moe_arch_mod__prompt_kernel(
    A_x: jax.Array,
    A_wqkv: jax.Array,
    A_wo: jax.Array,
    B_x: jax.Array,
    B_w_r: jax.Array,
    B_w_gate: jax.Array,
    B_w_up: jax.Array,
    B_w_down: jax.Array,
    gate_w: jax.Array,
):
    return _build()(A_x, A_wqkv, A_wo, B_x, B_w_r, B_w_gate, B_w_up, B_w_down, gate_w)
```

```python
import functools

import jax
import jax.numpy as jnp
from jax import lax
import jax.experimental.pallas as pl
import jax.experimental.pallas.tpu as pltpu

F32 = jnp.float32
BF16 = jnp.bfloat16
U32 = jnp.uint32
HEADS = 32
BIG = 1 << 30
FLAGS = {"XLA_TPU_EVENLY_DISTRIBUTE_CRITICAL_NODES": True}
NT = (((1,), (1,)), ((), ()))
TN = (((0,), (0,)), ((), ()))


def _phi(t):
    return jnp.where(t > 0, t + 1.0, jnp.exp(t)) + 1e-6


def _sigmoid(t):
    return 1.0 / (1.0 + jnp.exp(-t))


def _pack(v):
    return pltpu.bitcast(v, jnp.uint32)


def _unpack(v):
    return pltpu.bitcast(v, BF16)


def _kernel(x_hbm, wqkv_hbm, wo_hbm, wr_hbm, wg_hbm, wu_hbm, wd_hbm, gw_hbm,
            out_hbm,
            x_v, vec_v, wq_v, wk_v, wv_v, wo_v, wg_v, wu_v, wd_v,
            xp_v, xq_v, wqt_v, wkt_v, pk_v, g_v, m_v, on_v, z_v, gate_v, best_v, besti_v,
            xb_v, hg_v, hu_v, hb_v, y_v, o_v,
            sem_s, sem_x, sem_w, sem_k, sem_o,
            rc=256, rk=128, rq=128, tw=256, tb=256, xc=256, kr=256, nw=512, ns=4, skew=1,
            u_k1=1, lead=0.05, t_sel=1.05, t_up=1.72, t_mid=2.35, t_down=3.1):
    S, D = x_v.shape
    F = wg_v.shape[1]
    L = 128
    nc = D // rc
    nl = S // tw
    nb = S // tb
    dh = D // HEADS
    fh = F // 2

    def copies(src, dst, sem, rows, cols, shift, n):
        (r0, nr), (c0, ncol) = rows, cols
        return [pltpu.make_async_copy(src.at[pl.ds(r0 + k * nr // n, nr // n), pl.ds(c0 + shift, ncol)],
                                      dst.at[pl.ds(r0 + k * nr // n, nr // n), pl.ds(c0, ncol)], sem)
                for k in range(n)]

    cp_x = lambda i: copies(x_hbm, x_v, sem_x.at[i], (i * xc, xc), (0, D), 0, ns if i == 0 else 1)
    cp_k = lambda c: copies(wqkv_hbm, wk_v, sem_k.at[c], (0, D), (c * rc, rc), D, ns if c == 0 else 1)
    cp_qvo = lambda: (copies(wqkv_hbm, wq_v, sem_w.at[0], (0, D), (0, D), 0, 2)
                      + copies(wqkv_hbm, wv_v, sem_w.at[0], (0, D), (0, D), 2 * D, 2)
                      + copies(wo_hbm, wo_v, sem_w.at[0], (0, D), (0, D), 0, 2))
    cp_up = lambda j: (copies(wg_hbm, wg_v, sem_w.at[1 + j], (0, D), (j * fh, fh), 0, 2)
                       + copies(wu_hbm, wu_v, sem_w.at[1 + j], (0, D), (j * fh, fh), 0, 2))
    cp_d = lambda: copies(wd_hbm, wd_v, sem_w.at[3], (0, F), (0, D), 0, 4)

    def cp_o(i, t, n=None):
        cols = pl.ds(0, D) if n is None else pl.ds(n * L, L)
        return pltpu.make_async_copy(o_v.at[pl.ds(i * tb, tb), cols],
                                     out_hbm.at[pl.ds(pl.multiple_of(t * tb, tb), tb), cols],
                                     sem_o.at[i + (n or 0)])

    def start(*cps):
        return lambda: [cp.start() for cp in cps] and None

    def wait(*cps):
        return lambda: [cp.wait() for cp in cps] and None

    def packed(ref, lo, n):
        if isinstance(lo, int):
            return _unpack(ref[lo // 2:(lo + n) // 2, :])
        return _unpack(ref[pl.ds(pl.multiple_of(lo // 2, n // 2), n // 2), :])

    tokens = []
    start(*cp_k(0), *cp_x(0))()
    small = [pltpu.make_async_copy(src, vec_v.at[j], sem_s.at[j]) for j, src in enumerate((wr_hbm, gw_hbm))]
    start(*small, *cp_k(1))()
    wait(*small)()
    w_r, w_g = vec_v[0].astype(F32), vec_v[1].astype(F32)
    never = (pltpu.bitcast(w_g, jnp.int32) & 0xFFFF) != 0
    w_g, w_r = (jnp.concatenate([w[j:j + 1, :] for j in range(D // L)], axis=1) for w in (w_g, w_r))

    def digest(*vals):
        acc = None
        for v in vals:
            v = v if v.dtype == jnp.int32 else pltpu.bitcast(v, jnp.int32)
            for i in range(v.shape[0] // 8):
                for j in range(v.shape[1] // L):
                    e = v[i * 8:(i + 1) * 8, j * L:(j + 1) * L]
                    acc = e if acc is None else acc ^ e
        return acc

    def tie(v):
        if not tokens:
            return v
        head = jnp.where(never, pltpu.bitcast(digest(*tokens), v.dtype), v[0:8, 0:L])
        tokens.clear()
        if v.shape[1] > L:
            head = jnp.concatenate([head, v[0:8, L:]], axis=1)
        return jnp.concatenate([head, v[8:]], axis=0)

    def k_unit(c, t):
        r = slice(c * rk, (c + 1) * rk)
        if t < 3:
            xt = x_v[t * tw:(t + 1) * tw, :]
        else:
            xt = jnp.concatenate([packed(xp_v.at[n], t * tw, tw) for n in range(D // L)], axis=1)
        more = 8 if c == D // rk - 1 else 0
        w = _unpack(tie(wkt_v[c * rk // 2:(c + 1) * rk // 2 + more, :]))
        kt = lax.dot_general(w, xt, NT, preferred_element_type=F32)

        def post():
            if more:
                route(t * tw, kt[rk:rk + 8], kt[rk + 8:])
            tokens.append(besti_v[...])
            pk = _phi(tie(kt[:rk]))
            zs = pk[:, 0:L]
            for j in range(1, tw // L):
                zs = zs + pk[:, j * L:(j + 1) * L]
            if t > 0:
                zs = zs + z_v[r, :]
            if t == nl - 1:
                zs = jnp.broadcast_to(jnp.sum(zs, axis=-1, keepdims=True), zs.shape)
            z_v[r, :] = zs
            pk_v[c * rk // 2:(c + 1) * rk // 2, t * tw:(t + 1) * tw] = _pack(pk.astype(BF16))
        return post

    def g_unit(c, n):
        cols = slice(n * L, (n + 1) * L)
        g = jnp.dot(packed(pk_v, c * rc, rc), packed(xp_v.at[n], 0, S), preferred_element_type=F32)

        def post():
            g_v[c * rc // 2:(c + 1) * rc // 2, cols] = _pack(tie(g).astype(BF16))
        return post

    def kv_unit(j):
        q = slice(j * L, (j + 1) * L)
        kv = jnp.dot(packed(g_v, j * L, L), wv_v[:, q], preferred_element_type=F32)

        def post():
            same_head = (lax.broadcasted_iota(jnp.int32, (L, L), 0) // dh
                         == lax.broadcasted_iota(jnp.int32, (L, L), 1) // dh)
            kvs[j] = jnp.where(same_head, kv, 0.0).astype(BF16)
        return post

    def m_unit(j):
        m = jnp.dot(kvs.pop(j), wo_v[j * L:(j + 1) * L, :], preferred_element_type=F32)

        def post():
            m_v[j * L // 2:(j + 1) * L // 2, :] = _pack(m.astype(BF16))
        return post

    kvs, sel = {}, {}

    def block_of(i):
        return lax.rem(sel["blk"] + 1 + i, nb)

    def q_unit(i, c):
        r = slice(c * rq, (c + 1) * rq)
        q = lax.dot_general(packed(wqt_v, c * rq, rq), packed(xq_v, block_of(i) * tb, tb), NT,
                            preferred_element_type=F32)

        def post():
            pq = _phi(tie(q))
            z = jnp.tile(z_v[r, :], (1, tb // L))
            den = jnp.sum((pq * z).reshape(rq // dh, dh, tb), axis=1, keepdims=True) + 1e-6
            o = (pq.reshape(rq // dh, dh, tb) * (1.0 / den)).reshape(rq, tb)
            pairs = pltpu.pack_elementwise([o[:, :L], o[:, L:]], packed_dtype=BF16)
            on_v[(i % 2) * L:(i % 2 + 1) * L, r] = pltpu.bitcast(pairs, U32).T
        return post

    def out_unit(i, n):
        cols = slice(n * L, (n + 1) * L)
        a = jnp.dot(packed(on_v, (i % 2) * tb, tb), _unpack(m_v[:, cols]), preferred_element_type=F32)

        def post():
            lo = block_of(i) * tb
            gate = gate_v[pl.ds(pl.multiple_of(lo, tb), tb), :]
            bx = packed(xp_v.at[n], lo, tb).astype(F32)
            upd = bx * 0.0
            if i == nb - 1:
                y = jnp.sum(y_v[:, cols], axis=0, keepdims=True) * sel["w"]
                is_sel = lax.broadcasted_iota(jnp.int32, (tb, L), 0) + lo == sel["idx"]
                upd = upd + jnp.where(is_sel, y, 0.0)
            o_v[i * tb:(i + 1) * tb, cols] = (gate * tie(a) + (1.0 - gate) * (bx + upd)).astype(BF16)
            if i == nb - 1:
                cp_o(i, block_of(i), n).start()
            elif n == D // L - 1:
                cp_o(i, block_of(i)).start()
        return post

    def repack(i):
        xp = _pack(x_v[i * L:(i + 1) * L, :])
        for n in range(D // L):
            xp_v[n, i * L // 2:(i + 1) * L // 2, :] = xp[:, n * L:(n + 1) * L]
        return digest(xp)

    def split_parity(t):
        lo, n = t * tw // 2, tw // 4
        a, b = (jnp.concatenate([xp_v[k, pl.ds(lo + first, n, stride=2), :] for k in range(D // L)], axis=1)
                for first in (0, 1))
        even = (a & jnp.uint32(0xFFFF)) | (b << 16)
        odd = (a >> 16) | (b & jnp.uint32(0xFFFF0000))
        xq_v[lo:lo + n, :] = even
        xq_v[lo + n:lo + 2 * n, :] = odd
        return digest(even ^ odd)

    def transpose_w(src, dst, j):
        wt = _pack(src[:, j * L:(j + 1) * L].T)
        dst[j * L // 2:(j + 1) * L // 2, :] = wt
        return digest(wt)

    def route(lo, score, logit):
        score = score.astype(BF16).astype(F32)
        gate = _sigmoid(logit)
        best, besti = best_v[...], besti_v[...]
        for k in range(tw // L):
            s8 = score[:, k * L:(k + 1) * L]
            take = (s8 > best) | ((s8 == best) & (besti == BIG))
            best = jnp.where(take, s8, best)
            besti = jnp.where(take, lax.broadcasted_iota(jnp.int32, (8, L), 1) + (lo + k * L), besti)
            gate_v[lo + k * L:lo + (k + 1) * L, :] = jnp.tile(gate[:, k * L:(k + 1) * L], (L // 8, 1)).T
        best_v[...] = best
        besti_v[...] = besti

    def select():
        best, besti = best_v[...], besti_v[...]
        m = jnp.max(best[0:1], axis=1, keepdims=True)
        mi = jnp.min(jnp.where(best[0:1] == m, besti[0:1], BIG), axis=1, keepdims=True)
        none = mi == BIG
        sel["w"] = _sigmoid(jnp.where(none, jnp.nan, m))
        sel["idx"] = jnp.where(none, 0, mi)[0, 0]
        sel["blk"] = sel["idx"] // tb

    def gather():
        base = pl.multiple_of((sel["idx"] // 16) * 16, 16)
        slab = x_v[pl.ds(base, 16), :].astype(F32)
        pick = lax.broadcasted_iota(jnp.int32, (16, 1), 0) == sel["idx"] - base
        xs = jnp.sum(jnp.where(pick, slab, 0.0), axis=0, keepdims=True)
        xb_v[...] = jnp.broadcast_to(xs, (L, D)).T

    def ffn_up(j, k):
        f, r = slice(j * L, (j + 1) * L), slice(k * kr, (k + 1) * kr)
        xb = xb_v[r, :]
        parts = []
        for w_v, h_v in ((wg_v, hg_v), (wu_v, hu_v)):
            part = jnp.sum((w_v[r, f].astype(F32) * xb).reshape(kr // 8, 8, L), axis=0)
            parts.append(part if k == 0 else h_v[:, f] + part)
            h_v[:, f] = parts[-1]
        return digest(*parts)

    def ffn_act(j):
        f = slice(j * L, (j + 1) * L)
        hg = jnp.sum(hg_v[:, f], axis=0, keepdims=True)
        hu = jnp.sum(hu_v[:, f], axis=0, keepdims=True)
        hb = jnp.broadcast_to(hg * _sigmoid(hg) * hu, (L, L)).T
        hb_v[f, :] = hb
        return digest(hb)

    def ffn_down(j, n):
        f, cols = slice(j * L, (j + 1) * L), slice(n * nw, (n + 1) * nw)
        hb = jnp.tile(hb_v[f, :], (1, nw // L))
        part = jnp.sum((wd_v[f, cols].astype(F32) * hb).reshape(L // 8, 8, nw), axis=0)
        part = part if j == 0 else y_v[:, cols] + part
        y_v[:, cols] = part
        return digest(part)

    P = functools.partial
    units, before, after = [], {}, {}
    ks = rc // rk
    first = [(0, 0), (1, 0), (0, 1), (1, 1), (2, 0), (2, 1), (3, 0), (3, 1)]
    units += [P(k_unit, c * ks + h, t) for c, t in first for h in range(ks)]
    units += [P(k_unit, c, t) for t in range(2, nl) for c in range(nc * ks)]
    units += [P(g_unit, c, n) for c in range(nc) for n in range(D // L)]
    q_units = lambda i: [P(q_unit, i, c) for c in range(D // rq)]
    small_units = [P(kv_unit, j) for j in range(D // L)]
    for j in range(D // L):
        small_units.insert(2 * j + 2, P(m_unit, j))
    first_q = q_units(0)
    step = len(small_units) // len(first_q)
    for j, unit in enumerate(first_q):
        units += small_units[j * step:(j + 1) * step] + [unit]
    for i in range(nb):
        if i + 1 < nb:
            units += q_units(i + 1)
        units += [P(out_unit, i, n) for n in range(D // L)]
    cost = {k_unit: rk * tw * D, g_unit: rc * L * S, kv_unit: L * L * D, m_unit: L * L * D,
            q_unit: rq * tb * D, out_unit: tb * L * D}
    clock = [0]
    for unit in units:
        clock.append(clock[-1] + cost[unit.func] / (S * D * D))

    def at(time):
        return max(u for u in range(len(units)) if clock[u] <= time + 1e-9)

    def spread(jobs, t0, t1):
        for n, job in enumerate(jobs):
            after.setdefault(at(t0 + (t1 - t0) * n / len(jobs)), []).append(job)

    assert xc == tw == tb == rc == 2 * rk == 2 * L and nc == 4 and nl == 8
    xs = lambda *ids: [cp for i in ids for cp in cp_x(i)]
    wkt = lambda c: [P(transpose_w, wk_v, wkt_v, j) for j in range(c * rc // L, (c + 1) * rc // L)]
    best_v[...] = jnp.full(best_v.shape, -jnp.inf, F32)
    besti_v[...] = jnp.full(besti_v.shape, BIG, jnp.int32)
    wkt_v[D // 2:, :] = _pack(jnp.concatenate(
        [jnp.broadcast_to(w_r, (8, D)), jnp.broadcast_to(w_g, (8, D))], axis=0).astype(BF16))
    j0, j1, j2, j3 = wkt(0) + wkt(1)
    before[0] = [wait(*cp_k(0), *xs(0)), start(*xs(1), *cp_k(2)), j0]
    before[u_k1] = [wait(*cp_k(1)), start(*cp_k(3))] + [j2] * (u_k1 == 2)
    after[0], after[1], after[2] = [j1], [j2] * (u_k1 == 1), [j3]
    before[4] = [wait(*xs(1))]
    before[6] = [start(*xs(2, 3))]
    before[7] = [wait(*cp_k(2), *cp_k(3))]
    spread(wkt(2) + wkt(3), clock[7], clock[11])
    before[6 * ks] = [wait(*xs(2, 3)), start(*xs(4, 5, 6, 7))]
    spread([P(repack, i) for i in (6, 7, 4, 5, 0, 1, 2, 3)], clock[6 * ks], clock[12 * ks])
    before[12 * ks] = [wait(*xs(4, 5, 6, 7)), start(*cp_qvo(), *cp_up(0))]
    spread([P(repack, i) for i in range(8, 16)], clock[12 * ks], clock[20 * ks])
    spread([P(split_parity, t) for t in range(nl)], 1.1, 1.6)
    before.setdefault(at(t_up - lead), []).append(start(*cp_up(1)))
    before.setdefault(at(t_mid - lead), []).append(start(*cp_d()))
    u_sel = at(t_sel)
    after.setdefault(u_sel, []).append(select)
    after.setdefault(u_sel + 1, []).append(gather)
    assert at(t_up) >= u_sel + 2
    before.setdefault(at(t_up), []).append(wait(*cp_qvo(), *cp_up(0)))
    ups = lambda j0, j1: [job for j in range(j0, j1)
                          for job in [P(ffn_up, j, k) for k in range(D // kr)] + [P(ffn_act, j)]]
    spread(ups(0, fh // L), t_up, t_mid)
    before.setdefault(at(t_mid), []).append(wait(*cp_up(1)))
    spread(ups(fh // L, F // L), t_mid, t_down)
    spread([P(transpose_w, wq_v, wqt_v, j) for j in range(D // L)], t_up, 1.97)
    before.setdefault(at(t_down), []).append(wait(*cp_d()))
    spread([P(ffn_down, j, n) for j in range(F // L) for n in range(D // nw)],
           t_down, clock[len(units) - D // L - 2])

    posts = []
    for u, unit in enumerate(units):
        for job in before.get(u, []):
            job()
        posts.append(unit())
        if len(posts) > skew:
            posts.pop(0)()
        for job in after.get(u, []):
            token = job()
            if token is not None:
                tokens.append(token)
    for post in posts:
        post()
    for i in range(nb - 1):
        cp_o(i, block_of(i)).wait()
    for n in range(D // L):
        cp_o(nb - 1, block_of(nb - 1), n).wait()


def _build(flags=FLAGS, **tuning):
    def run(A_x, A_wqkv, A_wo, B_x, B_w_r, B_w_gate, B_w_up, B_w_down, gate_w):
        B, S, D = A_x.shape
        F = B_w_gate.shape[1]
        hbm = pl.BlockSpec(memory_space=pl.ANY)
        vmem, dma = pltpu.VMEM, pltpu.SemaphoreType.DMA
        out = pl.pallas_call(
            functools.partial(_kernel, **tuning),
            out_shape=jax.ShapeDtypeStruct((S, D), BF16),
            in_specs=[hbm] * 8,
            out_specs=hbm,
            scratch_shapes=[
                vmem((S, D), BF16),
                vmem((2, D // 128, 128), BF16),
                vmem((D, D), BF16), vmem((D, D), BF16),
                vmem((D, D), BF16), vmem((D, D), BF16),
                vmem((D, F), BF16), vmem((D, F), BF16), vmem((F, D), BF16),
                vmem((D // 128, S // 2 + 8, 128), U32), vmem((S // 2, D), U32),
                vmem((D // 2, D), U32), vmem((D // 2 + 8, D), U32),
                vmem((D // 2, S), U32),
                vmem((D // 2, D), U32), vmem((D // 2, D), U32),
                vmem((256, D), U32),
                vmem((D, 128), F32), vmem((S, 128), F32),
                vmem((8, 128), F32), vmem((8, 128), jnp.int32),
                vmem((D, 128), F32),
                vmem((8, F), F32), vmem((8, F), F32), vmem((F, 128), F32),
                vmem((8, D), F32),
                vmem((S, D), BF16),
                dma((2,)), dma((S // 256,)), dma((4,)), dma((D // 256,)), dma((S // 256 + D // 128 - 1,)),
            ],
            compiler_params=pltpu.CompilerParams(
                vmem_limit_bytes=110 * 1024 * 1024, flags=flags),
        )(A_x.reshape(S, D), A_wqkv, A_wo, B_w_r.reshape(D // 128, 128),
          B_w_gate, B_w_up, B_w_down, gate_w.reshape(D // 128, 128))
        return out.reshape(B, S, D)
    return run


@jax.jit
def pallas_gated_mix__linear_attn_block__moe_arch_mod__prompt_kernel(
    A_x: jax.Array,
    A_wqkv: jax.Array,
    A_wo: jax.Array,
    B_x: jax.Array,
    B_w_r: jax.Array,
    B_w_gate: jax.Array,
    B_w_up: jax.Array,
    B_w_down: jax.Array,
    gate_w: jax.Array,
):
    return _build()(A_x, A_wqkv, A_wo, B_x, B_w_r, B_w_gate, B_w_up, B_w_down, gate_w)
```

```python
import functools

import jax
import jax.numpy as jnp
from jax import lax
import jax.experimental.pallas as pl
import jax.experimental.pallas.tpu as pltpu

F32 = jnp.float32
BF16 = jnp.bfloat16
U32 = jnp.uint32
HEADS = 32
BIG = 1 << 30
FLAGS = {"XLA_TPU_EVENLY_DISTRIBUTE_CRITICAL_NODES": True}
NT = (((1,), (1,)), ((), ()))


def _phi(t):
    return jnp.where(t > 0, t + 1.0, jnp.exp(t)) + 1e-6


def _sigmoid(t):
    return 1.0 / (1.0 + jnp.exp(-t))


def _pack(v):
    return pltpu.bitcast(v, jnp.uint32)


def _unpack(v):
    return pltpu.bitcast(v, BF16)


def _kernel(x_hbm, wqkv_hbm, wo_hbm, wr_hbm, wg_hbm, wu_hbm, wd_hbm, gw_hbm,
            out_hbm,
            x_v, vec_v, wq_v, wk_v, wv_v, wo_v, wg_v, wu_v, wd_v,
            xp_v, xq_v, wqt_v, wkt_v, pk_v, g_v, m_v, on_v, z_v, gate_v, best_v, besti_v,
            xb_v, hg_v, hu_v, hb_v, y_v, o_v,
            sem_s, sem_x, sem_w, sem_k, sem_o,
            rc=256, rk=128, rq=128, tw=256, tb=256, xc=256, kr=256, nw=512, ns=4, skew=1,
            lead=0.1, t_sel=1.05, t_up=1.7, t_mid=2.35, t_down=3.1):
    S, D = x_v.shape
    F = wg_v.shape[1]
    L = 128
    nc = D // rc
    nl = S // tw
    nb = S // tb
    dh = D // HEADS
    fh = F // 2

    def copies(src, dst, sem, rows, cols, shift, n):
        (r0, nr), (c0, ncol) = rows, cols
        return [pltpu.make_async_copy(src.at[pl.ds(r0 + k * nr // n, nr // n), pl.ds(c0 + shift, ncol)],
                                      dst.at[pl.ds(r0 + k * nr // n, nr // n), pl.ds(c0, ncol)], sem)
                for k in range(n)]

    cp_x = lambda i: copies(x_hbm, x_v, sem_x.at[i], (i * xc, xc), (0, D), 0, ns if i == 0 else 1)
    cp_k = lambda c: copies(wqkv_hbm, wk_v, sem_k.at[c], (0, D), (c * rc, rc), D, ns if c == 0 else 1)
    cp_qvo = lambda: (copies(wqkv_hbm, wq_v, sem_w.at[0], (0, D), (0, D), 0, 2)
                      + copies(wqkv_hbm, wv_v, sem_w.at[0], (0, D), (0, D), 2 * D, 2)
                      + copies(wo_hbm, wo_v, sem_w.at[0], (0, D), (0, D), 0, 2))
    cp_up = lambda j: (copies(wg_hbm, wg_v, sem_w.at[1 + j], (0, D), (j * fh, fh), 0, 2)
                       + copies(wu_hbm, wu_v, sem_w.at[1 + j], (0, D), (j * fh, fh), 0, 2))
    cp_d = lambda: copies(wd_hbm, wd_v, sem_w.at[3], (0, F), (0, D), 0, 4)

    def cp_o(i, t, n=None):
        cols = pl.ds(0, D) if n is None else pl.ds(n * L, L)
        return pltpu.make_async_copy(o_v.at[pl.ds(i * tb, tb), cols],
                                     out_hbm.at[pl.ds(pl.multiple_of(t * tb, tb), tb), cols],
                                     sem_o.at[i + (n or 0)])

    def start(*cps):
        return lambda: [cp.start() for cp in cps] and None

    def wait(*cps):
        return lambda: [cp.wait() for cp in cps] and None

    def packed(ref, lo, n):
        if isinstance(lo, int):
            return _unpack(ref[lo // 2:(lo + n) // 2, :])
        return _unpack(ref[pl.ds(pl.multiple_of(lo // 2, n // 2), n // 2), :])

    tokens = []
    start(*cp_k(0), *cp_x(0))()
    small = [pltpu.make_async_copy(src, vec_v.at[j], sem_s.at[j]) for j, src in enumerate((wr_hbm, gw_hbm))]
    start(*small, *cp_k(1))()
    wait(*small)()
    w_r, w_g = vec_v[0].astype(F32), vec_v[1].astype(F32)
    never = (pltpu.bitcast(w_g, jnp.int32) & 0xFFFF) != 0
    w_g, w_r = (jnp.concatenate([w[j:j + 1, :] for j in range(D // L)], axis=1) for w in (w_g, w_r))

    def digest(*vals):
        acc = None
        for v in vals:
            v = v if v.dtype == jnp.int32 else pltpu.bitcast(v, jnp.int32)
            for i in range(v.shape[0] // 8):
                for j in range(v.shape[1] // L):
                    e = v[i * 8:(i + 1) * 8, j * L:(j + 1) * L]
                    acc = e if acc is None else acc ^ e
        return acc

    def tie(v):
        if not tokens:
            return v
        head = jnp.where(never, pltpu.bitcast(digest(*tokens), v.dtype), v[0:8, 0:L])
        tokens.clear()
        if v.shape[1] > L:
            head = jnp.concatenate([head, v[0:8, L:]], axis=1)
        return jnp.concatenate([head, v[8:]], axis=0)

    def k_unit(c, t):
        r = slice(c * rk, (c + 1) * rk)
        if t < 3:
            xt = x_v[t * tw:(t + 1) * tw, :]
        else:
            xt = jnp.concatenate([packed(xp_v.at[n], t * tw, tw) for n in range(D // L)], axis=1)
        more = 8 if c == D // rk - 1 else 0
        w = _unpack(tie(wkt_v[c * rk // 2:(c + 1) * rk // 2 + more, :]))
        kt = lax.dot_general(w, xt, NT, preferred_element_type=F32)

        def post():
            if more:
                route(t * tw, kt[rk:rk + 8], kt[rk + 8:])
            tokens.append(besti_v[...])
            pk = _phi(tie(kt[:rk]))
            zs = pk[:, 0:L]
            for j in range(1, tw // L):
                zs = zs + pk[:, j * L:(j + 1) * L]
            if t > 0:
                zs = zs + z_v[r, :]
            if t == nl - 1:
                zs = jnp.broadcast_to(jnp.sum(zs, axis=-1, keepdims=True), zs.shape)
            z_v[r, :] = zs
            pk_v[c * rk // 2:(c + 1) * rk // 2, t * tw:(t + 1) * tw] = _pack(pk.astype(BF16))
        return post

    def g_unit(c, n):
        cols = slice(n * L, (n + 1) * L)
        g = jnp.dot(packed(pk_v, c * rc, rc), packed(xp_v.at[n], 0, S), preferred_element_type=F32)

        def post():
            g_v[c * rc // 2:(c + 1) * rc // 2, cols] = _pack(tie(g).astype(BF16))
        return post

    def kv_unit(j):
        q = slice(j * L, (j + 1) * L)
        kv = jnp.dot(packed(g_v, j * L, L), wv_v[:, q], preferred_element_type=F32)

        def post():
            same_head = (lax.broadcasted_iota(jnp.int32, (L, L), 0) // dh
                         == lax.broadcasted_iota(jnp.int32, (L, L), 1) // dh)
            kvs[j] = jnp.where(same_head, kv, 0.0).astype(BF16)
        return post

    def m_unit(j):
        m = jnp.dot(kvs.pop(j), wo_v[j * L:(j + 1) * L, :], preferred_element_type=F32)

        def post():
            m_v[j * L // 2:(j + 1) * L // 2, :] = _pack(m.astype(BF16))
        return post

    kvs, sel = {}, {}

    def block_of(i):
        return lax.rem(sel["blk"] + 1 + i, nb)

    def q_unit(i, c):
        r = slice(c * rq, (c + 1) * rq)
        q = lax.dot_general(packed(wqt_v, c * rq, rq), packed(xq_v, block_of(i) * tb, tb), NT,
                            preferred_element_type=F32)

        def post():
            pq = _phi(tie(q))
            z = jnp.tile(z_v[r, :], (1, tb // L))
            den = jnp.sum((pq * z).reshape(rq // dh, dh, tb), axis=1, keepdims=True) + 1e-6
            o = (pq.reshape(rq // dh, dh, tb) * (1.0 / den)).reshape(rq, tb)
            bits = pltpu.bitcast(o.astype(BF16).astype(F32), U32)
            pairs = (bits[:, :L] >> 16) | (bits[:, L:] & jnp.uint32(0xFFFF0000))
            on_v[(i % 2) * L:(i % 2 + 1) * L, r] = pairs.T
        return post

    def out_unit(i, n):
        cols = slice(n * L, (n + 1) * L)
        a = jnp.dot(packed(on_v, (i % 2) * tb, tb), _unpack(m_v[:, cols]), preferred_element_type=F32)

        def post():
            lo = block_of(i) * tb
            gate = gate_v[pl.ds(pl.multiple_of(lo, tb), tb), :]
            bx = packed(xp_v.at[n], lo, tb).astype(F32)
            upd = bx * 0.0
            if i == nb - 1:
                y = jnp.sum(y_v[:, cols], axis=0, keepdims=True) * sel["w"]
                is_sel = lax.broadcasted_iota(jnp.int32, (tb, L), 0) + lo == sel["idx"]
                upd = upd + jnp.where(is_sel, y, 0.0)
            o_v[i * tb:(i + 1) * tb, cols] = (gate * tie(a) + (1.0 - gate) * (bx + upd)).astype(BF16)
            if i == nb - 1:
                cp_o(i, block_of(i), n).start()
            elif n == D // L - 1:
                cp_o(i, block_of(i)).start()
        return post

    def repack(i):
        xp = _pack(x_v[i * L:(i + 1) * L, :])
        for n in range(D // L):
            xp_v[n, i * L // 2:(i + 1) * L // 2, :] = xp[:, n * L:(n + 1) * L]
        return digest(xp)

    def split_parity(t):
        lo, n = t * tw // 2, tw // 4
        a, b = (jnp.concatenate([xp_v[k, pl.ds(lo + first, n, stride=2), :] for k in range(D // L)], axis=1)
                for first in (0, 1))
        even = (a & jnp.uint32(0xFFFF)) | (b << 16)
        odd = (a >> 16) | (b & jnp.uint32(0xFFFF0000))
        xq_v[lo:lo + n, :] = even
        xq_v[lo + n:lo + 2 * n, :] = odd
        return digest(even ^ odd)

    def transpose_w(src, dst, j):
        wt = _pack(src[:, j * L:(j + 1) * L].T)
        dst[j * L // 2:(j + 1) * L // 2, :] = wt
        return digest(wt)

    def route(lo, score, logit):
        score = score.astype(BF16).astype(F32)
        gate = _sigmoid(logit)
        best, besti = best_v[...], besti_v[...]
        for k in range(tw // L):
            s8 = score[:, k * L:(k + 1) * L]
            take = (s8 > best) | ((s8 == best) & (besti == BIG))
            best = jnp.where(take, s8, best)
            besti = jnp.where(take, lax.broadcasted_iota(jnp.int32, (8, L), 1) + (lo + k * L), besti)
            gate_v[lo + k * L:lo + (k + 1) * L, :] = jnp.tile(gate[:, k * L:(k + 1) * L], (L // 8, 1)).T
        best_v[...] = best
        besti_v[...] = besti

    def select():
        best, besti = best_v[...], besti_v[...]
        m = jnp.max(best[0:1], axis=1, keepdims=True)
        mi = jnp.min(jnp.where(best[0:1] == m, besti[0:1], BIG), axis=1, keepdims=True)
        none = mi == BIG
        sel["w"] = _sigmoid(jnp.where(none, jnp.nan, m))
        sel["idx"] = jnp.where(none, 0, mi)[0, 0]
        sel["blk"] = sel["idx"] // tb

    def gather():
        base = pl.multiple_of((sel["idx"] // 16) * 16, 16)
        slab = x_v[pl.ds(base, 16), :].astype(F32)
        pick = lax.broadcasted_iota(jnp.int32, (16, 1), 0) == sel["idx"] - base
        xs = jnp.sum(jnp.where(pick, slab, 0.0), axis=0, keepdims=True)
        xb_v[...] = jnp.broadcast_to(xs, (L, D)).T

    def ffn_up(j, k):
        f, r = slice(j * L, (j + 1) * L), slice(k * kr, (k + 1) * kr)
        xb = xb_v[r, :]
        parts = []
        for w_v, h_v in ((wg_v, hg_v), (wu_v, hu_v)):
            part = jnp.sum((w_v[r, f].astype(F32) * xb).reshape(kr // 8, 8, L), axis=0)
            parts.append(part if k == 0 else h_v[:, f] + part)
            h_v[:, f] = parts[-1]
        return digest(*parts)

    def ffn_act(j):
        f = slice(j * L, (j + 1) * L)
        hg = jnp.sum(hg_v[:, f], axis=0, keepdims=True)
        hu = jnp.sum(hu_v[:, f], axis=0, keepdims=True)
        hb = jnp.broadcast_to(hg * _sigmoid(hg) * hu, (L, L)).T
        hb_v[f, :] = hb
        return digest(hb)

    def ffn_down(j, n):
        f, cols = slice(j * L, (j + 1) * L), slice(n * nw, (n + 1) * nw)
        hb = jnp.tile(hb_v[f, :], (1, nw // L))
        part = jnp.sum((wd_v[f, cols].astype(F32) * hb).reshape(L // 8, 8, nw), axis=0)
        part = part if j == 0 else y_v[:, cols] + part
        y_v[:, cols] = part
        return digest(part)

    P = functools.partial
    units, before, after = [], {}, {}
    ks = rc // rk
    first = [(0, 0), (1, 0), (0, 1), (1, 1), (2, 0), (2, 1), (3, 0), (3, 1)]
    units += [P(k_unit, c * ks + h, t) for c, t in first for h in range(ks)]
    units += [P(k_unit, c, t) for t in range(2, nl) for c in range(nc * ks)]
    units += [P(g_unit, c, n) for c in range(nc) for n in range(D // L)]
    q_units = lambda i: [P(q_unit, i, c) for c in range(D // rq)]
    small_units = [P(kv_unit, j) for j in range(D // L)]
    for j in range(D // L):
        small_units.insert(2 * j + 2, P(m_unit, j))
    first_q = q_units(0)
    step = len(small_units) // len(first_q)
    for j, unit in enumerate(first_q):
        units += small_units[j * step:(j + 1) * step] + [unit]
    for i in range(nb):
        if i + 1 < nb:
            units += q_units(i + 1)
        units += [P(out_unit, i, n) for n in range(D // L)]
    cost = {k_unit: rk * tw * D, g_unit: rc * L * S, kv_unit: L * L * D, m_unit: L * L * D,
            q_unit: rq * tb * D, out_unit: tb * L * D}
    clock = [0]
    for unit in units:
        clock.append(clock[-1] + cost[unit.func] / (S * D * D))

    def at(time):
        return max(u for u in range(len(units)) if clock[u] <= time + 1e-9)

    def spread(jobs, t0, t1):
        for n, job in enumerate(jobs):
            after.setdefault(at(t0 + (t1 - t0) * n / len(jobs)), []).append(job)

    assert xc == tw == tb == rc == 2 * rk == 2 * L and nc == 4 and nl == 8
    xs = lambda *ids: [cp for i in ids for cp in cp_x(i)]
    wkt = lambda c: [P(transpose_w, wk_v, wkt_v, j) for j in range(c * rc // L, (c + 1) * rc // L)]
    best_v[...] = jnp.full(best_v.shape, -jnp.inf, F32)
    besti_v[...] = jnp.full(besti_v.shape, BIG, jnp.int32)
    wkt_v[D // 2:, :] = _pack(jnp.concatenate(
        [jnp.broadcast_to(w_r, (8, D)), jnp.broadcast_to(w_g, (8, D))], axis=0).astype(BF16))
    j0, j1, j2, j3 = wkt(0) + wkt(1)
    before[0] = [wait(*cp_k(0), *xs(0)), start(*xs(1), *cp_k(2)), j0]
    before[1] = [wait(*cp_k(1)), start(*cp_k(3))]
    after[0], after[1], after[2] = [j1], [j2], [j3]
    before[4] = [wait(*xs(1))]
    before[6] = [start(*xs(2, 3))]
    before[7] = [wait(*cp_k(2), *cp_k(3))]
    spread(wkt(2) + wkt(3), clock[7], clock[11])
    before[6 * ks] = [wait(*xs(2, 3)), start(*xs(4, 5, 6, 7))]
    spread([P(repack, i) for i in (6, 7, 4, 5, 0, 1, 2, 3)], clock[6 * ks], clock[12 * ks])
    before[12 * ks] = [wait(*xs(4, 5, 6, 7)), start(*cp_qvo(), *cp_up(0))]
    spread([P(repack, i) for i in range(8, 16)], clock[12 * ks], clock[20 * ks])
    spread([P(split_parity, t) for t in range(nl)], 1.1, 1.6)
    before.setdefault(at(t_up - lead), []).append(start(*cp_up(1)))
    before.setdefault(at(t_mid - lead), []).append(start(*cp_d()))
    u_sel = at(t_sel)
    after.setdefault(u_sel, []).append(select)
    after.setdefault(u_sel + 1, []).append(gather)
    assert at(t_up) >= u_sel + 2
    before.setdefault(at(t_up), []).append(wait(*cp_qvo(), *cp_up(0)))
    ups = lambda j0, j1: [job for j in range(j0, j1)
                          for job in [P(ffn_up, j, k) for k in range(D // kr)] + [P(ffn_act, j)]]
    spread(ups(0, fh // L), t_up, t_mid)
    before.setdefault(at(t_mid), []).append(wait(*cp_up(1)))
    spread(ups(fh // L, F // L), t_mid, t_down)
    spread([P(transpose_w, wq_v, wqt_v, j) for j in range(D // L)], t_up, 1.97)
    before.setdefault(at(t_down), []).append(wait(*cp_d()))
    spread([P(ffn_down, j, n) for j in range(F // L) for n in range(D // nw)],
           t_down, clock[len(units) - D // L - 2])

    posts = []
    for u, unit in enumerate(units):
        for job in before.get(u, []):
            job()
        posts.append(unit())
        if len(posts) > skew:
            posts.pop(0)()
        for job in after.get(u, []):
            token = job()
            if token is not None:
                tokens.append(token)
    for post in posts:
        post()
    for i in range(nb - 1):
        cp_o(i, block_of(i)).wait()
    for n in range(D // L):
        cp_o(nb - 1, block_of(nb - 1), n).wait()


def _build(flags=FLAGS, **tuning):
    def run(A_x, A_wqkv, A_wo, B_x, B_w_r, B_w_gate, B_w_up, B_w_down, gate_w):
        B, S, D = A_x.shape
        F = B_w_gate.shape[1]
        hbm = pl.BlockSpec(memory_space=pl.ANY)
        vmem, dma = pltpu.VMEM, pltpu.SemaphoreType.DMA
        out = pl.pallas_call(
            functools.partial(_kernel, **tuning),
            out_shape=jax.ShapeDtypeStruct((S, D), BF16),
            in_specs=[hbm] * 8,
            out_specs=hbm,
            scratch_shapes=[
                vmem((S, D), BF16),
                vmem((2, D // 128, 128), BF16),
                vmem((D, D), BF16), vmem((D, D), BF16),
                vmem((D, D), BF16), vmem((D, D), BF16),
                vmem((D, F), BF16), vmem((D, F), BF16), vmem((F, D), BF16),
                vmem((D // 128, S // 2 + 8, 128), U32), vmem((S // 2, D), U32),
                vmem((D // 2, D), U32), vmem((D // 2 + 8, D), U32),
                vmem((D // 2, S), U32),
                vmem((D // 2, D), U32), vmem((D // 2, D), U32),
                vmem((256, D), U32),
                vmem((D, 128), F32), vmem((S, 128), F32),
                vmem((8, 128), F32), vmem((8, 128), jnp.int32),
                vmem((D, 128), F32),
                vmem((8, F), F32), vmem((8, F), F32), vmem((F, 128), F32),
                vmem((8, D), F32),
                vmem((S, D), BF16),
                dma((2,)), dma((S // 256,)), dma((4,)), dma((D // 256,)), dma((S // 256 + D // 128 - 1,)),
            ],
            compiler_params=pltpu.CompilerParams(
                vmem_limit_bytes=110 * 1024 * 1024, flags=flags),
        )(A_x.reshape(S, D), A_wqkv, A_wo, B_w_r.reshape(D // 128, 128),
          B_w_gate, B_w_up, B_w_down, gate_w.reshape(D // 128, 128))
        return out.reshape(B, S, D)
    return run


@jax.jit
def pallas_gated_mix__linear_attn_block__moe_arch_mod__prompt_kernel(
    A_x: jax.Array,
    A_wqkv: jax.Array,
    A_wo: jax.Array,
    B_x: jax.Array,
    B_w_r: jax.Array,
    B_w_gate: jax.Array,
    B_w_up: jax.Array,
    B_w_down: jax.Array,
    gate_w: jax.Array,
):
    return _build()(A_x, A_wqkv, A_wo, B_x, B_w_r, B_w_gate, B_w_up, B_w_down, gate_w)
```
